```python
import jax
import jax.numpy as jnp

def _softmax(x, axis=-1):
    return jax.nn.softmax(x, axis=axis)

def _gelu(x):
    return jax.nn.gelu(x, approximate=True)

def _silu(x):
    return jax.nn.silu(x)

def _sigmoid(x):
    return jax.nn.sigmoid(x)

def _layernorm(x, axis=-1, eps=1e-05):
    m = jnp.mean(x, axis=axis, keepdims=True)
    v = jnp.var(x, axis=axis, keepdims=True)
    return (x - m) / jnp.sqrt(v + eps)

def _scatter_add(tgt, idx, src, axis=0):
    return tgt.at[idx].add(src)

def _segment_sum(src, seg, n):
    return jax.ops.segment_sum(src, seg, n)

class _Rng:

    def __init__(self, key):
        self._k = key

    def _next(self):
        self._k, sub = jax.random.split(self._k)
        return sub

    def normal(self, shape):
        return jax.random.normal(self._next(), shape, dtype=jnp.bfloat16)

    def randint(self, lo, hi, shape):
        return jax.random.randint(self._next(), shape, lo, hi, dtype=jnp.int32)

    def uniform(self, shape, lo=0.0, hi=1.0):
        return jax.random.uniform(self._next(), shape, jnp.bfloat16, lo, hi)

    def permutation(self, n):
        return jax.random.permutation(self._next(), n)
kernel_name = 'adaLN_cond__memory_aug_recurrent_mem_tr__glu_gated_swiglu__prompt'

def setup_inputs():
    _rng = _Rng(jax.random.key(int.from_bytes(__import__("os").urandom(4), "little")))
    _w = lambda a: (lambda t: t.astype(jnp.bfloat16) if jnp.issubdtype(t.dtype, jnp.floating) else t)(jnp.asarray(a))

    def _A_setup():
        B, S, Dm = (1, 2048, 1024)
        H, Dh = (32, 128)
        M, seg = (8, 32)
        seg = min(seg, S)
        S = S // seg * seg
        return {'x': _w((lambda *s: _rng.normal(s) * 0.05)(B, S, Dm)), 'mem0': _w((lambda *s: _rng.normal(s) * 0.05)(B, M, Dm)), 'Wq': _w((lambda *s: _rng.normal(s) * 0.05)(Dm, H, Dh) * Dm ** (-0.5)), 'Wk': _w((lambda *s: _rng.normal(s) * 0.05)(Dm, H, Dh) * Dm ** (-0.5)), 'Wv': _w((lambda *s: _rng.normal(s) * 0.05)(Dm, H, Dh) * Dm ** (-0.5)), 'Wo': _w((lambda *s: _rng.normal(s) * 0.05)(H, Dh, Dm) * (H * Dh) ** (-0.5)), 'seg_len': seg}
    _A_in = _A_setup()

    def _B_setup():
        B, S, D, F = (1, 2048, 1024, 3584)
        return {'x': _w((lambda *s: _rng.normal(s) * 0.05)(B, S, D)), 'w1': _w((lambda *s: _rng.normal(s) * 0.05)(D, F) * (2.0 / D) ** 0.5), 'w3': _w((lambda *s: _rng.normal(s) * 0.05)(D, F) * (2.0 / D) ** 0.5), 'w2': _w((lambda *s: _rng.normal(s) * 0.05)(F, D) * (2.0 / F) ** 0.5)}
    _B_in = _B_setup()
    return {'A_x': _A_in['x'], 'A_mem0': _A_in['mem0'], 'A_Wq': _A_in['Wq'], 'A_Wk': _A_in['Wk'], 'A_Wv': _A_in['Wv'], 'A_Wo': _A_in['Wo'], 'A_seg_len': _A_in['seg_len'], 'B_x': _B_in['x'], 'B_w1': _B_in['w1'], 'B_w3': _B_in['w3'], 'B_w2': _B_in['w2'], 'c': _w((lambda *s: _rng.normal(s) * 0.05)(1, 1024)), 'w_mod': _w((lambda *s: _rng.normal(s) * 0.05)(1024, 6 * 1024) * 1024 ** (-0.5))}

def reference(A_x, A_mem0, A_Wq, A_Wk, A_Wv, A_Wo, A_seg_len, B_x, B_w1, B_w3, B_w2, c, w_mod):

    def _A_ref(x, mem0, Wq, Wk, Wv, Wo, seg_len):
        B, S, Dm = x.shape
        H, Dh = (Wq.shape[1], Wq.shape[2])
        M = mem0.shape[1]
        scale = Dh ** (-0.5)
        n_seg = S // seg_len
        L = M + seg_len
        idx = jnp.arange(L)
        mask = (idx[:, None] < M) | (idx[:, None] >= idx[None, :])
        mem = mem0
        outs = []
        for s in range(n_seg):
            xs = x[:, s * seg_len:(s + 1) * seg_len, :].copy()
            h = jnp.concatenate([mem, xs], axis=1)
            q = jnp.einsum('btd,dhe->bhte', h, Wq)
            k = jnp.einsum('btd,dhe->bhte', h, Wk)
            v = jnp.einsum('btd,dhe->bhte', h, Wv)
            scores = jnp.einsum('bhqe,bhke->bhqk', q, k) * scale
            scores = jnp.where(mask[None, None], scores, -1000000000.0)
            p = _softmax(scores, axis=-1)
            o = jnp.einsum('bhqk,bhke->bhqe', p, v)
            o = jnp.einsum('bhte,hed->btd', o, Wo)
            mem = o[:, :M, :].copy()
            outs.append(o[:, M:, :])
        return jnp.concatenate(outs, axis=1)

    def _B_ref(x, w1, w3, w2):
        gate = jnp.einsum('bsd,df->bsf', x, w1)
        up = jnp.einsum('bsd,df->bsf', x, w3)
        h = _silu(gate) * up
        out = jnp.einsum('bsf,fd->bsd', h, w2)
        return out
    x = A_x
    mod = (_silu(c) @ w_mod).reshape(c.shape[0], 6, 1, -1)
    sa, ca, ga, sb, cb, gb = (mod[:, 0].copy(), mod[:, 1].copy(), mod[:, 2].copy(), mod[:, 3].copy(), mod[:, 4].copy(), mod[:, 5].copy())
    h = _layernorm(x, axis=-1) * (1 + ca) + sa
    x = x + ga * _A_ref(h, A_mem0, A_Wq, A_Wk, A_Wv, A_Wo, A_seg_len)
    h = _layernorm(x, axis=-1) * (1 + cb) + sb
    x = x + gb * _B_ref(h, B_w1, B_w3, B_w2)
    return x
```

```python
import functools

import jax
import jax.numpy as jnp
from jax import lax
import jax.experimental.pallas as pl
import jax.experimental.pallas.tpu as pltpu

F32 = jnp.float32
BF16 = jnp.bfloat16
LANE = 128
EPS = 1e-5


def _dot(a, b):
    return jnp.dot(a, b, preferred_element_type=F32)


def _ada_ln(x, shift, scale1):
    m = jnp.mean(x, axis=-1, keepdims=True)
    d = x - m
    v = jnp.mean(d * d, axis=-1, keepdims=True)
    return d * lax.rsqrt(v + EPS) * scale1 + shift


def _silu(x):
    return x * (1.0 / (1.0 + jnp.exp(-x)))


def _kernel(x_hbm, mem0_ref, wq_hbm, wk_hbm, wv_hbm, wo_hbm, w1_hbm, w3_hbm, w2_hbm,
            c_ref, wmod_hbm, out_hbm,
            wqkv, buf_a, buf_b, w13, ring, oring, xb, xf, mod, hb, lhs, act, fill_ref, sems, osems,
            *, S, D, H, F, M, SEG):
    NSEG = S // SEG
    XR = SEG - M
    P = S - NSEG * XR
    R = ring.shape[1]
    QOFF = R - P
    OOFF = (-NSEG * XR) % R
    ND = D // LANE
    NF = F // LANE
    HP = H // 2
    HD = H * LANE
    scale = float(LANE) ** -0.5

    def slab_copies(src, n0, n, dst_fn, sem):
        return [pltpu.make_async_copy(src.at[:, pl.ds((n0 + j) * LANE, LANE)], dst_fn(j), sem)
                for j in range(n)]

    cp_x0 = pltpu.make_async_copy(x_hbm.at[pl.ds(0, P)], xb.at[pl.ds(0, P)], sems.at[0])
    cp_x1 = pltpu.make_async_copy(x_hbm.at[pl.ds(P, S - P)], xb.at[pl.ds(P, S - P)], sems.at[1])
    cp_mod0 = slab_copies(wmod_hbm, 0, 2 * ND, lambda j: w13.at[j], sems.at[2])
    cp_mod1 = slab_copies(wmod_hbm, 2 * ND, 4 * ND, lambda j: w13.at[2 * ND + j], sems.at[3])
    cp_q = pltpu.make_async_copy(wq_hbm, buf_a, sems.at[4])
    cp_k = pltpu.make_async_copy(wk_hbm, buf_b, sems.at[5])
    cp_v = pltpu.make_async_copy(wv_hbm, buf_a, sems.at[6])
    cp_o = slab_copies(wo_hbm, 0, ND, lambda j: buf_b.at[pl.ds(j * HD, HD)], sems.at[7])
    cp_ffn = (slab_copies(w1_hbm, 0, NF, lambda j: w13.at[2 * j], sems.at[8])
              + slab_copies(w3_hbm, 0, NF, lambda j: w13.at[2 * j + 1], sems.at[8])
              + slab_copies(w2_hbm, 0, ND, lambda j: buf_a.at[pl.ds(j * F, F)], sems.at[8]))

    def start(cps):
        for cp in cps:
            cp.start()

    def wait(cps):
        for cp in cps:
            cp.wait()

    start(cp_mod0)
    cp_x0.start()
    cp_q.start()

    cc = jnp.broadcast_to(c_ref[...].astype(F32), (16, D))
    sc = _silu(cc).astype(BF16)

    def mod_part(j0, j1):
        for j in range(j0, j1):
            r = _dot(sc, w13[j])[0:8]
            if j // ND in (1, 4):
                r = r + 1.0
            mod[j // ND, :, pl.ds((j % ND) * LANE, LANE)] = r

    def modv(i):
        return mod[i, 0:1, :]

    G = 2 * (M + SEG)
    ri = lax.broadcasted_iota(jnp.int32, (G, LANE), 0)
    ci = lax.broadcasted_iota(jnp.int32, (G, LANE), 1)

    def head_pos(i):
        head = jnp.where(i < 2 * M, i // M, (i - 2 * M) // SEG)
        pos = jnp.where(i < 2 * M, i % M, M + (i - 2 * M) % SEG)
        return head, pos

    rh, rp = head_pos(ri)
    ch, cp_ = head_pos(ci)
    visible = (rp < M) | (rp >= cp_)
    fill_ref[...] = jnp.where(rh == ch, jnp.where(visible, 0.0, -1e9), -jnp.inf).astype(F32)

    wait(cp_mod0)
    cp_k.start()
    cp_x1.start()
    mod_part(0, 2 * ND)
    cp_x0.wait()

    LB = 128

    def ln0_body(i, carry):
        r0 = pl.multiple_of(i * LB, LB)
        xv = xb[pl.ds(r0, LB), :].astype(F32)
        xf[pl.ds(r0, LB), :] = xv
        hb[pl.ds(r0, LB), :] = _ada_ln(xv, modv(0), modv(1)).astype(BF16)
        return carry

    lax.fori_loop(0, P // LB, ln0_body, 0)

    def project(t, stage):
        words = stage.bitcast(jnp.uint32)

        def body(a, carry):
            view = words.at[pl.ds(pl.multiple_of(4 * a, 4), D * HP - (HP - 4))]
            for b in range(4):
                even = view[pl.ds(b, D // 2, stride=2 * HP), :]
                odd = view[pl.ds(b + HP, D // 2, stride=2 * HP), :]
                lo = (even & jnp.uint32(0xFFFF)) | (odd << 16)
                hi = (even >> 16) | (odd & jnp.uint32(0xFFFF0000))
                for i, w in enumerate((lo, hi)):
                    w = pltpu.bitcast(w, BF16)
                    n = t * H + 8 * a + 2 * b + i
                    wqkv[n] = w
                    ring[n, pl.ds(QOFF, P), :] = _dot(hb[pl.ds(0, P), :], w)
            return carry

        lax.fori_loop(0, HP // 4, body, 0)

    cp_q.wait()
    start(cp_mod1)
    project(0, buf_a)
    cp_v.start()
    cp_k.wait()
    project(1, buf_b)
    start(cp_o)
    cp_x1.wait()

    def cvt_body(i, carry):
        r0 = pl.multiple_of(P + i * LB, LB)
        xf[pl.ds(r0, LB), :] = xb[pl.ds(r0, LB), :].astype(F32)
        return carry

    lax.fori_loop(0, (S - P) // LB, cvt_body, 0)
    wait(cp_mod1)
    mod_part(2 * ND, 6 * ND)
    cp_v.wait()
    project(2, buf_a)
    start(cp_ffn)
    lhs[0:M, :] = mem0_ref[...].astype(F32)
    lhs[M:SEG, :] = _ada_ln(xf[pl.ds(P, XR), :], modv(0), modv(1))
    wait(cp_o)

    def step(s, carry):
        q_wr = pl.multiple_of(lax.rem(s * XR, R), 8)
        q_rd = pl.multiple_of(lax.rem(s * SEG + QOFF, R), 8)
        o_wr = pl.multiple_of(lax.rem(s * SEG + OOFF, R), 8)
        o_rd = pl.multiple_of(lax.rem(s * XR + OOFF, R), 8)
        h = lhs[...].astype(BF16)
        nxt = pl.multiple_of(jnp.minimum(P + (s + 1) * XR, S - XR), 8)
        lhs[M:SEG, :] = _ada_ln(xf[pl.ds(nxt, XR), :], modv(0), modv(1))
        pad = jnp.zeros((LANE - G, LANE), BF16)

        def qkv(g):
            res = []
            for t in range(3):
                n = t * H + 2 * g
                mem_rows = []
                for i in range(2):
                    r = _dot(h, wqkv[n + i])
                    ring[n + i, pl.ds(q_wr, XR), :] = r[M:]
                    mem_rows.append(r[:M])
                res.append(jnp.concatenate(
                    mem_rows + [ring[n + i, pl.ds(q_rd, SEG), :] for i in range(2)],
                    axis=0).astype(BF16))
            return res

        def scores(q, k):
            sc_ = lax.dot_general(q, jnp.concatenate([k, pad], axis=0), (((1,), (1,)), ((), ())),
                                  preferred_element_type=F32)
            fill = fill_ref[...]
            sc_ = jnp.where(fill == 0.0, sc_ * scale, fill)
            e = jnp.exp(sc_ - jnp.max(sc_, axis=-1, keepdims=True))
            return e.astype(BF16), 1.0 / jnp.sum(e, axis=-1, keepdims=True)

        def attend(g, e, inv, v):
            o = _dot(e, jnp.concatenate([v, pad], axis=0)) * inv
            res = []
            for i in range(2):
                oring[2 * g + i, pl.ds(o_wr, SEG), :] = o[2 * M + i * SEG:2 * M + (i + 1) * SEG]
                res.append(jnp.concatenate(
                    [o[i * M:(i + 1) * M], oring[2 * g + i, pl.ds(o_rd, XR), :]],
                    axis=0).astype(BF16))
            return res

        acc = [None] * ND
        heads = {}

        def oproj(g0, g1):
            a = jnp.concatenate([r for g in range(g0, g1) for r in heads[g]], axis=1)
            for j in range(ND):
                r = _dot(a, buf_b[pl.ds(j * HD + g0 * 2 * LANE, (g1 - g0) * 2 * LANE), :])
                acc[j] = r if acc[j] is None else acc[j] + r

        proj, prob = {}, {}
        NQ = 4
        for i in range(HP + NQ):
            if i < HP:
                proj[i] = qkv(i)
            else:
                oproj((i - HP) * HP // NQ, (i - HP + 1) * HP // NQ)
            if 0 <= i - 1 < HP:
                prob[i - 1] = scores(proj[i - 1][0], proj[i - 1][1])
            if 0 <= i - 2 < HP:
                heads[i - 2] = attend(i - 2, *prob[i - 2], proj[i - 2][2])

        a = jnp.concatenate(acc, axis=1)
        lhs[0:M, :] = a[:M]
        rows = pl.ds(pl.multiple_of(s * XR, 8), XR)
        xf[rows, :] = xf[rows, :] + modv(2) * a[M:]
        return carry

    lax.fori_loop(0, NSEG, step, 0)

    OB = 256

    def otail(i, carry):
        r0 = pl.multiple_of(i * OB, OB)
        a = jnp.concatenate([oring[n, pl.ds(r0, OB), :].astype(BF16) for n in range(H)], axis=1)
        rows = pl.ds(pl.multiple_of(NSEG * XR + r0, OB), OB)
        for j in range(ND):
            cols = pl.ds(j * LANE, LANE)
            xf[rows, cols] = xf[rows, cols] + mod[2, 0:1, cols] * _dot(a, buf_b[pl.ds(j * HD, HD), :])
        return carry

    lax.fori_loop(0, P // OB, otail, 0)

    wait(cp_ffn)
    FB = act.shape[1]
    FC = 4

    def out_copy(i):
        r0 = pl.multiple_of(i * FB, FB)
        return pltpu.make_async_copy(xb.at[pl.ds(r0, FB)], out_hbm.at[pl.ds(r0, FB)], osems.at[i])

    def ffn(i, carry):
        r0 = pl.multiple_of(i * FB, FB)
        rows = pl.ds(r0, FB)
        hb[pl.ds(0, FB), :] = _ada_ln(xf[rows, :], modv(3), modv(4)).astype(BF16)

        def up(k, c):
            for u in range(FC):
                f = k * FC + u
                hv = hb[pl.ds(0, FB), :]
                act[f] = (_silu(_dot(hv, w13[2 * f])) * _dot(hv, w13[2 * f + 1])).astype(BF16)
            return c

        lax.fori_loop(0, NF // FC, up, 0)
        a = jnp.concatenate([act[f] for f in range(NF)], axis=1)
        for j in range(ND):
            cols = pl.ds(j * LANE, LANE)
            y = _dot(a, buf_a[pl.ds(j * F, F), :])
            xb[rows, cols] = (xf[rows, cols] + mod[5, 0:1, cols] * y).astype(BF16)
        out_copy(i).start()
        return carry

    lax.fori_loop(0, S // FB, ffn, 0)
    for i in range(S // FB):
        out_copy(i).wait()


@functools.partial(jax.jit, static_argnames=("A_seg_len",))
def pallas_adaLN_cond__memory_aug_recurrent_mem_tr__glu_gated_swiglu__prompt_kernel(
    A_x, A_mem0, A_Wq, A_Wk, A_Wv, A_Wo, A_seg_len, B_x, B_w1, B_w3, B_w2, c, w_mod,
):
    del B_x
    B, S, D = A_x.shape
    _, H, Dh = A_Wq.shape
    M = A_mem0.shape[1]
    F = B_w1.shape[1]
    SEG = int(A_seg_len)
    assert (B, S, D, H, Dh, M, SEG) == (1, 2048, 1024, 32, LANE, 8, 32) and F % 512 == 0
    P = S // SEG * M
    R = 576
    FB = 512

    hbm = pl.BlockSpec(memory_space=pl.ANY)
    vmem = pl.BlockSpec(memory_space=pltpu.VMEM)
    out = pl.pallas_call(
        functools.partial(_kernel, S=S, D=D, H=H, F=F, M=M, SEG=SEG),
        out_shape=jax.ShapeDtypeStruct((S, D), A_x.dtype),
        in_specs=[hbm, vmem, hbm, hbm, hbm, hbm, hbm, hbm, hbm, vmem, hbm],
        out_specs=hbm,
        scratch_shapes=[
            pltpu.VMEM((3 * H, D, LANE), BF16),
            pltpu.VMEM((D * H, LANE), BF16),
            pltpu.VMEM((D * H, LANE), BF16),
            pltpu.VMEM((2 * F // LANE, D, LANE), BF16),
            pltpu.VMEM((3 * H, R, LANE), F32),
            pltpu.VMEM((H, R, LANE), F32),
            pltpu.VMEM((S, D), BF16),
            pltpu.VMEM((S, D), F32),
            pltpu.VMEM((6, 8, D), F32),
            pltpu.VMEM((max(P, FB), D), BF16),
            pltpu.VMEM((SEG, D), F32),
            pltpu.VMEM((F // LANE, FB, LANE), BF16),
            pltpu.VMEM((2 * (M + SEG), LANE), F32),
            pltpu.SemaphoreType.DMA((9,)),
            pltpu.SemaphoreType.DMA((S // FB,)),
        ],
        compiler_params=pltpu.CompilerParams(vmem_limit_bytes=126 * 2**20),
        name="adaln_rmt_swiglu",
    )(A_x.reshape(S, D), A_mem0.reshape(M, D), A_Wq.reshape(D * H, Dh), A_Wk.reshape(D * H, Dh),
      A_Wv.reshape(D * H, Dh), A_Wo.reshape(H * Dh, D), B_w1, B_w3, B_w2, c, w_mod)
    return out.reshape(B, S, D)
```

```python
import functools

import jax
import jax.numpy as jnp
from jax import lax
import jax.experimental.pallas as pl
import jax.experimental.pallas.tpu as pltpu

F32 = jnp.float32
BF16 = jnp.bfloat16
U32 = jnp.uint32
LANE = 128
EPS = 1e-5
VLAG = 2


def _dot(a, b):
    return jnp.dot(a, b, preferred_element_type=F32)


def _ada_ln(x, shift, scale1):
    m = jnp.mean(x, axis=-1, keepdims=True)
    d = x - m
    v = jnp.mean(d * d, axis=-1, keepdims=True)
    return d * lax.rsqrt(v + EPS) * scale1 + shift


def _silu(x):
    return x * (1.0 / (1.0 + jnp.exp(-x)))


def _kernel(x_hbm, mem0_ref, wq_hbm, wk_hbm, wv_hbm, wo_hbm, w1_hbm, w3_hbm, w2_hbm,
            c_ref, wmod_hbm, out_hbm,
            wqkv, buf_a32, buf_b32, w13_32, ring, oring, xb, xf, mod, hb, lhs, act, fill_ref, prob, acc, sems, osems,
            *, S, D, H, F, M, SEG):
    NSEG = S // SEG
    XR = SEG - M
    P = S - NSEG * XR
    R = ring.shape[1]
    QOFF = R - P
    OOFF = (-NSEG * XR) % R
    ND = D // LANE
    NF = F // LANE
    HP = H // 2
    HD = H * LANE
    scale = float(LANE) ** -0.5
    buf_a, buf_b, w13 = (r.bitcast(BF16) for r in (buf_a32, buf_b32, w13_32))

    def slab(ref, row0, rows):
        return pltpu.bitcast(ref[pl.ds(row0 // 2, rows // 2), :], BF16)

    def slab_copies(src, n0, n, dst_fn, sem):
        return [pltpu.make_async_copy(src.at[:, pl.ds((n0 + j) * LANE, LANE)], dst_fn(j), sem)
                for j in range(n)]

    cp_x0 = pltpu.make_async_copy(x_hbm.at[pl.ds(0, P)], xb.at[pl.ds(0, P)], sems.at[0])
    cp_x1 = pltpu.make_async_copy(x_hbm.at[pl.ds(P, S - P)], xb.at[pl.ds(P, S - P)], sems.at[1])
    cp_mod0 = slab_copies(wmod_hbm, 0, 2 * ND, lambda j: w13.at[j], sems.at[2])
    cp_mod1 = slab_copies(wmod_hbm, 2 * ND, 4 * ND, lambda j: w13.at[2 * ND + j], sems.at[3])
    cp_q = pltpu.make_async_copy(wq_hbm, buf_a, sems.at[4])
    cp_k = pltpu.make_async_copy(wk_hbm, buf_b, sems.at[5])
    cp_v = pltpu.make_async_copy(wv_hbm, buf_a, sems.at[6])
    cp_o = slab_copies(wo_hbm, 0, ND, lambda j: buf_b.at[pl.ds(j * HD, HD)], sems.at[7])
    cp_ffn = (slab_copies(w1_hbm, 0, NF, lambda j: w13.at[2 * j], sems.at[8])
              + slab_copies(w3_hbm, 0, NF, lambda j: w13.at[2 * j + 1], sems.at[8])
              + slab_copies(w2_hbm, 0, ND, lambda j: buf_a.at[pl.ds(j * F, F)], sems.at[8]))

    def start(cps):
        for cp in cps:
            cp.start()

    def wait(cps):
        for cp in cps:
            cp.wait()

    start(cp_mod0)
    cp_x0.start()
    cp_q.start()

    cc = jnp.broadcast_to(c_ref[...].astype(F32), (16, D))
    sc = _silu(cc).astype(BF16)

    def mod_part(j0, j1):
        for j in range(j0, j1):
            r = _dot(sc, pltpu.bitcast(w13_32[j], BF16))[0:8]
            if j // ND in (1, 4):
                r = r + 1.0
            mod[j // ND, :, pl.ds((j % ND) * LANE, LANE)] = r

    def modv(i):
        return mod[i, 0:1, :]

    G = 2 * (M + SEG)
    ri = lax.broadcasted_iota(jnp.int32, (G, LANE), 0)
    ci = lax.broadcasted_iota(jnp.int32, (G, LANE), 1)

    def head_pos(i):
        head = jnp.where(i < 2 * M, i // M, (i - 2 * M) // SEG)
        pos = jnp.where(i < 2 * M, i % M, M + (i - 2 * M) % SEG)
        return head, pos

    rh, rp = head_pos(ri)
    ch, cp_ = head_pos(ci)
    visible = (rp < M) | (rp >= cp_)
    fill_ref[...] = jnp.where(rh == ch, jnp.where(visible, 0.0, -1e9), -jnp.inf).astype(F32)

    wait(cp_mod0)
    cp_k.start()
    cp_x1.start()
    mod_part(0, 2 * ND)
    cp_x0.wait()

    LB = 128
    PG = 8

    def ln0_body(i, carry):
        r0 = pl.multiple_of(i * LB, LB)
        xv = xb[pl.ds(r0, LB), :].astype(F32)
        xf[pl.ds(r0, LB), :] = xv
        hb[pl.ds(r0, LB), :] = _ada_ln(xv, modv(0), modv(1)).astype(BF16)
        return carry

    lax.fori_loop(0, P // LB, ln0_body, 0)

    def project(t, words):

        def body(a, carry):
            view = words.at[pl.ds(pl.multiple_of(PG * a, PG), D * HP - (HP - PG))]
            for b in range(PG):
                even = view[pl.ds(b, D // 2, stride=2 * HP), :]
                odd = view[pl.ds(b + HP, D // 2, stride=2 * HP), :]
                lo = (even & jnp.uint32(0xFFFF)) | (odd << 16)
                hi = (even >> 16) | (odd & jnp.uint32(0xFFFF0000))
                for i, w in enumerate((lo, hi)):
                    n = t * H + 2 * (PG * a + b) + i
                    wqkv[n] = w
                    ring[n, pl.ds(QOFF, P), :] = _dot(hb[pl.ds(0, P), :], pltpu.bitcast(w, BF16))
            return carry

        lax.fori_loop(0, HP // PG, body, 0)

    cp_q.wait()
    start(cp_mod1)
    project(0, buf_a32)
    cp_v.start()
    cp_k.wait()
    project(1, buf_b32)
    start(cp_o)
    cp_x1.wait()

    def cvt_body(i, carry):
        r0 = pl.multiple_of(P + i * LB, LB)
        xf[pl.ds(r0, LB), :] = xb[pl.ds(r0, LB), :].astype(F32)
        return carry

    lax.fori_loop(0, (S - P) // LB, cvt_body, 0)
    wait(cp_mod1)
    mod_part(2 * ND, 6 * ND)
    cp_v.wait()
    project(2, buf_a32)
    start(cp_ffn)
    lhs[0:M, :] = mem0_ref[...].astype(F32)
    lhs[M:SEG, :] = _ada_ln(xf[pl.ds(P, XR), :], modv(0), modv(1))
    wait(cp_o)

    def step(s, carry):
        q_wr = pl.multiple_of(lax.rem(s * XR, R), 8)
        q_rd = pl.multiple_of(lax.rem(s * SEG + QOFF, R), 8)
        o_wr = pl.multiple_of(lax.rem(s * SEG + OOFF, R), 8)
        o_rd = pl.multiple_of(lax.rem(s * XR + OOFF, R), 8)
        h = lhs[...].astype(BF16)
        nxt = pl.multiple_of(jnp.minimum(P + (s + 1) * XR, S - XR), 8)
        lhs[M:SEG, :] = _ada_ln(xf[pl.ds(nxt, XR), :], modv(0), modv(1))
        pad = jnp.zeros((LANE - G, LANE), BF16)

        def head_pair(t, g):
            n = t * H + 2 * g
            mem_rows = []
            for i in range(2):
                r = _dot(h, pltpu.bitcast(wqkv[n + i], BF16))
                ring[n + i, pl.ds(q_wr, XR), :] = r[M:]
                mem_rows.append(r[:M])
            return jnp.concatenate(
                mem_rows + [ring[n + i, pl.ds(q_rd, SEG), :] for i in range(2)],
                axis=0).astype(BF16)

        def scores(q, k):
            sc_ = lax.dot_general(q, jnp.concatenate([k, pad], axis=0), (((1,), (1,)), ((), ())),
                                  preferred_element_type=F32)
            fill = fill_ref[...]
            sc_ = jnp.where(fill == 0.0, sc_ * scale, fill)
            e = jnp.exp(sc_ - jnp.max(sc_, axis=-1, keepdims=True))
            return (e * (1.0 / jnp.sum(e, axis=-1, keepdims=True))).astype(BF16)

        def attend(g, p, v):
            o = _dot(p, jnp.concatenate([v, pad], axis=0))
            res = []
            for i in range(2):
                oring[2 * g + i, pl.ds(o_wr, SEG), :] = o[2 * M + i * SEG:2 * M + (i + 1) * SEG]
                res.append(jnp.concatenate(
                    [o[i * M:(i + 1) * M], oring[2 * g + i, pl.ds(o_rd, XR), :]],
                    axis=0).astype(BF16))
            return res

        heads = {}

        def oproj(g0, g1, j0=0, j1=ND):
            a = jnp.concatenate([r for g in range(g0, g1) for r in heads[g]], axis=1)
            for j in range(j0, j1):
                cols = pl.ds(j * LANE, LANE)
                r = _dot(a, slab(buf_b32, j * HD + g0 * 2 * LANE, (g1 - g0) * 2 * LANE))
                if g0 > 0:
                    r = r + acc[:, cols]
                if g1 < HP:
                    acc[:, cols] = r
                else:
                    lhs[0:M, cols] = r[:M]
                    xf[rows, cols] = xf[rows, cols] + mod[2, 0:1, cols] * r[M:]

        rows = pl.ds(pl.multiple_of(s * XR, 8), XR)
        qk, val = {}, {}
        LAG = VLAG
        for i in range(2 * HP + LAG):
            if i < HP:
                qk[i] = head_pair(0, i), head_pair(1, i)
            elif i < 2 * HP:
                val[i - HP] = head_pair(2, i - HP)
            else:
                oproj(0, HP // 2, i - 2 * HP, i - 2 * HP + 1)
            if 0 <= i - 1 < HP:
                prob[i - 1] = pltpu.bitcast(scores(*qk[i - 1]), U32)
            g = i - HP - LAG
            if g >= 0:
                heads[g] = attend(g, pltpu.bitcast(prob[g], BF16), val[g])
        oproj(0, HP // 2, LAG, ND)
        oproj(HP // 2, HP)
        return carry

    lax.fori_loop(0, NSEG, step, 0)

    OB = 256

    def otail(i, carry):
        r0 = pl.multiple_of(i * OB, OB)
        a = jnp.concatenate([oring[n, pl.ds(r0, OB), :].astype(BF16) for n in range(H)], axis=1)
        rows = pl.ds(pl.multiple_of(NSEG * XR + r0, OB), OB)
        for j in range(ND):
            cols = pl.ds(j * LANE, LANE)
            xf[rows, cols] = xf[rows, cols] + mod[2, 0:1, cols] * _dot(a, slab(buf_b32, j * HD, HD))
        return carry

    lax.fori_loop(0, P // OB, otail, 0)

    wait(cp_ffn)
    FB = act.shape[1]
    FC = 4

    def out_copy(i):
        r0 = pl.multiple_of(i * FB, FB)
        return pltpu.make_async_copy(xb.at[pl.ds(r0, FB)], out_hbm.at[pl.ds(r0, FB)], osems.at[i])

    def ffn(i, carry):
        r0 = pl.multiple_of(i * FB, FB)
        rows = pl.ds(r0, FB)
        hb[pl.ds(0, FB), :] = _ada_ln(xf[rows, :], modv(3), modv(4)).astype(BF16)

        def up(k, c):
            for u in range(FC):
                f = k * FC + u
                hv = hb[pl.ds(0, FB), :]
                act[f] = (_silu(_dot(hv, pltpu.bitcast(w13_32[2 * f], BF16)))
                          * _dot(hv, pltpu.bitcast(w13_32[2 * f + 1], BF16))).astype(BF16)
            return c

        lax.fori_loop(0, NF // FC, up, 0)
        a = jnp.concatenate([act[f] for f in range(NF)], axis=1)
        for j in range(ND):
            cols = pl.ds(j * LANE, LANE)
            y = _dot(a, slab(buf_a32, j * F, F))
            xb[rows, cols] = (xf[rows, cols] + mod[5, 0:1, cols] * y).astype(BF16)
        out_copy(i).start()
        return carry

    lax.fori_loop(0, S // FB, ffn, 0)
    for i in range(S // FB):
        out_copy(i).wait()


@functools.partial(jax.jit, static_argnames=("A_seg_len",))
def pallas_adaLN_cond__memory_aug_recurrent_mem_tr__glu_gated_swiglu__prompt_kernel(
    A_x, A_mem0, A_Wq, A_Wk, A_Wv, A_Wo, A_seg_len, B_x, B_w1, B_w3, B_w2, c, w_mod,
):
    del B_x
    B, S, D = A_x.shape
    _, H, Dh = A_Wq.shape
    M = A_mem0.shape[1]
    F = B_w1.shape[1]
    SEG = int(A_seg_len)
    assert (B, S, D, H, Dh, M, SEG) == (1, 2048, 1024, 32, LANE, 8, 32) and F % 512 == 0
    P = S // SEG * M
    R = 576
    FB = 512

    hbm = pl.BlockSpec(memory_space=pl.ANY)
    vmem = pl.BlockSpec(memory_space=pltpu.VMEM)
    out = pl.pallas_call(
        functools.partial(_kernel, S=S, D=D, H=H, F=F, M=M, SEG=SEG),
        out_shape=jax.ShapeDtypeStruct((S, D), A_x.dtype),
        in_specs=[hbm, vmem, hbm, hbm, hbm, hbm, hbm, hbm, hbm, vmem, hbm],
        out_specs=hbm,
        scratch_shapes=[
            pltpu.VMEM((3 * H, D // 2, LANE), U32),
            pltpu.VMEM((D * H // 2, LANE), U32),
            pltpu.VMEM((D * H // 2, LANE), U32),
            pltpu.VMEM((2 * F // LANE, D // 2, LANE), U32),
            pltpu.VMEM((3 * H, R, LANE), F32),
            pltpu.VMEM((H, R, LANE), F32),
            pltpu.VMEM((S, D), BF16),
            pltpu.VMEM((S, D), F32),
            pltpu.VMEM((6, 8, D), F32),
            pltpu.VMEM((max(P, FB), D), BF16),
            pltpu.VMEM((SEG, D), F32),
            pltpu.VMEM((F // LANE, FB, LANE), BF16),
            pltpu.VMEM((2 * (M + SEG), LANE), F32),
            pltpu.VMEM((H // 2, M + SEG, LANE), U32),
            pltpu.VMEM((SEG, D), F32),
            pltpu.SemaphoreType.DMA((9,)),
            pltpu.SemaphoreType.DMA((S // FB,)),
        ],
        compiler_params=pltpu.CompilerParams(vmem_limit_bytes=126 * 2**20),
        name="adaln_rmt_swiglu",
    )(A_x.reshape(S, D), A_mem0.reshape(M, D), A_Wq.reshape(D * H, Dh), A_Wk.reshape(D * H, Dh),
      A_Wv.reshape(D * H, Dh), A_Wo.reshape(H * Dh, D), B_w1, B_w3, B_w2, c, w_mod)
    return out.reshape(B, S, D)
```

```python
import functools

import jax
import jax.numpy as jnp
from jax import lax
import jax.experimental.pallas as pl
import jax.experimental.pallas.tpu as pltpu

F32 = jnp.float32
BF16 = jnp.bfloat16
U32 = jnp.uint32
LANE = 128
EPS = 1e-5
VLAG = 2
UNROLL_UP = 2


def _dot(a, b):
    return jnp.dot(a, b, preferred_element_type=F32)


def _norm(x):
    m = jnp.mean(x, axis=-1, keepdims=True)
    d = x - m
    v = jnp.mean(d * d, axis=-1, keepdims=True)
    return d * lax.rsqrt(v + EPS)


def _ada_ln(x, shift, scale1):
    return _norm(x) * scale1 + shift


def _silu(x):
    return x * (1.0 / (1.0 + jnp.exp(-x)))


def _words(x):
    return pltpu.bitcast(x.astype(BF16), U32)


def _strassen_lhs(a11, a12, a21, a22):
    return [_words(a) for a in (a11 + a22, a21 + a22, a11, a22, a11 + a12, a21 - a11, a12 - a22)]


def _strassen(lhs_fn, b11, b12, b21, b22):
    f11, f12, f21, f22 = (b.astype(F32) for b in (b11, b12, b21, b22))

    def prod(i, b):
        return _dot(pltpu.bitcast(lhs_fn(i), BF16), b.astype(BF16))

    m2 = prod(1, b11)
    m4 = prod(3, f21 - f11)
    c21 = m2 + m4
    m3 = prod(2, f12 - f22)
    m5 = prod(4, b22)
    c12 = m3 + m5
    m1 = prod(0, f11 + f22)
    c22 = (m1 - m2 + m3) + prod(5, f11 + f12)
    c11 = (m1 + m4 - m5) + prod(6, f21 + f22)
    return c11, c12, c21, c22


def _kernel(x_hbm, mem0_ref, wq_hbm, wk_hbm, wv_hbm, wo_hbm, w1_hbm, w3_hbm, w2_hbm,
            c_ref, wmod_hbm, out_hbm,
            wqkv, big32, w13_32, ring, oring, xb, xf, mod, lhs, hs, fill_ref, prob, acc, sems, osems,
            *, S, D, H, F, M, SEG, FB):
    NSEG = S // SEG
    XR = SEG - M
    P = S - NSEG * XR
    R = ring.shape[1]
    QOFF = R - P
    OOFF = (-NSEG * XR) % R
    ND = D // LANE
    NF = F // LANE
    HP = H // 2
    HD = H * LANE
    scale = float(LANE) ** -0.5
    big, w13 = big32.bitcast(BF16), w13_32.bitcast(BF16)
    DH = D // 2
    CH = DH * H
    WO = 2 * CH

    def slab(row0, rows):
        return pltpu.bitcast(big32[pl.ds(row0 // 2, rows // 2), :], BF16)

    def slab_copies(src, tiles, dst_fn, sem):
        return [pltpu.make_async_copy(src.at[:, pl.ds(j * LANE, LANE)], dst_fn(j), sem) for j in tiles]

    def half_tiles(c):
        return [v * ND + c * ND // 2 + j for v in range(2) for j in range(ND // 2)]

    cp_x0 = pltpu.make_async_copy(x_hbm.at[pl.ds(0, P)], xb.at[pl.ds(0, P)], sems.at[0])
    cp_x1 = pltpu.make_async_copy(x_hbm.at[pl.ds(P, S - P)], xb.at[pl.ds(P, S - P)], sems.at[1])
    mod_tiles = [half_tiles(0), half_tiles(1), list(range(2 * ND, 6 * ND))]
    cp_mod = [slab_copies(wmod_hbm, t, lambda j: w13.at[j], sems.at[2 + i])
              for i, t in enumerate(mod_tiles)]
    cp_w = [pltpu.make_async_copy(w.at[pl.ds(c * CH, CH)], big.at[pl.ds((2 * t + c) % 4 * CH, CH)],
                                  sems.at[5 + 2 * t + c])
            for t, w in enumerate((wq_hbm, wk_hbm, wv_hbm)) for c in range(2)]
    cp_o = slab_copies(wo_hbm, range(ND), lambda j: big.at[pl.ds(WO + j * HD, HD)], sems.at[11])
    cp_ffn = (slab_copies(w1_hbm, range(NF), lambda j: w13.at[2 * j], sems.at[12])
              + slab_copies(w3_hbm, range(NF), lambda j: w13.at[2 * j + 1], sems.at[12])
              + slab_copies(w2_hbm, range(ND), lambda j: big.at[pl.ds(j * F, F)], sems.at[12]))

    def start(cps):
        for cp in cps:
            cp.start()

    def wait(cps):
        for cp in cps:
            cp.wait()

    start(cp_mod[0])
    cp_x0.start()
    cp_w[0].start()

    cc = jnp.broadcast_to(c_ref[...].astype(F32), (16, D))
    sc = _silu(cc).astype(BF16)

    def mod_part(i):
        wait(cp_mod[i])
        for j in mod_tiles[i]:
            r = _dot(sc, pltpu.bitcast(w13_32[j], BF16))[0:8]
            if j // ND in (1, 4):
                r = r + 1.0
            mod[j // ND, :, pl.ds((j % ND) * LANE, LANE)] = r

    def modv(i):
        return mod[i, 0:1, :]

    G = 2 * (M + SEG)
    ri = lax.broadcasted_iota(jnp.int32, (G, LANE), 0)
    ci = lax.broadcasted_iota(jnp.int32, (G, LANE), 1)

    def head_pos(i):
        head = jnp.where(i < 2 * M, i // M, (i - 2 * M) // SEG)
        pos = jnp.where(i < 2 * M, i % M, M + (i - 2 * M) % SEG)
        return head, pos

    rh, rp = head_pos(ri)
    ch, cp_ = head_pos(ci)
    visible = (rp < M) | (rp >= cp_)
    fill_ref[...] = jnp.where(rh == ch, jnp.where(visible, 0.0, -1e9), -jnp.inf).astype(F32)

    LB = 128
    PG = 8
    PH = P // 2
    DQ = D // 4

    def norm_half(c):
        cols = slice(c * DH, (c + 1) * DH)

        def norm0(k, carry):
            top, bot = (_norm(xb[pl.ds(pl.multiple_of(o + k * LB, LB), LB), :].astype(F32))[:, cols]
                        * mod[1, 0:1, cols] + mod[0, 0:1, cols] for o in (0, PH))
            ops = _strassen_lhs(top[:, :DQ], top[:, DQ:], bot[:, :DQ], bot[:, DQ:])
            for i in range(7):
                hs[i, pl.ds(pl.multiple_of(c * (PH // 2) + k * (LB // 2), LB // 2), LB // 2), 0:DQ] = ops[i]
            return carry

        lax.fori_loop(0, PH // LB, norm0, 0)

    events = {
        0: lambda: (start(cp_mod[1]), cp_w[1].start(), cp_w[0].wait(), cp_w[2].start()),
        1: lambda: (mod_part(1), norm_half(1), cp_w[1].wait(), cp_w[3].start(), cp_x1.start(),
                    cp_w[4].start()),
        2: lambda: (cp_w[2].wait(), cp_x1.wait(), cp_w[5].start(), start(cp_mod[2])),
        3: lambda: cp_w[3].wait(),
        4: lambda: (cp_w[4].wait(), start(cp_o)),
        5: lambda: cp_w[5].wait(),
    }
    NA = HP // PG
    CV = (S - P) // (4 * NA)

    def project(it, carry):
        chunk, a = it // NA, it % NA
        half = chunk % 2
        for ev, fn in events.items():
            pl.when(it == ev * NA)(lambda fn=fn: (fn(), None)[1])
        view = big32.at[pl.ds(pl.multiple_of(chunk % 4 * (CH // 2) + PG * a, PG), CH // 2 - (HP - PG))]
        hrows = pl.ds(pl.multiple_of(half * (PH // 2), PH // 2), PH // 2)
        for b in range(PG):
            even = view[pl.ds(b, DH // 2, stride=2 * HP), :]
            odd = view[pl.ds(b + HP, DH // 2, stride=2 * HP), :]
            n = chunk // 2 * H + 2 * (PG * a + b)
            ws = ((even & jnp.uint32(0xFFFF)) | (odd << 16), (even >> 16) | (odd & jnp.uint32(0xFFFF0000)))
            for i in range(2):
                wqkv[n + i, pl.ds(pl.multiple_of(half * (DH // 2), DH // 2), DH // 2), :] = ws[i]
            lo, hi = (pltpu.bitcast(w, BF16) for w in ws)
            res = _strassen(lambda i: hs[i, hrows, 0:DQ], lo[:DQ], hi[:DQ], lo[DQ:], hi[DQ:])
            for i in (2, 1, 3, 0):
                dst = ring.at[n + i % 2, pl.ds(QOFF + i // 2 * PH, PH)]
                dst[...] = res[i] + jnp.where(half == 1, dst[...], 0.0)
        r0 = jnp.where(it < 2 * NA, jnp.minimum(it * CV, P - CV), P + (it - 2 * NA) * CV)
        rows = pl.ds(pl.multiple_of(r0, 64), CV)
        xf[rows, :] = xb[rows, :].astype(F32)
        return carry

    mod_part(0)
    cp_x0.wait()
    norm_half(0)
    lax.fori_loop(0, 6 * NA, project, 0)
    mod_part(2)
    start(cp_ffn)
    lhs[0:M, :] = mem0_ref[...].astype(F32)
    lhs[M:SEG, :] = _ada_ln(xf[pl.ds(P, XR), :], modv(0), modv(1))
    wait(cp_o)

    def step(s, carry):
        q_wr = pl.multiple_of(lax.rem(s * XR, R), 8)
        q_rd = pl.multiple_of(lax.rem(s * SEG + QOFF, R), 8)
        o_wr = pl.multiple_of(lax.rem(s * SEG + OOFF, R), 8)
        o_rd = pl.multiple_of(lax.rem(s * XR + OOFF, R), 8)
        h = lhs[...].astype(BF16)
        nxt = pl.multiple_of(jnp.minimum(P + (s + 1) * XR, S - XR), 8)
        lhs[M:SEG, :] = _ada_ln(xf[pl.ds(nxt, XR), :], modv(0), modv(1))
        pad = jnp.zeros((LANE - G, LANE), BF16)

        def head_pair(t, g):
            n = t * H + 2 * g
            mem_rows = []
            for i in range(2):
                r = _dot(h, pltpu.bitcast(wqkv[n + i], BF16))
                ring[n + i, pl.ds(q_wr, XR), :] = r[M:]
                mem_rows.append(r[:M])
            return jnp.concatenate(
                mem_rows + [ring[n + i, pl.ds(q_rd, SEG), :] for i in range(2)],
                axis=0).astype(BF16)

        def scores(q, k):
            sc_ = lax.dot_general(q, jnp.concatenate([k, pad], axis=0), (((1,), (1,)), ((), ())),
                                  preferred_element_type=F32)
            fill = fill_ref[...]
            sc_ = jnp.where(fill == 0.0, sc_ * scale, fill)
            e = jnp.exp(sc_ - jnp.max(sc_, axis=-1, keepdims=True))
            return (e * (1.0 / jnp.sum(e, axis=-1, keepdims=True))).astype(BF16)

        def attend(g, p, v):
            o = _dot(p, jnp.concatenate([v, pad], axis=0))
            res = []
            for i in range(2):
                oring[2 * g + i, pl.ds(o_wr, SEG), :] = o[2 * M + i * SEG:2 * M + (i + 1) * SEG]
                res.append(jnp.concatenate(
                    [o[i * M:(i + 1) * M], oring[2 * g + i, pl.ds(o_rd, XR), :]],
                    axis=0).astype(BF16))
            return res

        heads = {}

        def oproj(g0, g1, j0=0, j1=ND):
            a = jnp.concatenate([r for g in range(g0, g1) for r in heads[g]], axis=1)
            for j in range(j0, j1):
                cols = pl.ds(j * LANE, LANE)
                r = _dot(a, slab(WO + j * HD + g0 * 2 * LANE, (g1 - g0) * 2 * LANE))
                if g0 > 0:
                    r = r + acc[:, cols]
                if g1 < HP:
                    acc[:, cols] = r
                else:
                    lhs[0:M, cols] = r[:M]
                    xf[rows, cols] = xf[rows, cols] + mod[2, 0:1, cols] * r[M:]

        rows = pl.ds(pl.multiple_of(s * XR, 8), XR)
        qk, val = {}, {}
        LAG = VLAG
        for i in range(2 * HP + LAG):
            if i < HP:
                qk[i] = head_pair(0, i), head_pair(1, i)
            elif i < 2 * HP:
                val[i - HP] = head_pair(2, i - HP)
            else:
                oproj(0, HP // 2, i - 2 * HP, i - 2 * HP + 1)
            if 0 <= i - 1 < HP:
                prob[i - 1] = pltpu.bitcast(scores(*qk[i - 1]), U32)
            g = i - HP - LAG
            if g >= 0:
                heads[g] = attend(g, pltpu.bitcast(prob[g], BF16), val[g])
        oproj(0, HP // 2, LAG, ND)
        oproj(HP // 2, HP)
        return carry

    lax.fori_loop(0, NSEG, step, 0)

    MH = FB // 2
    ring32 = ring.bitcast(U32)

    def ffn_norm(blk, k):
        top, bot = (_ada_ln(xf[pl.ds(pl.multiple_of(blk * FB + o + k * LB, LB), LB), :], modv(3), modv(4))
                    for o in (0, MH))
        ops = _strassen_lhs(top[:, :DH], top[:, DH:], bot[:, :DH], bot[:, DH:])
        for i in range(7):
            hs[i, pl.ds(pl.multiple_of(k * (LB // 2), LB // 2), LB // 2), :] = ops[i]

    def opack(g, carry):
        ops = _strassen_lhs(*(oring[n * HP + g, pl.ds(o, PH), :] for o in (0, PH) for n in range(2)))
        for i in range(7):
            ring32[i * HP // 2 + g // 2, pl.ds(pl.multiple_of(g % 2 * (PH // 2), PH // 2), PH // 2), :] = ops[i]
        return carry

    lax.fori_loop(0, HP, opack, 0, unroll=2)

    def otail(j, carry):
        def wo_rows(jj, n):
            return slab(pl.multiple_of(WO + jj * HD + n * (HD // 2), HD // 2), HD // 2)

        ys = _strassen(
            lambda i: jnp.concatenate([ring32[i * HP // 2 + g // 2, pl.ds(g % 2 * (PH // 2), PH // 2), :]
                                       for g in range(HP)], axis=1),
            wo_rows(2 * j, 0), wo_rows(2 * j + 1, 0), wo_rows(2 * j, 1), wo_rows(2 * j + 1, 1))
        ffn_norm(0, j)
        for n in (2, 1, 3, 0):
            rows = pl.ds(NSEG * XR + n // 2 * PH, PH)
            cols = pl.ds(pl.multiple_of((2 * j + n % 2) * LANE, LANE), LANE)
            xf[rows, cols] = xf[rows, cols] + mod[2, 0:1, cols] * ys[n]
        return carry

    lax.fori_loop(0, ND // 2, otail, 0)

    wait(cp_ffn)

    def act_slot(k, i):
        n = 7 * k + i
        return ring32.at[n // 2, pl.ds(pl.multiple_of((n % 2) * (MH // 2), MH // 2), MH // 2)]

    def out_copy(blk, j):
        idx = (pl.ds(pl.multiple_of(blk * FB, FB), FB), pl.ds(pl.multiple_of(j * 2 * LANE, 2 * LANE), 2 * LANE))
        return pltpu.make_async_copy(xb.at[idx], out_hbm.at[idx], osems.at[blk * (ND // 2) + j])

    def ffn(blk, carry):
        r0 = pl.multiple_of(blk * FB, FB)

        def up(k, c):
            res = []
            for t in range(2):
                b1, b2 = (pltpu.bitcast(w13_32[4 * k + 2 * u + t], BF16) for u in range(2))
                res.append(_strassen(lambda i: hs[i], b1[:DH], b2[:DH], b1[DH:], b2[DH:]))
            ops = _strassen_lhs(*(_silu(g) * u for g, u in zip(*res)))
            for i in range(7):
                act_slot(k, i)[...] = ops[i]
            return c

        lax.fori_loop(0, NF // 2, up, 0, unroll=UNROLL_UP)

        def down(j, c):
            def w2_rows(jj, par):
                base = pl.multiple_of(jj * (F // 2), LANE // 2)
                return jnp.concatenate(
                    [pltpu.bitcast(big32[pl.ds(base + (2 * k + par) * (LANE // 2), LANE // 2), :], BF16)
                     for k in range(NF // 2)], axis=0)

            ys = _strassen(
                lambda i: jnp.concatenate([act_slot(k, i)[...] for k in range(NF // 2)], axis=1),
                w2_rows(2 * j, 0), w2_rows(2 * j + 1, 0), w2_rows(2 * j, 1), w2_rows(2 * j + 1, 1))
            ffn_norm(jnp.minimum(blk + 1, S // FB - 1), j)
            for n in (2, 1, 3, 0):
                rows = pl.ds(pl.multiple_of(r0 + (n // 2) * MH, MH), MH)
                cols = pl.ds(pl.multiple_of((2 * j + n % 2) * LANE, LANE), LANE)
                xb[rows, cols] = (xf[rows, cols] + mod[5, 0:1, cols] * ys[n]).astype(BF16)
            out_copy(blk, j).start()
            return c

        lax.fori_loop(0, ND // 2, down, 0)
        return carry

    lax.fori_loop(0, S // FB, ffn, 0)
    for blk in range(S // FB):
        for j in range(ND // 2):
            out_copy(blk, j).wait()


@functools.partial(jax.jit, static_argnames=("A_seg_len",))
def pallas_adaLN_cond__memory_aug_recurrent_mem_tr__glu_gated_swiglu__prompt_kernel(
    A_x, A_mem0, A_Wq, A_Wk, A_Wv, A_Wo, A_seg_len, B_x, B_w1, B_w3, B_w2, c, w_mod,
):
    del B_x
    B, S, D = A_x.shape
    _, H, Dh = A_Wq.shape
    M = A_mem0.shape[1]
    F = B_w1.shape[1]
    SEG = int(A_seg_len)
    assert (B, S, D, H, Dh, M, SEG) == (1, 2048, 1024, 32, LANE, 8, 32) and F % 512 == 0
    P = S // SEG * M
    R = 576
    FB = 1024

    hbm = pl.BlockSpec(memory_space=pl.ANY)
    vmem = pl.BlockSpec(memory_space=pltpu.VMEM)
    out = pl.pallas_call(
        functools.partial(_kernel, S=S, D=D, H=H, F=F, M=M, SEG=SEG, FB=FB),
        out_shape=jax.ShapeDtypeStruct((S, D), A_x.dtype),
        in_specs=[hbm, vmem, hbm, hbm, hbm, hbm, hbm, hbm, hbm, vmem, hbm],
        out_specs=hbm,
        scratch_shapes=[
            pltpu.VMEM((3 * H, D // 2, LANE), U32),
            pltpu.VMEM((D * H, LANE), U32),
            pltpu.VMEM((2 * F // LANE, D // 2, LANE), U32),
            pltpu.VMEM((3 * H, R, LANE), F32),
            pltpu.VMEM((H, R, LANE), F32),
            pltpu.VMEM((S, D), BF16),
            pltpu.VMEM((S, D), F32),
            pltpu.VMEM((6, 8, D), F32),
            pltpu.VMEM((SEG, D), F32),
            pltpu.VMEM((7, FB // 4, D // 2), U32),
            pltpu.VMEM((2 * (M + SEG), LANE), F32),
            pltpu.VMEM((H // 2, M + SEG, LANE), U32),
            pltpu.VMEM((SEG, D), F32),
            pltpu.SemaphoreType.DMA((13,)),
            pltpu.SemaphoreType.DMA((S // FB * D // (2 * LANE),)),
        ],
        compiler_params=pltpu.CompilerParams(vmem_limit_bytes=126 * 2**20),
        name="adaln_rmt_swiglu",
    )(A_x.reshape(S, D), A_mem0.reshape(M, D), A_Wq.reshape(D * H, Dh), A_Wk.reshape(D * H, Dh),
      A_Wv.reshape(D * H, Dh), A_Wo.reshape(H * Dh, D), B_w1, B_w3, B_w2, c, w_mod)
    return out.reshape(B, S, D)
```

```python
import functools

import jax
import jax.numpy as jnp
from jax import lax
import jax.experimental.pallas as pl
import jax.experimental.pallas.tpu as pltpu

F32 = jnp.float32
BF16 = jnp.bfloat16
U32 = jnp.uint32
LANE = 128
EPS = 1e-5
VLAG = 2
UNROLL_UP = 2


def _dot(a, b):
    return jnp.dot(a, b, preferred_element_type=F32)


def _norm(x):
    m = jnp.mean(x, axis=-1, keepdims=True)
    d = x - m
    v = jnp.mean(d * d, axis=-1, keepdims=True)
    return d * lax.rsqrt(v + EPS)


def _ada_ln(x, shift, scale1):
    return _norm(x) * scale1 + shift


def _silu(x):
    h = 0.5 * x
    return h + h * jnp.tanh(h)


def _words(x):
    return pltpu.bitcast(x.astype(BF16), U32)


def _strassen_lhs(a11, a12, a21, a22):
    return [_words(a) for a in (a11 + a22, a21 + a22, a11, a22, a11 + a12, a21 - a11, a12 - a22)]


def _strassen(lhs_fn, b11, b12, b21, b22, emit):
    f11, f12, f21, f22 = (b.astype(F32) for b in (b11, b12, b21, b22))

    def prod(i, b):
        return _dot(pltpu.bitcast(lhs_fn(i), BF16), b.astype(BF16))

    m2 = prod(1, b11)
    m4 = prod(3, f21 - f11)
    emit(2, m2 + m4)
    m3 = prod(2, f12 - f22)
    m5 = prod(4, b22)
    emit(1, m3 + m5)
    m1 = prod(0, f11 + f22)
    emit(3, (m1 - m2 + m3) + prod(5, f11 + f12))
    emit(0, (m1 + m4 - m5) + prod(6, f21 + f22))


def _kernel(x_hbm, mem0_ref, wq_hbm, wk_hbm, wv_hbm, wo_hbm, w1_hbm, w3_hbm, w2_hbm,
            c_ref, wmod_hbm, out_hbm,
            wqkv, big32, w13_32, ring, oring, xb, xf, mod, lhs, hs, hf, ot, fill_ref, prob, acc, sems, osems,
            *, S, D, H, F, M, SEG, FB):
    NSEG = S // SEG
    XR = SEG - M
    P = S - NSEG * XR
    R = ring.shape[1]
    QOFF = R - P
    OOFF = (-NSEG * XR) % R
    ND = D // LANE
    NF = F // LANE
    HP = H // 2
    HD = H * LANE
    scale = float(LANE) ** -0.5
    big, w13 = big32.bitcast(BF16), w13_32.bitcast(BF16)
    DH = D // 2
    CH = DH * H
    WP = wqkv.shape[0] // (3 * H)
    WO = 2 * CH

    def slab(row0, rows):
        return pltpu.bitcast(big32[pl.ds(row0 // 2, rows // 2), :], BF16)

    def slab_copies(src, tiles, dst_fn, sem):
        return [pltpu.make_async_copy(src.at[:, pl.ds(j * LANE, LANE)], dst_fn(j), sem) for j in tiles]

    def half_tiles(c):
        return [v * ND + c * ND // 2 + j for v in range(2) for j in range(ND // 2)]

    cp_x0 = pltpu.make_async_copy(x_hbm.at[pl.ds(0, P)], xb.at[pl.ds(0, P)], sems.at[0])
    cp_x1 = pltpu.make_async_copy(x_hbm.at[pl.ds(P, S - P)], xb.at[pl.ds(P, S - P)], sems.at[1])
    mod_tiles = [half_tiles(0), half_tiles(1), list(range(2 * ND, 6 * ND))]
    cp_mod = [slab_copies(wmod_hbm, t, lambda j: w13.at[j], sems.at[2 + i])
              for i, t in enumerate(mod_tiles)]
    cp_w = [pltpu.make_async_copy(w.at[pl.ds(c * CH, CH)], big.at[pl.ds((2 * t + c) % 4 * CH, CH)],
                                  sems.at[5 + 2 * t + c])
            for t, w in enumerate((wq_hbm, wk_hbm, wv_hbm)) for c in range(2)]
    cp_o = slab_copies(wo_hbm, range(ND), lambda j: big.at[pl.ds(WO + j * HD, HD)], sems.at[11])
    cp_ffn = (slab_copies(w1_hbm, range(NF), lambda j: w13.at[2 * j], sems.at[12])
              + slab_copies(w3_hbm, range(NF), lambda j: w13.at[2 * j + 1], sems.at[12])
              + slab_copies(w2_hbm, range(ND), lambda j: big.at[pl.ds(j * F, F)], sems.at[12]))

    def start(cps):
        for cp in cps:
            cp.start()

    def wait(cps):
        for cp in cps:
            cp.wait()

    start(cp_mod[0])
    cp_x0.start()
    cp_w[0].start()

    cc = jnp.broadcast_to(c_ref[...].astype(F32), (16, D))
    sc = _silu(cc).astype(BF16)

    def mod_part(i):
        wait(cp_mod[i])
        for j in mod_tiles[i]:
            r = _dot(sc, pltpu.bitcast(w13_32[j], BF16))[0:8]
            if j // ND in (1, 4):
                r = r + 1.0
            mod[j // ND, :, pl.ds((j % ND) * LANE, LANE)] = r

    def modv(i):
        return mod[i, 0:1, :]

    G = 2 * (M + SEG)
    ri = lax.broadcasted_iota(jnp.int32, (G, LANE), 0)
    ci = lax.broadcasted_iota(jnp.int32, (G, LANE), 1)

    def head_pos(i):
        head = jnp.where(i < 2 * M, i // M, (i - 2 * M) // SEG)
        pos = jnp.where(i < 2 * M, i % M, M + (i - 2 * M) % SEG)
        return head, pos

    rh, rp = head_pos(ri)
    ch, cp_ = head_pos(ci)
    visible = (rp < M) | (rp >= cp_)
    fill_ref[...] = jnp.where(rh == ch, jnp.where(visible, 0.0, -1e9), -jnp.inf).astype(F32)

    LB = 128
    PG = 8
    PH = P // 2
    DQ = D // 4

    def norm_half(c):
        cols = slice(c * DH, (c + 1) * DH)

        def norm0(k, carry):
            top, bot = (_norm(xb[pl.ds(pl.multiple_of(o + k * LB, LB), LB), :].astype(F32))[:, cols]
                        * mod[1, 0:1, cols] + mod[0, 0:1, cols] for o in (0, PH))
            ops = _strassen_lhs(top[:, :DQ], top[:, DQ:], bot[:, :DQ], bot[:, DQ:])
            for i in range(7):
                hs[i, pl.ds(pl.multiple_of(c * (PH // 2) + k * (LB // 2), LB // 2), LB // 2), :] = ops[i]
            return carry

        lax.fori_loop(0, PH // LB, norm0, 0)

    NA = HP // PG
    CV = (S - P) // (4 * NA)
    events = {
        NA - 1: lambda: (cp_w[1].wait(), cp_w[3].start(), cp_x1.start()),
        NA: lambda: (mod_part(1), norm_half(1), cp_w[4].start()),
        2 * NA - 1: lambda: cp_w[2].wait(),
        2 * NA: lambda: (cp_x1.wait(), cp_w[5].start(), start(cp_mod[2])),
        3 * NA - 1: lambda: cp_w[3].wait(),
        4 * NA - 1: lambda: (cp_w[4].wait(), start(cp_o)),
        5 * NA - 1: lambda: cp_w[5].wait(),
    }

    def head_rows(it):
        chunk, a = it // NA, it % NA
        base = (chunk // 2 * H + 2 * PG * a) * WP + chunk % 2 * (DH // 2)
        return wqkv.at[pl.ds(pl.multiple_of(base, 8), 2 * PG * WP - DH // 2)]

    def retile(it, r0, r1):
        src = big32.at[pl.ds(pl.multiple_of(it // NA % 4 * (CH // 2) + PG * (it % NA), PG),
                             CH // 2 - (HP - PG))]
        dst = head_rows(it)
        for r in range(r0, r1):
            even, odd = src[pl.ds(2 * r * HP, PG), :], src[pl.ds((2 * r + 1) * HP, PG), :]
            dst[pl.ds(r, PG, stride=2 * WP), :] = (even & jnp.uint32(0xFFFF)) | (odd << 16)
            dst[pl.ds(WP + r, PG, stride=2 * WP), :] = (even >> 16) | (odd & jnp.uint32(0xFFFF0000))

    def project(it, carry):
        for ev, fn in events.items():
            pl.when(it == ev)(lambda fn=fn: (fn(), None)[1])
        half = it // NA % 2
        hrows = pl.ds(pl.multiple_of(half * (PH // 2), PH // 2), PH // 2)
        nxt = jnp.minimum(it + 1, 6 * NA - 1)
        for b in range(PG):
            n = it // (2 * NA) * H + 2 * (PG * (it % NA) + b)
            lo, hi = (pltpu.bitcast(head_rows(it)[pl.ds((2 * b + i) * WP, DH // 2), :], BF16)
                      for i in range(2))

            def emit(i, r, n=n):
                dst = ring.at[n + i % 2, pl.ds(QOFF + i // 2 * PH, PH)]
                dst[...] = r + jnp.where(half == 1, dst[...], 0.0)

            _strassen(lambda i: hs[i, hrows, :], lo[:DQ], hi[:DQ], lo[DQ:], hi[DQ:], emit)
            retile(nxt, b * (DH // 2) // PG, (b + 1) * (DH // 2) // PG)
        r0 = jnp.where(it < 2 * NA, jnp.minimum(it * CV, P - CV), P + (it - 2 * NA) * CV)
        rows = pl.ds(pl.multiple_of(r0, 64), CV)
        xf[rows, :] = xb[rows, :].astype(F32)
        return carry

    mod_part(0)
    start(cp_mod[1])
    cp_w[1].start()
    cp_x0.wait()
    norm_half(0)
    cp_w[0].wait()
    cp_w[2].start()
    retile(0, 0, DH // 2)
    lax.fori_loop(0, 6 * NA, project, 0)
    mod_part(2)
    start(cp_ffn)
    lhs[0:M, :] = mem0_ref[...].astype(F32)
    lhs[M:SEG, :] = _ada_ln(xf[pl.ds(P, XR), :], modv(0), modv(1))
    wait(cp_o)

    HG = SEG // 2
    xf3, xb3 = xf.reshape(NSEG, SEG, D), xb.reshape(NSEG, SEG, D)

    def ffn_norm(grp):
        hn = _ada_ln(xf[pl.ds(pl.multiple_of(grp * SEG, SEG), SEG), :], modv(3), modv(4))
        ops = _strassen_lhs(hn[:HG, :DH], hn[:HG, DH:], hn[HG:, :DH], hn[HG:, DH:])
        for i in range(7):
            hf[i, pl.ds(pl.multiple_of(grp * (HG // 2), HG // 2), HG // 2), :] = ops[i]

    def step(s, carry):
        q_wr = pl.multiple_of(lax.rem(s * XR, R), 8)
        q_rd = pl.multiple_of(lax.rem(s * SEG + QOFF, R), 8)
        o_wr = pl.multiple_of(lax.rem(s * SEG + OOFF, R), 8)
        o_rd = pl.multiple_of(lax.rem(s * XR + OOFF, R), 8)
        h = lhs[...].astype(BF16)
        nxt = pl.multiple_of(jnp.minimum(P + (s + 1) * XR, S - XR), 8)
        lhs[M:SEG, :] = _ada_ln(xf[pl.ds(nxt, XR), :], modv(0), modv(1))
        ffn_norm(jnp.maximum(s * XR // SEG - 1, 0))
        tail_rows = pl.ds(pl.multiple_of(jnp.maximum(s - NSEG * XR // SEG, 0) * (HG // 2), HG // 2), HG // 2)
        pad = jnp.zeros((LANE - G, LANE), BF16)

        def head_pair(t, g):
            n = t * H + 2 * g
            mem_rows = []
            for i in range(2):
                r = _dot(h, pltpu.bitcast(wqkv[pl.ds((n + i) * WP, DH), :], BF16))
                ring[n + i, pl.ds(q_wr, XR), :] = r[M:]
                mem_rows.append(r[:M])
            return jnp.concatenate(
                mem_rows + [ring[n + i, pl.ds(q_rd, SEG), :] for i in range(2)],
                axis=0).astype(BF16)

        def scores(q, k):
            sc_ = lax.dot_general(q, jnp.concatenate([k, pad], axis=0), (((1,), (1,)), ((), ())),
                                  preferred_element_type=F32)
            fill = fill_ref[...]
            sc_ = jnp.where(fill == 0.0, sc_ * scale, fill)
            e = jnp.exp(sc_ - jnp.max(sc_, axis=-1, keepdims=True))
            return (e * (1.0 / jnp.sum(e, axis=-1, keepdims=True))).astype(BF16)

        def attend(g, p, v):
            o = _dot(p, jnp.concatenate([v, pad], axis=0))
            ops = _strassen_lhs(*(o[2 * M + i * SEG + r:2 * M + i * SEG + r + HG]
                                  for r in (0, HG) for i in range(2)))
            for i in range(7):
                ot[i, tail_rows, pl.ds(g * LANE, LANE)] = ops[i]
            res = []
            for i in range(2):
                oring[2 * g + i, pl.ds(o_wr, SEG), :] = o[2 * M + i * SEG:2 * M + (i + 1) * SEG]
                res.append(jnp.concatenate(
                    [o[i * M:(i + 1) * M], oring[2 * g + i, pl.ds(o_rd, XR), :]],
                    axis=0).astype(BF16))
            return res

        heads = {}

        def oproj(g0, g1, j0=0, j1=ND):
            a = jnp.concatenate([r for g in range(g0, g1) for r in heads[g]], axis=1)
            for j in range(j0, j1):
                cols = pl.ds(j * LANE, LANE)
                r = _dot(a, slab(WO + j * HD + g0 * 2 * LANE, (g1 - g0) * 2 * LANE))
                if g0 > 0:
                    r = r + acc[:, cols]
                if g1 < HP:
                    acc[:, cols] = r
                else:
                    lhs[0:M, cols] = r[:M]
                    xf[rows, cols] = xf[rows, cols] + mod[2, 0:1, cols] * r[M:]

        rows = pl.ds(pl.multiple_of(s * XR, 8), XR)
        qk, val = {}, {}
        LAG = VLAG
        for i in range(2 * HP + LAG):
            if i < HP:
                qk[i] = head_pair(0, i), head_pair(1, i)
            elif i < 2 * HP:
                val[i - HP] = head_pair(2, i - HP)
            else:
                oproj(0, HP // 2, i - 2 * HP, i - 2 * HP + 1)
            if 0 <= i - 1 < HP:
                prob[i - 1] = pltpu.bitcast(scores(*qk[i - 1]), U32)
            g = i - HP - LAG
            if g >= 0:
                heads[g] = attend(g, pltpu.bitcast(prob[g], BF16), val[g])
        oproj(0, HP // 2, LAG, ND)
        oproj(HP // 2, HP)
        return carry

    lax.fori_loop(0, NSEG, step, 0)

    MH = FB // 2
    ring32 = ring.bitcast(U32)


    def row_tiles(row0, n, par):
        base = pl.multiple_of(row0 // 2, LANE // 2)
        return jnp.concatenate(
            [pltpu.bitcast(big32[pl.ds(base + (2 * k + par) * (LANE // 2), LANE // 2), :], BF16)
             for k in range(n // 2)], axis=0)

    def otail(j, carry):
        def emit(n, y):
            cols = pl.ds(pl.multiple_of((2 * j + n % 2) * LANE, LANE), LANE)
            idx = (pl.ds(NSEG * XR // SEG, P // SEG), pl.ds(n // 2 * HG, HG), cols)
            xf3[idx] = xf3[idx] + (mod[2, 0:1, cols] * y).reshape(P // SEG, HG, LANE)

        _strassen(lambda i: ot[i],
                  *(row_tiles(WO + (2 * j + u) * HD, H, par) for par in range(2) for u in range(2)), emit)
        return carry

    lax.fori_loop(0, ND // 2, otail, 0)
    G0 = (NSEG - 1) * XR // SEG - 1

    def norm_tail(i, carry):
        for u in range(6):
            ffn_norm(G0 + 6 * i + u)
        return carry

    lax.fori_loop(0, (NSEG - G0) // 6, norm_tail, 0)

    wait(cp_ffn)

    def act_slot(k, i):
        n = 7 * k + i
        return ring32.at[n // 2, pl.ds(pl.multiple_of((n % 2) * (MH // 2), MH // 2), MH // 2)]

    def out_copy(blk, j):
        idx = (pl.ds(pl.multiple_of(blk * FB, FB), FB), pl.ds(pl.multiple_of(j * 2 * LANE, 2 * LANE), 2 * LANE))
        return pltpu.make_async_copy(xb.at[idx], out_hbm.at[idx], osems.at[blk * (ND // 2) + j])

    def ffn(blk, carry):
        def up(k, c):
            res = {}, {}
            for t in range(2):
                b1, b2 = (pltpu.bitcast(w13_32[4 * k + 2 * u + t], BF16) for u in range(2))
                _strassen(lambda i: hf[i, pl.ds(pl.multiple_of(blk * (MH // 2), MH // 2), MH // 2), :],
                          b1[:DH], b2[:DH], b1[DH:], b2[DH:], res[t].__setitem__)
            ops = _strassen_lhs(*(_silu(res[0][n]) * res[1][n] for n in range(4)))
            for i in (1, 3, 6, 0, 2, 4, 5):
                act_slot(k, i)[...] = ops[i]
            return c

        lax.fori_loop(0, NF // 2, up, 0, unroll=UNROLL_UP)

        def down(j, c):
            def emit(n, y):
                cols = pl.ds(pl.multiple_of((2 * j + n % 2) * LANE, LANE), LANE)
                idx = (pl.ds(blk * (FB // SEG), FB // SEG), pl.ds(n // 2 * HG, HG), cols)
                xb3[idx] = (xf3[idx] + (mod[5, 0:1, cols] * y).reshape(FB // SEG, HG, LANE)).astype(BF16)

            _strassen(lambda i: jnp.concatenate([act_slot(k, i)[...] for k in range(NF // 2)], axis=1),
                      *(row_tiles((2 * j + u) * F, NF, par) for par in range(2) for u in range(2)), emit)
            out_copy(blk, j).start()
            return c

        lax.fori_loop(0, ND // 2, down, 0)
        return carry

    lax.fori_loop(0, S // FB, ffn, 0)
    for blk in range(S // FB):
        for j in range(ND // 2):
            out_copy(blk, j).wait()


@functools.partial(jax.jit, static_argnames=("A_seg_len",))
def pallas_adaLN_cond__memory_aug_recurrent_mem_tr__glu_gated_swiglu__prompt_kernel(
    A_x, A_mem0, A_Wq, A_Wk, A_Wv, A_Wo, A_seg_len, B_x, B_w1, B_w3, B_w2, c, w_mod,
):
    del B_x
    B, S, D = A_x.shape
    _, H, Dh = A_Wq.shape
    M = A_mem0.shape[1]
    F = B_w1.shape[1]
    SEG = int(A_seg_len)
    assert (B, S, D, H, Dh, M, SEG) == (1, 2048, 1024, 32, LANE, 8, 32) and F % 512 == 0
    P = S // SEG * M
    R = 576
    FB = 1024

    hbm = pl.BlockSpec(memory_space=pl.ANY)
    vmem = pl.BlockSpec(memory_space=pltpu.VMEM)
    out = pl.pallas_call(
        functools.partial(_kernel, S=S, D=D, H=H, F=F, M=M, SEG=SEG, FB=FB),
        out_shape=jax.ShapeDtypeStruct((S, D), A_x.dtype),
        in_specs=[hbm, vmem, hbm, hbm, hbm, hbm, hbm, hbm, hbm, vmem, hbm],
        out_specs=hbm,
        scratch_shapes=[
            pltpu.VMEM((3 * H * (D // 2 + 2), LANE), U32),
            pltpu.VMEM((D * H, LANE), U32),
            pltpu.VMEM((2 * F // LANE, D // 2, LANE), U32),
            pltpu.VMEM((3 * H, R, LANE), F32),
            pltpu.VMEM((H, R, LANE), F32),
            pltpu.VMEM((S, D), BF16),
            pltpu.VMEM((S, D), F32),
            pltpu.VMEM((6, 8, D), F32),
            pltpu.VMEM((SEG, D), F32),
            pltpu.VMEM((7, P // 2, D // 4), U32),
            pltpu.VMEM((7, S // 4, D // 2), U32),
            pltpu.VMEM((7, P // 4, H * Dh // 2), U32),
            pltpu.VMEM((2 * (M + SEG), LANE), F32),
            pltpu.VMEM((H // 2, M + SEG, LANE), U32),
            pltpu.VMEM((SEG, D), F32),
            pltpu.SemaphoreType.DMA((13,)),
            pltpu.SemaphoreType.DMA((S // FB * D // (2 * LANE),)),
        ],
        compiler_params=pltpu.CompilerParams(vmem_limit_bytes=126 * 2**20),
        name="adaln_rmt_swiglu",
    )(A_x.reshape(S, D), A_mem0.reshape(M, D), A_Wq.reshape(D * H, Dh), A_Wk.reshape(D * H, Dh),
      A_Wv.reshape(D * H, Dh), A_Wo.reshape(H * Dh, D), B_w1, B_w3, B_w2, c, w_mod)
    return out.reshape(B, S, D)
```

```python
import functools

import jax
import jax.numpy as jnp
from jax import lax
import jax.experimental.pallas as pl
import jax.experimental.pallas.tpu as pltpu

F32 = jnp.float32
BF16 = jnp.bfloat16
U32 = jnp.uint32
LANE = 128
EPS = 1e-5
VLAG = 3
AG = 1
OLAG = 0
AGS = 8
PIN1 = 2
PIN2 = 6
UNROLL_STEP = 2
SPLIT = 2
UNROLL_UP = 2


def _dot(a, b):
    return jnp.dot(a, b, preferred_element_type=F32)


def _norm(x):
    m = jnp.mean(x, axis=-1, keepdims=True)
    d = x - m
    v = jnp.mean(d * d, axis=-1, keepdims=True)
    return d * lax.rsqrt(v + EPS)


def _ada_ln(x, shift, scale1):
    return _norm(x) * scale1 + shift


def _silu(x):
    h = 0.5 * x
    return h + h * jnp.tanh(h)


def _words(x):
    return pltpu.bitcast(x.astype(BF16), U32)


def _strassen_lhs(a11, a12, a21, a22):
    return [_words(a) for a in (a11 + a22, a21 + a22, a11, a22, a11 + a12, a21 - a11, a12 - a22)]


def _strassen(lhs_fn, b11, b12, b21, b22, emit):
    f11, f12, f21, f22 = (b.astype(F32) for b in (b11, b12, b21, b22))

    def prod(i, b):
        return _dot(pltpu.bitcast(lhs_fn(i), BF16), b.astype(BF16))

    m2 = prod(1, b11)
    m4 = prod(3, f21 - f11)
    emit(2, m2 + m4)
    m3 = prod(2, f12 - f22)
    m5 = prod(4, b22)
    emit(1, m3 + m5)
    m1 = prod(0, f11 + f22)
    emit(3, (m1 - m2 + m3) + prod(5, f11 + f12))
    emit(0, (m1 + m4 - m5) + prod(6, f21 + f22))


def _kernel(x_hbm, mem0_ref, wq_hbm, wk_hbm, wv_hbm, wo_hbm, w1_hbm, w3_hbm, w2_hbm,
            c_ref, wmod_hbm, out_hbm,
            wqkv, big32, w13_32, ring, oring, xb, xf, mod, hs, ot, fill_ref, prob, acc, early, sems, osems,
            *, S, D, H, F, M, SEG, FB):
    NSEG = S // SEG
    XR = SEG - M
    P = S - NSEG * XR
    R = ring.shape[1]
    QOFF = R - P
    OOFF = (-NSEG * XR) % R
    ND = D // LANE
    NF = F // LANE
    HP = H // 2
    HD = H * LANE
    scale = float(LANE) ** -0.5
    big, w13 = big32.bitcast(BF16), w13_32.bitcast(BF16)
    DH = D // 2
    CH = DH * H
    WP = wqkv.shape[0] // (3 * H)
    WO = 2 * CH

    def slab(row0, rows):
        return pltpu.bitcast(big32[pl.ds(row0 // 2, rows // 2), :], BF16)

    def slab_copies(src, tiles, dst_fn, sem):
        return [pltpu.make_async_copy(src.at[:, pl.ds(j * LANE, LANE)], dst_fn(j), sem) for j in tiles]

    def half_tiles(c):
        return [v * ND + c * ND // 2 + j for v in range(2) for j in range(ND // 2)]

    cp_x0 = pltpu.make_async_copy(x_hbm.at[pl.ds(0, P)], xb.at[pl.ds(0, P)], sems.at[0])
    cp_x1 = pltpu.make_async_copy(x_hbm.at[pl.ds(P, S - P)], xb.at[pl.ds(P, S - P)], sems.at[1])
    mod_tiles = [half_tiles(0), half_tiles(1), list(range(2 * ND, 6 * ND))]
    cp_mod = [slab_copies(wmod_hbm, t, lambda j: w13.at[j], sems.at[2 + i])
              for i, t in enumerate(mod_tiles)]
    cp_w = [pltpu.make_async_copy(w.at[pl.ds(c * CH, CH)], big.at[pl.ds((2 * t + c) % 4 * CH, CH)],
                                  sems.at[5 + 2 * t + c])
            for t, w in enumerate((wq_hbm, wk_hbm, wv_hbm)) for c in range(2)]
    cp_o = slab_copies(wo_hbm, range(ND), lambda j: big.at[pl.ds(WO + j * HD, HD)], sems.at[11])
    cp_ffn = (slab_copies(w1_hbm, range(NF), lambda j: w13.at[2 * j], sems.at[12])
              + slab_copies(w3_hbm, range(NF), lambda j: w13.at[2 * j + 1], sems.at[12])
              + slab_copies(w2_hbm, range(ND), lambda j: big.at[pl.ds(j * F, F)], sems.at[12]))

    def start(cps):
        for cp in cps:
            cp.start()

    def wait(cps):
        for cp in cps:
            cp.wait()

    start(cp_mod[0])
    cp_x0.start()
    cp_w[0].start()

    cc = jnp.broadcast_to(c_ref[...].astype(F32), (16, D))
    sc = _silu(cc).astype(BF16)

    def mod_part(i):
        wait(cp_mod[i])
        for j in mod_tiles[i]:
            r = _dot(sc, pltpu.bitcast(w13_32[j], BF16))[0:8]
            if j // ND in (1, 4):
                r = r + 1.0
            mod[j // ND, :, pl.ds((j % ND) * LANE, LANE)] = r

    def modv(i):
        return mod[i, 0:1, :]

    G = 2 * (M + SEG)
    ri = lax.broadcasted_iota(jnp.int32, (G, LANE), 0)
    ci = lax.broadcasted_iota(jnp.int32, (G, LANE), 1)

    def head_pos(i):
        head = jnp.where(i < 2 * M, i // M, (i - 2 * M) // SEG)
        pos = jnp.where(i < 2 * M, i % M, M + (i - 2 * M) % SEG)
        return head, pos

    rh, rp = head_pos(ri)
    ch, cp_ = head_pos(ci)
    visible = (rp < M) | (rp >= cp_)
    fill_ref[...] = jnp.where(rh == ch, jnp.where(visible, 0.0, -1e9), -jnp.inf).astype(F32)

    LB = 128
    PG = 8
    PH = P // 2
    DQ = D // 4

    def norm_half(c):
        cols = slice(c * DH, (c + 1) * DH)

        def norm0(k, carry):
            top, bot = (_norm(xb[pl.ds(pl.multiple_of(o + k * LB, LB), LB), :].astype(F32))[:, cols]
                        * mod[1, 0:1, cols] + mod[0, 0:1, cols] for o in (0, PH))
            ops = _strassen_lhs(top[:, :DQ], top[:, DQ:], bot[:, :DQ], bot[:, DQ:])
            for i in range(7):
                hs[i, pl.ds(pl.multiple_of(c * (PH // 2) + k * (LB // 2), LB // 2), LB // 2), :] = ops[i]
            return carry

        lax.fori_loop(0, PH // LB, norm0, 0)

    NA = HP // PG
    CV = (S - P) // (4 * NA)
    events = {
        NA - 1: lambda: (cp_w[1].wait(), cp_w[3].start(), cp_x1.start()),
        NA: lambda: (mod_part(1), norm_half(1), cp_w[4].start()),
        2 * NA - 1: lambda: cp_w[2].wait(),
        2 * NA: lambda: (cp_x1.wait(), cp_w[5].start(), start(cp_mod[2])),
        3 * NA - 1: lambda: cp_w[3].wait(),
        4 * NA - 1: lambda: (cp_w[4].wait(), start(cp_o)),
        5 * NA - 1: lambda: cp_w[5].wait(),
    }

    def head_rows(it):
        chunk, a = it // NA, it % NA
        base = (chunk // 2 * H + 2 * PG * a) * WP + chunk % 2 * (DH // 2)
        return wqkv.at[pl.ds(pl.multiple_of(base, 8), 2 * PG * WP - DH // 2)]

    def retile(it, r0, r1):
        src = big32.at[pl.ds(pl.multiple_of(it // NA % 4 * (CH // 2) + PG * (it % NA), PG),
                             CH // 2 - (HP - PG))]
        dst = head_rows(it)
        for r in range(r0, r1):
            even, odd = src[pl.ds(2 * r * HP, PG), :], src[pl.ds((2 * r + 1) * HP, PG), :]
            dst[pl.ds(r, PG, stride=2 * WP), :] = (even & jnp.uint32(0xFFFF)) | (odd << 16)
            dst[pl.ds(WP + r, PG, stride=2 * WP), :] = (even >> 16) | (odd & jnp.uint32(0xFFFF0000))

    def project(it, carry):
        for ev, fn in events.items():
            pl.when(it == ev)(lambda fn=fn: (fn(), None)[1])
        half = it // NA % 2
        hrows = pl.ds(pl.multiple_of(half * (PH // 2), PH // 2), PH // 2)
        nxt = jnp.minimum(it + 1, 6 * NA - 1)
        for b in range(PG):
            n = it // (2 * NA) * H + 2 * (PG * (it % NA) + b)
            lo, hi = (pltpu.bitcast(head_rows(it)[pl.ds((2 * b + i) * WP, DH // 2), :], BF16)
                      for i in range(2))

            def emit(i, r, n=n):
                dst = ring.at[n + i % 2, pl.ds(QOFF + i // 2 * PH, PH)]
                dst[...] = r + jnp.where(half == 1, dst[...], 0.0)

            _strassen(lambda i: hs[i, hrows, :], lo[:DQ], hi[:DQ], lo[DQ:], hi[DQ:], emit)
            retile(nxt, b * (DH // 2) // PG, (b + 1) * (DH // 2) // PG)
        r0 = jnp.where(it < 2 * NA, jnp.minimum(it * CV, P - CV), P + (it - 2 * NA) * CV)
        rows = pl.ds(pl.multiple_of(r0, 64), CV)
        xf[rows, :] = xb[rows, :].astype(F32)
        return carry

    mod_part(0)
    start(cp_mod[1])
    cp_w[1].start()
    cp_x0.wait()
    norm_half(0)
    cp_w[0].wait()
    cp_w[2].start()
    retile(0, 0, DH // 2)
    lax.fori_loop(0, 6 * NA, project, 0)
    mod_part(2)
    start(cp_ffn)

    HG = SEG // 2
    xf3, xb3 = xf.reshape(NSEG, SEG, D), xb.reshape(NSEG, SEG, D)

    def ffn_norm(grp):
        hn = _ada_ln(xf[pl.ds(pl.multiple_of(grp * SEG, SEG), SEG), :], modv(3), modv(4))
        ops = _strassen_lhs(hn[:HG, :DH], hn[:HG, DH:], hn[HG:, :DH], hn[HG:, DH:])
        for i in range(7):
            for t in range(ND // 2):
                ring[3 * H + i * (ND // 2) + t, pl.ds(pl.multiple_of(grp * (HG // 2), HG // 2), HG // 2), :] = (
                    pltpu.bitcast(ops[i][:, t * LANE:(t + 1) * LANE], F32))

    lhs = ring.at[3 * H + 7 * (ND // 2)]

    def next_rows(r0):
        hn = _ada_ln(xf[pl.ds(r0, XR), :], modv(0), modv(1))
        for t in range(ND):
            lhs[pl.ds(t * SEG + M, XR), :] = hn[:, t * LANE:(t + 1) * LANE]

    for t in range(ND):
        lhs[pl.ds(t * SEG, M), :] = mem0_ref[:, pl.ds(t * LANE, LANE)].astype(F32)
    next_rows(P)
    wait(cp_o)

    def step(s, carry):
        q_wr = pl.multiple_of(lax.rem(s * XR, R), 8)
        q_rd = pl.multiple_of(lax.rem(s * SEG + QOFF, R), 8)
        o_wr = pl.multiple_of(lax.rem(s * SEG + OOFF, R), 8)
        o_rd = pl.multiple_of(lax.rem(s * XR + OOFF, R), 8)
        h = jnp.concatenate([lhs[pl.ds(t * SEG, SEG), :] for t in range(ND)], axis=1).astype(BF16)
        tail_rows = pl.ds(pl.multiple_of(jnp.maximum(s - NSEG * XR // SEG, 0) * (HG // 2), HG // 2), HG // 2)
        pad = jnp.zeros((LANE - G, LANE), BF16)

        for u in range(4 * SPLIT):
            n = u // 2 % 2 * H + u // 4 * 2 + u % 2
            early[u] = _dot(h[:, :DH], pltpu.bitcast(wqkv[pl.ds(n * WP, DH // 2), :], BF16))

        def head_pair(t, g):
            n = t * H + 2 * g
            mem_rows = []
            for i in range(2):
                if t < 2 and g < SPLIT:
                    r = (_dot(h[:, DH:], pltpu.bitcast(wqkv[pl.ds((n + i) * WP + DH // 2, DH // 2), :], BF16))
                         + early[4 * g + 2 * t + i])
                else:
                    r = _dot(h, pltpu.bitcast(wqkv[pl.ds((n + i) * WP, DH), :], BF16))
                ring[n + i, pl.ds(q_wr, XR), :] = r[M:]
                mem_rows.append(r[:M])
            return jnp.concatenate(
                mem_rows + [ring[n + i, pl.ds(q_rd, SEG), :] for i in range(2)],
                axis=0).astype(BF16)

        def scores(q, k):
            sc_ = lax.dot_general(q, jnp.concatenate([k, pad], axis=0), (((1,), (1,)), ((), ())),
                                  preferred_element_type=F32)
            fill = fill_ref[...]
            sc_ = jnp.where(fill == 0.0, sc_ * scale, fill)
            e = jnp.exp(sc_ - jnp.max(sc_, axis=-1, keepdims=True))
            return (e * (1.0 / jnp.sum(e, axis=-1, keepdims=True))).astype(BF16)

        def attend(g, p, v):
            o = _dot(p, jnp.concatenate([v, pad], axis=0))
            ops = _strassen_lhs(*(o[2 * M + i * SEG + r:2 * M + i * SEG + r + HG]
                                  for r in (0, HG) for i in range(2)))
            for i in range(7):
                ot[i, tail_rows, pl.ds(g * LANE, LANE)] = ops[i]
            for i in range(2):
                oring[2 * g + i, pl.ds(o_wr, SEG), :] = o[2 * M + i * SEG:2 * M + (i + 1) * SEG]
            return functools.cache(lambda: [jnp.concatenate(
                [o[i * M:(i + 1) * M], oring[2 * g + i, pl.ds(o_rd, XR), :]],
                axis=0).astype(BF16) for i in range(2)])

        heads = {}

        def oproj(g0, g1, j0=0, j1=ND):
            a = jnp.concatenate([r for g in range(g0, g1) for r in heads[g]()], axis=1)
            for j in range(j0, j1):
                cols = pl.ds(j * LANE, LANE)
                r = _dot(a, slab(WO + j * HD + g0 * 2 * LANE, (g1 - g0) * 2 * LANE))
                if g0 > 0:
                    r = r + acc[:, cols]
                if g1 < HP:
                    acc[:, cols] = r
                else:
                    lhs[pl.ds(j * SEG, M), :] = r[:M]
                    xf[rows, cols] = xf[rows, cols] + mod[2, 0:1, cols] * r[M:]

        rows = pl.ds(pl.multiple_of(s * XR, 8), XR)
        qk, val = {}, {}
        LAG = VLAG
        for i in range(2 * HP + LAG):
            if i == PIN1:
                next_rows(pl.multiple_of(jnp.minimum(P + (s + 1) * XR, S - XR), 8))
            if i == PIN2:
                ffn_norm(jnp.maximum(s * XR // SEG - 1, 0))
            if i < HP:
                qk[i] = head_pair(0, i), head_pair(1, i)
            elif i < 2 * HP:
                val[i - HP] = head_pair(2, i - HP)
            else:
                oproj(0, HP // 2, i - 2 * HP, i - 2 * HP + 1)
            if i % AGS == 0 and 0 < i <= HP:
                for g, q, k in [(g, *qk[g]) for g in range(i - AGS, i)]:
                    prob[g] = pltpu.bitcast(scores(q, k), U32)
            g1 = i - HP - LAG + 1
            if g1 % AG == 0 and g1 > 0:
                for g, v in [(g, val[g]) for g in range(g1 - AG, g1)]:
                    heads[g] = attend(g, pltpu.bitcast(prob[g], BF16), v)
                for g in range(max(g1 - AG - OLAG, 0), g1 - OLAG):
                    heads[g]()
        oproj(0, HP // 2, LAG, ND)
        oproj(HP // 2, HP)
        return carry

    lax.fori_loop(0, NSEG, step, 0, unroll=UNROLL_STEP)

    MH = FB // 2

    def row_tiles(row0, n, par):
        base = pl.multiple_of(row0 // 2, LANE // 2)
        return jnp.concatenate(
            [pltpu.bitcast(big32[pl.ds(base + (2 * k + par) * (LANE // 2), LANE // 2), :], BF16)
             for k in range(n // 2)], axis=0)

    def otail(j, carry):
        def emit(n, y):
            cols = pl.ds(pl.multiple_of((2 * j + n % 2) * LANE, LANE), LANE)
            idx = (pl.ds(NSEG * XR // SEG, P // SEG), pl.ds(n // 2 * HG, HG), cols)
            xf3[idx] = xf3[idx] + (mod[2, 0:1, cols] * y).reshape(P // SEG, HG, LANE)

        _strassen(lambda i: ot[i],
                  *(row_tiles(WO + (2 * j + u) * HD, H, par) for par in range(2) for u in range(2)), emit)
        return carry

    lax.fori_loop(0, ND // 2, otail, 0)
    G0 = (NSEG - 1) * XR // SEG - 1

    def norm_tail(i, carry):
        for u in range(6):
            ffn_norm(G0 + 6 * i + u)
        return carry

    lax.fori_loop(0, (NSEG - G0) // 6, norm_tail, 0)

    wait(cp_ffn)

    def act_slot(k, i):
        return wqkv.at[pl.ds(pl.multiple_of((7 * k + i) * (MH // 2), MH // 2), MH // 2)]

    def out_copy(blk, j):
        idx = (pl.ds(pl.multiple_of(blk * FB, FB), FB), pl.ds(pl.multiple_of(j * 2 * LANE, 2 * LANE), 2 * LANE))
        return pltpu.make_async_copy(xb.at[idx], out_hbm.at[idx], osems.at[blk * (ND // 2) + j])

    def ffn(blk, carry):
        def normed(i):
            rows = pl.ds(pl.multiple_of(blk * (MH // 2), MH // 2), MH // 2)
            return jnp.concatenate([ring[3 * H + i * (ND // 2) + t, rows, :] for t in range(ND // 2)], axis=1)

        def up(k, c):
            res = {}, {}
            for t in range(2):
                b1, b2 = (pltpu.bitcast(w13_32[4 * k + 2 * u + t], BF16) for u in range(2))
                _strassen(normed,
                          b1[:DH], b2[:DH], b1[DH:], b2[DH:], res[t].__setitem__)
            ops = _strassen_lhs(*(_silu(res[0][n]) * res[1][n] for n in range(4)))
            for i in (1, 3, 6, 0, 2, 4, 5):
                act_slot(k, i)[...] = ops[i]
            return c

        lax.fori_loop(0, NF // 2, up, 0, unroll=UNROLL_UP)

        def down(j, c):
            def emit(n, y):
                cols = pl.ds(pl.multiple_of((2 * j + n % 2) * LANE, LANE), LANE)
                idx = (pl.ds(blk * (FB // SEG), FB // SEG), pl.ds(n // 2 * HG, HG), cols)
                xb3[idx] = (xf3[idx] + (mod[5, 0:1, cols] * y).reshape(FB // SEG, HG, LANE)).astype(BF16)

            _strassen(lambda i: jnp.concatenate([act_slot(k, i)[...] for k in range(NF // 2)], axis=1),
                      *(row_tiles((2 * j + u) * F, NF, par) for par in range(2) for u in range(2)), emit)
            out_copy(blk, j).start()
            return c

        lax.fori_loop(0, ND // 2, down, 0)
        return carry

    lax.fori_loop(0, S // FB, ffn, 0)
    for blk in range(S // FB):
        for j in range(ND // 2):
            out_copy(blk, j).wait()


@functools.partial(jax.jit, static_argnames=("A_seg_len",))
def pallas_adaLN_cond__memory_aug_recurrent_mem_tr__glu_gated_swiglu__prompt_kernel(
    A_x, A_mem0, A_Wq, A_Wk, A_Wv, A_Wo, A_seg_len, B_x, B_w1, B_w3, B_w2, c, w_mod,
):
    del B_x
    B, S, D = A_x.shape
    _, H, Dh = A_Wq.shape
    M = A_mem0.shape[1]
    F = B_w1.shape[1]
    SEG = int(A_seg_len)
    assert (B, S, D, H, Dh, M, SEG) == (1, 2048, 1024, 32, LANE, 8, 32) and F % 512 == 0
    P = S // SEG * M
    R = 576
    FB = 1024

    hbm = pl.BlockSpec(memory_space=pl.ANY)
    vmem = pl.BlockSpec(memory_space=pltpu.VMEM)
    out = pl.pallas_call(
        functools.partial(_kernel, S=S, D=D, H=H, F=F, M=M, SEG=SEG, FB=FB),
        out_shape=jax.ShapeDtypeStruct((S, D), A_x.dtype),
        in_specs=[hbm, vmem, hbm, hbm, hbm, hbm, hbm, hbm, hbm, vmem, hbm],
        out_specs=hbm,
        scratch_shapes=[
            pltpu.VMEM((3 * H * (D // 2 + 2), LANE), U32),
            pltpu.VMEM((D * H, LANE), U32),
            pltpu.VMEM((2 * F // LANE, D // 2, LANE), U32),
            pltpu.VMEM((3 * H + 7 * D // (2 * LANE) + 1, R, LANE), F32),
            pltpu.VMEM((H, R, LANE), F32),
            pltpu.VMEM((S, D), BF16),
            pltpu.VMEM((S, D), F32),
            pltpu.VMEM((6, 8, D), F32),
            pltpu.VMEM((7, P // 2, D // 4), U32),
            pltpu.VMEM((7, P // 4, H * Dh // 2), U32),
            pltpu.VMEM((2 * (M + SEG), LANE), F32),
            pltpu.VMEM((H // 2, M + SEG, LANE), U32),
            pltpu.VMEM((SEG, D), F32),
            pltpu.VMEM((8, SEG, LANE), F32),
            pltpu.SemaphoreType.DMA((13,)),
            pltpu.SemaphoreType.DMA((S // FB * D // (2 * LANE),)),
        ],
        compiler_params=pltpu.CompilerParams(vmem_limit_bytes=126 * 2**20),
        name="adaln_rmt_swiglu",
    )(A_x.reshape(S, D), A_mem0.reshape(M, D), A_Wq.reshape(D * H, Dh), A_Wk.reshape(D * H, Dh),
      A_Wv.reshape(D * H, Dh), A_Wo.reshape(H * Dh, D), B_w1, B_w3, B_w2, c, w_mod)
    return out.reshape(B, S, D)
```

```python
import functools

import jax
import jax.numpy as jnp
from jax import lax
import jax.experimental.pallas as pl
import jax.experimental.pallas.tpu as pltpu

F32 = jnp.float32
BF16 = jnp.bfloat16
U32 = jnp.uint32
LANE = 128
EPS = 1e-5
VLAG = 3
AG = 1
OLAG = 0
AGS = 8
PIN1 = 2
PIN2 = 6
UNROLL_STEP = 2
SPLIT = 2
UNROLL_UP = 2


def _dot(a, b):
    return jnp.dot(a, b, preferred_element_type=F32)


def _norm(x):
    m = jnp.mean(x, axis=-1, keepdims=True)
    d = x - m
    v = jnp.mean(d * d, axis=-1, keepdims=True)
    return d * lax.rsqrt(v + EPS)


def _ada_ln(x, shift, scale1):
    return _norm(x) * scale1 + shift


def _silu(x):
    h = 0.5 * x
    return h + h * jnp.tanh(h)


def _words(x):
    return pltpu.bitcast(x.astype(BF16), U32)


def _strassen_lhs(a11, a12, a21, a22):
    return [_words(a) for a in (a11 + a22, a21 + a22, a11, a22, a11 + a12, a21 - a11, a12 - a22)]


def _strassen(lhs_fn, b11, b12, b21, b22, emit):
    f11, f12, f21, f22 = (b.astype(F32) for b in (b11, b12, b21, b22))

    def prod(i, b):
        return _dot(pltpu.bitcast(lhs_fn(i), BF16), b.astype(BF16))

    m2 = prod(1, b11)
    m4 = prod(3, f21 - f11)
    emit(2, m2 + m4)
    m3 = prod(2, f12 - f22)
    m5 = prod(4, b22)
    emit(1, m3 + m5)
    m1 = prod(0, f11 + f22)
    emit(3, (m1 - m2 + m3) + prod(5, f11 + f12))
    emit(0, (m1 + m4 - m5) + prod(6, f21 + f22))


def _kernel(x_hbm, mem0_ref, wq_hbm, wk_hbm, wv_hbm, wo_hbm, w1_hbm, w3_hbm, w2_hbm,
            c_ref, wmod_hbm, out_hbm,
            wqkv, big32, w13_32, ring, oring, xb, xf, mod, hs, ot, fill_ref, prob, acc, early, sems, osems,
            *, S, D, H, F, M, SEG, FB):
    NSEG = S // SEG
    XR = SEG - M
    P = S - NSEG * XR
    R = ring.shape[1]
    QOFF = R - P
    OOFF = (-NSEG * XR) % R
    ND = D // LANE
    NF = F // LANE
    HP = H // 2
    HD = H * LANE
    scale = float(LANE) ** -0.5
    big, w13 = big32.bitcast(BF16), w13_32.bitcast(BF16)
    DH = D // 2
    PG = 8
    NA = HP // PG
    NSLOT = big32.shape[0] // DH
    WP = wqkv.shape[0] // (3 * H)
    WO = ND * HD

    def slab(row0, rows):
        return pltpu.bitcast(big32[pl.ds(row0 // 16, rows // 16)].reshape(rows // 2, LANE), BF16)

    def slab_copies(src, tiles, dst_fn, sem):
        return [pltpu.make_async_copy(src.at[..., pl.ds(j * LANE, LANE)], dst_fn(j), sem) for j in tiles]

    def half_tiles(c):
        return [v * ND + c * ND // 2 + j for v in range(2) for j in range(ND // 2)]

    cp_x0 = pltpu.make_async_copy(x_hbm.at[pl.ds(0, P)], xb.at[pl.ds(0, P)], sems.at[0])
    cp_x1 = pltpu.make_async_copy(x_hbm.at[pl.ds(P, S - P)], xb.at[pl.ds(P, S - P)], sems.at[1])
    mod_tiles = [half_tiles(0), half_tiles(1), list(range(2 * ND, 6 * ND))]
    cp_mod = [slab_copies(wmod_hbm, t, lambda j: w13.at[j], sems.at[2 + i])
              for i, t in enumerate(mod_tiles)]
    cp_w = [pltpu.make_async_copy(w.at[pl.ds(c * DH, DH), a],
                                  big.at[pl.ds(((2 * t + c) * NA + a) % NSLOT * DH, DH)],
                                  sems.at[7 + (2 * t + c) * NA + a])
            for t, w in enumerate((wq_hbm, wk_hbm, wv_hbm)) for c in range(2) for a in range(NA)]
    cp_o = slab_copies(wo_hbm, range(ND), lambda j: big.at[pl.ds((WO + j * HD) // 16, HD // 16)], sems.at[5])
    cp_ffn = (slab_copies(w1_hbm, range(NF), lambda j: w13.at[2 * j], sems.at[6])
              + slab_copies(w3_hbm, range(NF), lambda j: w13.at[2 * j + 1], sems.at[6])
              + slab_copies(w2_hbm, range(ND), lambda j: big.at[pl.ds(j * F // 16, F // 16)], sems.at[6]))

    def start(cps):
        for cp in cps:
            cp.start()

    def wait(cps):
        for cp in cps:
            cp.wait()

    start(cp_mod[0])
    cp_x0.start()
    cp_w[0].start()

    cc = jnp.broadcast_to(c_ref[...].astype(F32), (16, D))
    sc = _silu(cc).astype(BF16)

    def mod_part(i):
        wait(cp_mod[i])
        for j in mod_tiles[i]:
            r = _dot(sc, pltpu.bitcast(w13_32[j], BF16))[0:8]
            if j // ND in (1, 4):
                r = r + 1.0
            mod[j // ND, :, pl.ds((j % ND) * LANE, LANE)] = r

    def modv(i):
        return mod[i, 0:1, :]

    G = 2 * (M + SEG)
    ri = lax.broadcasted_iota(jnp.int32, (G, LANE), 0)
    ci = lax.broadcasted_iota(jnp.int32, (G, LANE), 1)

    def head_pos(i):
        head = jnp.where(i < 2 * M, i // M, (i - 2 * M) // SEG)
        pos = jnp.where(i < 2 * M, i % M, M + (i - 2 * M) % SEG)
        return head, pos

    rh, rp = head_pos(ri)
    ch, cp_ = head_pos(ci)
    visible = (rp < M) | (rp >= cp_)
    fill_ref[...] = jnp.where(rh == ch, jnp.where(visible, 0.0, -1e9), -jnp.inf).astype(F32)

    LB = 128
    PH = P // 2
    DQ = D // 4

    def norm_half(c):
        cols = slice(c * DH, (c + 1) * DH)

        def norm0(k, carry):
            halves = []
            for o in (0, PH):
                rows = pl.ds(pl.multiple_of(o + k * LB, LB), LB)
                xv = xb[rows, :].astype(F32)
                xf[rows, cols] = xv[:, cols]
                halves.append(_norm(xv)[:, cols] * mod[1, 0:1, cols] + mod[0, 0:1, cols])
            top, bot = halves
            ops = _strassen_lhs(top[:, :DQ], top[:, DQ:], bot[:, :DQ], bot[:, DQ:])
            for i in range(7):
                hs[i, pl.ds(pl.multiple_of(c * (PH // 2) + k * (LB // 2), LB // 2), LB // 2), :] = ops[i]
            return carry

        lax.fori_loop(0, PH // LB, norm0, 0)

    def arrivals(it):
        if it == 0:
            cp_w[0].wait()
            start(cp_w[2:3] + cp_mod[1] + cp_w[3:4])
        else:
            wait(cp_w[it + (it > 1):it + 2])
        if it == 1:
            start(cp_w[4:6])
        if it == NA:
            start(cp_w[6:NSLOT])
            mod_part(1)
            norm_half(1)
        if 3 <= it < 3 + len(cp_w) - NSLOT:
            cp_w[NSLOT + it - 3].start()
        if it == 4:
            cp_x1.start()
        if it == NSLOT - 2:
            start(cp_mod[2])
        if it == NSLOT - 1:
            start(cp_o)

    def head_rows(it):
        chunk, a = it // NA, it % NA
        base = (chunk // 2 * H + 2 * PG * a) * WP + chunk % 2 * (DH // 2)
        return wqkv.at[pl.ds(pl.multiple_of(base, 8), 2 * PG * WP - DH // 2)]

    def retile(it, r0, r1):
        src = big32.at[pl.ds(it % NSLOT * DH, DH)]
        dst = head_rows(it)
        for r in range(r0, r1):
            even, odd = src[2 * r], src[2 * r + 1]
            dst[pl.ds(r, PG, stride=2 * WP), :] = (even & jnp.uint32(0xFFFF)) | (odd << 16)
            dst[pl.ds(WP + r, PG, stride=2 * WP), :] = (even >> 16) | (odd & jnp.uint32(0xFFFF0000))

    def project(it, carry):
        for ev in range(len(cp_w) - 1):
            pl.when(it == ev)(functools.partial(arrivals, ev))
        pl.when(it < 2)(lambda: retile(it, 0, DH // 2))
        half = it // NA % 2
        hrows = pl.ds(pl.multiple_of(half * (PH // 2), PH // 2), PH // 2)
        nxt = jnp.where(it == 0, 0, jnp.minimum(it + 1, 6 * NA - 1))
        for b in range(PG):
            n = it // (2 * NA) * H + 2 * (PG * (it % NA) + b)
            lo, hi = (pltpu.bitcast(head_rows(it)[pl.ds((2 * b + i) * WP, DH // 2), :], BF16)
                      for i in range(2))

            def emit(i, r, n=n):
                dst = ring.at[n + i % 2, pl.ds(QOFF + i // 2 * PH, PH)]
                dst[...] = r + jnp.where(half == 1, dst[...], 0.0)

            _strassen(lambda i: hs[i, hrows, :], lo[:DQ], hi[:DQ], lo[DQ:], hi[DQ:], emit)
            retile(nxt, b * (DH // 2) // PG, (b + 1) * (DH // 2) // PG)
        return carry

    mod_part(0)
    cp_w[1].start()
    cp_x0.wait()
    norm_half(0)
    lax.fori_loop(0, 6 * NA, project, 0)
    mod_part(2)
    start(cp_ffn)

    HG = SEG // 2
    xf3, xb3 = xf.reshape(NSEG, SEG, D), xb.reshape(NSEG, SEG, D)

    def ffn_norm(grp):
        hn = _ada_ln(xf[pl.ds(pl.multiple_of(grp * SEG, SEG), SEG), :], modv(3), modv(4))
        ops = _strassen_lhs(hn[:HG, :DH], hn[:HG, DH:], hn[HG:, :DH], hn[HG:, DH:])
        for i in range(7):
            for t in range(ND // 2):
                ring[3 * H + i * (ND // 2) + t, pl.ds(pl.multiple_of(grp * (HG // 2), HG // 2), HG // 2), :] = (
                    pltpu.bitcast(ops[i][:, t * LANE:(t + 1) * LANE], F32))

    lhs = ring.at[3 * H + 7 * (ND // 2)]

    def widen(grp):
        rows = pl.ds(pl.multiple_of(grp * SEG, SEG), SEG)
        xf[rows, :] = xb[rows, :].astype(F32)

    def next_rows(r0):
        hn = _ada_ln(xf[pl.ds(r0, XR), :], modv(0), modv(1))
        for t in range(ND):
            lhs[pl.ds(t * SEG + M, XR), :] = hn[:, t * LANE:(t + 1) * LANE]

    for t in range(ND):
        lhs[pl.ds(t * SEG, M), :] = mem0_ref[:, pl.ds(t * LANE, LANE)].astype(F32)
    cp_x1.wait()
    widen(P // SEG)
    next_rows(P)
    wait(cp_o)

    def step(s, carry):
        q_wr = pl.multiple_of(lax.rem(s * XR, R), 8)
        q_rd = pl.multiple_of(lax.rem(s * SEG + QOFF, R), 8)
        o_wr = pl.multiple_of(lax.rem(s * SEG + OOFF, R), 8)
        o_rd = pl.multiple_of(lax.rem(s * XR + OOFF, R), 8)
        h = jnp.concatenate([lhs[pl.ds(t * SEG, SEG), :] for t in range(ND)], axis=1).astype(BF16)
        tail_rows = pl.ds(pl.multiple_of(jnp.maximum(s - NSEG * XR // SEG, 0) * (HG // 2), HG // 2), HG // 2)
        pad = jnp.zeros((LANE - G, LANE), BF16)

        for u in range(4 * SPLIT):
            n = u // 2 % 2 * H + u // 4 * 2 + u % 2
            early[u] = _dot(h[:, :DH], pltpu.bitcast(wqkv[pl.ds(n * WP, DH // 2), :], BF16))

        def head_pair(t, g):
            n = t * H + 2 * g
            mem_rows = []
            for i in range(2):
                if t < 2 and g < SPLIT:
                    r = (_dot(h[:, DH:], pltpu.bitcast(wqkv[pl.ds((n + i) * WP + DH // 2, DH // 2), :], BF16))
                         + early[4 * g + 2 * t + i])
                else:
                    r = _dot(h, pltpu.bitcast(wqkv[pl.ds((n + i) * WP, DH), :], BF16))
                ring[n + i, pl.ds(q_wr, XR), :] = r[M:]
                mem_rows.append(r[:M])
            return jnp.concatenate(
                mem_rows + [ring[n + i, pl.ds(q_rd, SEG), :] for i in range(2)],
                axis=0).astype(BF16)

        def scores(q, k):
            sc_ = lax.dot_general(q, jnp.concatenate([k, pad], axis=0), (((1,), (1,)), ((), ())),
                                  preferred_element_type=F32)
            fill = fill_ref[...]
            sc_ = jnp.where(fill == 0.0, sc_ * scale, fill)
            e = jnp.exp(sc_ - jnp.max(sc_, axis=-1, keepdims=True))
            return (e * (1.0 / jnp.sum(e, axis=-1, keepdims=True))).astype(BF16)

        def attend(g, p, v):
            o = _dot(p, jnp.concatenate([v, pad], axis=0))
            ops = _strassen_lhs(*(o[2 * M + i * SEG + r:2 * M + i * SEG + r + HG]
                                  for r in (0, HG) for i in range(2)))
            for i in range(7):
                ot[i, tail_rows, pl.ds(g * LANE, LANE)] = ops[i]
            for i in range(2):
                oring[2 * g + i, pl.ds(o_wr, SEG), :] = o[2 * M + i * SEG:2 * M + (i + 1) * SEG]
            return functools.cache(lambda: [jnp.concatenate(
                [o[i * M:(i + 1) * M], oring[2 * g + i, pl.ds(o_rd, XR), :]],
                axis=0).astype(BF16) for i in range(2)])

        heads = {}

        def oproj(g0, g1, j0=0, j1=ND):
            a = jnp.concatenate([r for g in range(g0, g1) for r in heads[g]()], axis=1)
            for j in range(j0, j1):
                cols = pl.ds(j * LANE, LANE)
                r = _dot(a, slab(WO + j * HD + g0 * 2 * LANE, (g1 - g0) * 2 * LANE))
                if g0 > 0:
                    r = r + acc[:, cols]
                if g1 < HP:
                    acc[:, cols] = r
                else:
                    lhs[pl.ds(j * SEG, M), :] = r[:M]
                    xf[rows, cols] = xf[rows, cols] + mod[2, 0:1, cols] * r[M:]

        rows = pl.ds(pl.multiple_of(s * XR, 8), XR)
        qk, val = {}, {}
        LAG = VLAG
        for i in range(2 * HP + LAG):
            if i == PIN1:
                widen(jnp.minimum(P // SEG + 1 + s, NSEG - 1))
                next_rows(pl.multiple_of(jnp.minimum(P + (s + 1) * XR, S - XR), 8))
            if i == PIN2:
                ffn_norm(jnp.maximum(s * XR // SEG - 1, 0))
            if i < HP:
                qk[i] = head_pair(0, i), head_pair(1, i)
            elif i < 2 * HP:
                val[i - HP] = head_pair(2, i - HP)
            else:
                oproj(0, HP // 2, i - 2 * HP, i - 2 * HP + 1)
            if i % AGS == 0 and 0 < i <= HP:
                for g, q, k in [(g, *qk[g]) for g in range(i - AGS, i)]:
                    prob[g] = pltpu.bitcast(scores(q, k), U32)
            g1 = i - HP - LAG + 1
            if g1 % AG == 0 and g1 > 0:
                for g, v in [(g, val[g]) for g in range(g1 - AG, g1)]:
                    heads[g] = attend(g, pltpu.bitcast(prob[g], BF16), v)
                for g in range(max(g1 - AG - OLAG, 0), g1 - OLAG):
                    heads[g]()
        oproj(0, HP // 2, LAG, ND)
        oproj(HP // 2, HP)
        return carry

    lax.fori_loop(0, NSEG, step, 0, unroll=UNROLL_STEP)

    MH = FB // 2

    def row_tiles(row0, n, par):
        return jnp.concatenate([slab(row0 + (2 * k + par) * LANE, LANE) for k in range(n // 2)], axis=0)

    def otail(j, carry):
        def emit(n, y):
            cols = pl.ds(pl.multiple_of((2 * j + n % 2) * LANE, LANE), LANE)
            idx = (pl.ds(NSEG * XR // SEG, P // SEG), pl.ds(n // 2 * HG, HG), cols)
            xf3[idx] = xf3[idx] + (mod[2, 0:1, cols] * y).reshape(P // SEG, HG, LANE)

        _strassen(lambda i: ot[i],
                  *(row_tiles(WO + (2 * j + u) * HD, H, par) for par in range(2) for u in range(2)), emit)
        return carry

    lax.fori_loop(0, ND // 2, otail, 0)
    G0 = (NSEG - 1) * XR // SEG - 1

    def norm_tail(i, carry):
        for u in range(6):
            ffn_norm(G0 + 6 * i + u)
        return carry

    lax.fori_loop(0, (NSEG - G0) // 6, norm_tail, 0)

    wait(cp_ffn)

    def act_slot(k, i):
        return wqkv.at[pl.ds(pl.multiple_of((7 * k + i) * (MH // 2), MH // 2), MH // 2)]

    def out_copy(blk, j):
        idx = (pl.ds(pl.multiple_of(blk * FB, FB), FB), pl.ds(pl.multiple_of(j * 2 * LANE, 2 * LANE), 2 * LANE))
        return pltpu.make_async_copy(xb.at[idx], out_hbm.at[idx], osems.at[blk * (ND // 2) + j])

    def ffn(blk, carry):
        def normed(i):
            rows = pl.ds(pl.multiple_of(blk * (MH // 2), MH // 2), MH // 2)
            return jnp.concatenate([ring[3 * H + i * (ND // 2) + t, rows, :] for t in range(ND // 2)], axis=1)

        def up(k, c):
            res = {}, {}
            for t in range(2):
                b1, b2 = (pltpu.bitcast(w13_32[4 * k + 2 * u + t], BF16) for u in range(2))
                _strassen(normed,
                          b1[:DH], b2[:DH], b1[DH:], b2[DH:], res[t].__setitem__)
            ops = _strassen_lhs(*(_silu(res[0][n]) * res[1][n] for n in range(4)))
            for i in (1, 3, 6, 0, 2, 4, 5):
                act_slot(k, i)[...] = ops[i]
            return c

        lax.fori_loop(0, NF // 2, up, 0, unroll=UNROLL_UP)

        def down(j, c):
            def emit(n, y):
                cols = pl.ds(pl.multiple_of((2 * j + n % 2) * LANE, LANE), LANE)
                idx = (pl.ds(blk * (FB // SEG), FB // SEG), pl.ds(n // 2 * HG, HG), cols)
                xb3[idx] = (xf3[idx] + (mod[5, 0:1, cols] * y).reshape(FB // SEG, HG, LANE)).astype(BF16)

            _strassen(lambda i: jnp.concatenate([act_slot(k, i)[...] for k in range(NF // 2)], axis=1),
                      *(row_tiles((2 * j + u) * F, NF, par) for par in range(2) for u in range(2)), emit)
            out_copy(blk, j).start()
            return c

        lax.fori_loop(0, ND // 2, down, 0)
        return carry

    lax.fori_loop(0, S // FB, ffn, 0)
    for blk in range(S // FB):
        for j in range(ND // 2):
            out_copy(blk, j).wait()


@functools.partial(jax.jit, static_argnames=("A_seg_len",))
def pallas_adaLN_cond__memory_aug_recurrent_mem_tr__glu_gated_swiglu__prompt_kernel(
    A_x, A_mem0, A_Wq, A_Wk, A_Wv, A_Wo, A_seg_len, B_x, B_w1, B_w3, B_w2, c, w_mod,
):
    del B_x
    B, S, D = A_x.shape
    _, H, Dh = A_Wq.shape
    M = A_mem0.shape[1]
    F = B_w1.shape[1]
    SEG = int(A_seg_len)
    assert (B, S, D, H, Dh, M, SEG) == (1, 2048, 1024, 32, LANE, 8, 32) and F % 512 == 0
    P = S // SEG * M
    R = 576
    FB = 1024

    hbm = pl.BlockSpec(memory_space=pl.ANY)
    vmem = pl.BlockSpec(memory_space=pltpu.VMEM)
    out = pl.pallas_call(
        functools.partial(_kernel, S=S, D=D, H=H, F=F, M=M, SEG=SEG, FB=FB),
        out_shape=jax.ShapeDtypeStruct((S, D), A_x.dtype),
        in_specs=[hbm, vmem, hbm, hbm, hbm, hbm, hbm, hbm, hbm, vmem, hbm],
        out_specs=hbm,
        scratch_shapes=[
            pltpu.VMEM((3 * H * (D // 2 + 2), LANE), U32),
            pltpu.VMEM((D * H // 8, 8, LANE), U32),
            pltpu.VMEM((2 * F // LANE, D // 2, LANE), U32),
            pltpu.VMEM((3 * H + 7 * D // (2 * LANE) + 1, R, LANE), F32),
            pltpu.VMEM((H, R, LANE), F32),
            pltpu.VMEM((S, D), BF16),
            pltpu.VMEM((S, D), F32),
            pltpu.VMEM((6, 8, D), F32),
            pltpu.VMEM((7, P // 2, D // 4), U32),
            pltpu.VMEM((7, P // 4, H * Dh // 2), U32),
            pltpu.VMEM((2 * (M + SEG), LANE), F32),
            pltpu.VMEM((H // 2, M + SEG, LANE), U32),
            pltpu.VMEM((SEG, D), F32),
            pltpu.VMEM((8, SEG, LANE), F32),
            pltpu.SemaphoreType.DMA((7 + 6 * H // 16,)),
            pltpu.SemaphoreType.DMA((S // FB * D // (2 * LANE),)),
        ],
        compiler_params=pltpu.CompilerParams(vmem_limit_bytes=126 * 2**20),
        name="adaln_rmt_swiglu",
    )(A_x.reshape(S, D), A_mem0.reshape(M, D), *(w.reshape(D, H // 16, 16, Dh) for w in (A_Wq, A_Wk, A_Wv)),
      A_Wo.reshape(H * Dh // 16, 16, D), B_w1, B_w3, B_w2.reshape(F // 16, 16, D), c, w_mod)
    return out.reshape(B, S, D)
```

```python
import functools

import jax
import jax.numpy as jnp
from jax import lax
import jax.experimental.pallas as pl
import jax.experimental.pallas.tpu as pltpu

F32 = jnp.float32
BF16 = jnp.bfloat16
U32 = jnp.uint32
LANE = 128
EPS = 1e-5
VLAG = 4
AG = 1
OLAG = 0
OCUT = 0
SLAG = 1
AGS = 4
PIN1 = 14
PIN2 = 18
UNROLL_STEP = 2
SPLIT = 2
UNROLL_UP = 2


def _dot(a, b):
    return jnp.dot(a, b, preferred_element_type=F32)


def _norm(x):
    m = jnp.mean(x, axis=-1, keepdims=True)
    d = x - m
    v = jnp.mean(d * d, axis=-1, keepdims=True)
    return d * lax.rsqrt(v + EPS)


def _ada_ln(x, shift, scale1):
    return _norm(x) * scale1 + shift


def _silu(x):
    h = 0.5 * x
    return h + h * jnp.tanh(h)


def _words(x):
    return pltpu.bitcast(x.astype(BF16), U32)


def _strassen_lhs(a11, a12, a21, a22):
    return [_words(a) for a in (a11 + a22, a21 + a22, a11, a22, a11 + a12, a21 - a11, a12 - a22)]


def _strassen(lhs_fn, b11, b12, b21, b22, emit):
    f11, f12, f21, f22 = (b.astype(F32) for b in (b11, b12, b21, b22))

    def prod(i, b):
        return _dot(pltpu.bitcast(lhs_fn(i), BF16), b.astype(BF16))

    m2 = prod(1, b11)
    m4 = prod(3, f21 - f11)
    emit(2, m2 + m4)
    m3 = prod(2, f12 - f22)
    m5 = prod(4, b22)
    emit(1, m3 + m5)
    m1 = prod(0, f11 + f22)
    emit(3, (m1 - m2 + m3) + prod(5, f11 + f12))
    emit(0, (m1 + m4 - m5) + prod(6, f21 + f22))


def _kernel(x_hbm, mem0_ref, wq_hbm, wk_hbm, wv_hbm, wo_hbm, w1_hbm, w3_hbm, w2_hbm,
            c_ref, wmod_hbm, out_hbm,
            wqkv, big32, w13_32, ring, oring, xb, xf, mod, hs, ot, fill_ref, prob, acc, early, sems, osems,
            *, S, D, H, F, M, SEG, FB):
    NSEG = S // SEG
    XR = SEG - M
    P = S - NSEG * XR
    R = ring.shape[1]
    QOFF = R - P
    OOFF = (-NSEG * XR) % R
    ND = D // LANE
    NF = F // LANE
    HP = H // 2
    HD = H * LANE
    scale = float(LANE) ** -0.5
    big, w13 = big32.bitcast(BF16), w13_32.bitcast(BF16)
    DH = D // 2
    PG = 8
    NA = HP // PG
    NSLOT = big32.shape[0] // DH
    WP = wqkv.shape[0] // (3 * H)
    WO = ND * HD

    def slab(row0, rows):
        return pltpu.bitcast(big32[pl.ds(row0 // 16, rows // 16)].reshape(rows // 2, LANE), BF16)

    def slab_copies(src, tiles, dst_fn, sem):
        return [pltpu.make_async_copy(src.at[..., pl.ds(j * LANE, LANE)], dst_fn(j), sem) for j in tiles]

    def half_tiles(c):
        return [v * ND + c * ND // 2 + j for v in range(2) for j in range(ND // 2)]

    cp_x0 = pltpu.make_async_copy(x_hbm.at[pl.ds(0, P)], xb.at[pl.ds(0, P)], sems.at[0])
    cp_x1 = pltpu.make_async_copy(x_hbm.at[pl.ds(P, S - P)], xb.at[pl.ds(P, S - P)], sems.at[1])
    mod_tiles = [half_tiles(0), half_tiles(1), list(range(2 * ND, 6 * ND))]
    cp_mod = [slab_copies(wmod_hbm, t, lambda j: w13.at[j], sems.at[2 + i])
              for i, t in enumerate(mod_tiles)]
    cp_w = [pltpu.make_async_copy(w.at[pl.ds(c * DH, DH), a],
                                  big.at[pl.ds(((2 * t + c) * NA + a) % NSLOT * DH, DH)],
                                  sems.at[7 + (2 * t + c) * NA + a])
            for t, w in enumerate((wq_hbm, wk_hbm, wv_hbm)) for c in range(2) for a in range(NA)]
    cp_o = slab_copies(wo_hbm, range(ND), lambda j: big.at[pl.ds((WO + j * HD) // 16, HD // 16)], sems.at[5])
    cp_ffn = (slab_copies(w1_hbm, range(NF), lambda j: w13.at[2 * j], sems.at[6])
              + slab_copies(w3_hbm, range(NF), lambda j: w13.at[2 * j + 1], sems.at[6])
              + slab_copies(w2_hbm, range(ND), lambda j: big.at[pl.ds(j * F // 16, F // 16)], sems.at[6]))

    def start(cps):
        for cp in cps:
            cp.start()

    def wait(cps):
        for cp in cps:
            cp.wait()

    start(cp_mod[0])
    cp_x0.start()
    cp_w[0].start()

    cc = jnp.broadcast_to(c_ref[...].astype(F32), (16, D))
    sc = _silu(cc).astype(BF16)

    def mod_part(i):
        wait(cp_mod[i])
        for j in mod_tiles[i]:
            r = _dot(sc, pltpu.bitcast(w13_32[j], BF16))[0:8]
            if j // ND in (1, 4):
                r = r + 1.0
            mod[j // ND, :, pl.ds((j % ND) * LANE, LANE)] = r

    def modv(i):
        return mod[i, 0:1, :]

    G = 2 * (M + SEG)
    ri = lax.broadcasted_iota(jnp.int32, (G, LANE), 0)
    ci = lax.broadcasted_iota(jnp.int32, (G, LANE), 1)

    def head_pos(i):
        head = jnp.where(i < 2 * M, i // M, (i - 2 * M) // SEG)
        pos = jnp.where(i < 2 * M, i % M, M + (i - 2 * M) % SEG)
        return head, pos

    rh, rp = head_pos(ri)
    ch, cp_ = head_pos(ci)
    visible = (rp < M) | (rp >= cp_)
    fill_ref[...] = jnp.where(rh == ch, jnp.where(visible, 0.0, -1e9), -jnp.inf).astype(F32)

    LB = 128
    PH = P // 2
    DQ = D // 4

    def norm_half(c):
        cols = slice(c * DH, (c + 1) * DH)

        def norm0(k, carry):
            halves = []
            for o in (0, PH):
                rows = pl.ds(pl.multiple_of(o + k * LB, LB), LB)
                xv = xb[rows, :].astype(F32)
                xf[rows, cols] = xv[:, cols]
                halves.append(_norm(xv)[:, cols] * mod[1, 0:1, cols] + mod[0, 0:1, cols])
            top, bot = halves
            ops = _strassen_lhs(top[:, :DQ], top[:, DQ:], bot[:, :DQ], bot[:, DQ:])
            for i in range(7):
                hs[i, pl.ds(pl.multiple_of(c * (PH // 2) + k * (LB // 2), LB // 2), LB // 2), :] = ops[i]
            return carry

        lax.fori_loop(0, PH // LB, norm0, 0)

    def arrivals(it):
        if it == 0:
            cp_w[0].wait()
            start(cp_w[2:3] + cp_mod[1] + cp_w[3:4])
        else:
            wait(cp_w[it + (it > 1):it + 2])
        if it == 1:
            start(cp_w[4:6])
        if it == NA:
            start(cp_w[6:NSLOT])
            mod_part(1)
            norm_half(1)
        if it == 4:
            start(cp_w[NSLOT:] + [cp_x1] + cp_mod[2])
        if it == NSLOT - 1:
            wait(cp_w[it + 2:])
            start(cp_o)

    def head_rows(it):
        chunk, a = it // NA, it % NA
        base = (chunk // 2 * H + 2 * PG * a) * WP + chunk % 2 * (DH // 2)
        return wqkv.at[pl.ds(pl.multiple_of(base, 8), 2 * PG * WP - DH // 2)]

    def retile(it, r0, r1):
        src = big32.at[pl.ds(it % NSLOT * DH, DH)]
        dst = head_rows(it)
        for r in range(r0, r1):
            even, odd = src[2 * r], src[2 * r + 1]
            dst[pl.ds(r, PG, stride=2 * WP), :] = (even & jnp.uint32(0xFFFF)) | (odd << 16)
            dst[pl.ds(WP + r, PG, stride=2 * WP), :] = (even >> 16) | (odd & jnp.uint32(0xFFFF0000))

    def project(it, carry):
        for ev in range(NSLOT):
            pl.when(it == ev)(functools.partial(arrivals, ev))
        pl.when(it < 2)(lambda: retile(it, 0, DH // 2))
        half = it // NA % 2
        hrows = pl.ds(pl.multiple_of(half * (PH // 2), PH // 2), PH // 2)
        nxt = jnp.where(it == 0, 0, jnp.minimum(it + 1, 6 * NA - 1))
        for b in range(PG):
            n = it // (2 * NA) * H + 2 * (PG * (it % NA) + b)
            lo, hi = (pltpu.bitcast(head_rows(it)[pl.ds((2 * b + i) * WP, DH // 2), :], BF16)
                      for i in range(2))

            def emit(i, r, n=n):
                dst = ring.at[n + i % 2, pl.ds(QOFF + i // 2 * PH, PH)]
                dst[...] = r + jnp.where(half == 1, dst[...], 0.0)

            _strassen(lambda i: hs[i, hrows, :], lo[:DQ], hi[:DQ], lo[DQ:], hi[DQ:], emit)
            retile(nxt, b * (DH // 2) // PG, (b + 1) * (DH // 2) // PG)
        return carry

    mod_part(0)
    cp_w[1].start()
    cp_x0.wait()
    norm_half(0)
    lax.fori_loop(0, 6 * NA, project, 0)
    mod_part(2)
    start(cp_ffn)

    HG = SEG // 2
    xf3, xb3 = xf.reshape(NSEG, SEG, D), xb.reshape(NSEG, SEG, D)

    def ffn_norm(grp):
        hn = _ada_ln(xf[pl.ds(pl.multiple_of(grp * SEG, SEG), SEG), :], modv(3), modv(4))
        ops = _strassen_lhs(hn[:HG, :DH], hn[:HG, DH:], hn[HG:, :DH], hn[HG:, DH:])
        for i in range(7):
            for t in range(ND // 2):
                ring[3 * H + i * (ND // 2) + t, pl.ds(pl.multiple_of(grp * (HG // 2), HG // 2), HG // 2), :] = (
                    pltpu.bitcast(ops[i][:, t * LANE:(t + 1) * LANE], F32))

    lhs = ring.at[3 * H + 7 * (ND // 2)]

    def widen(grp):
        rows = pl.ds(pl.multiple_of(grp * SEG, SEG), SEG)
        xf[rows, :] = xb[rows, :].astype(F32)

    def next_rows(r0):
        hn = _ada_ln(xf[pl.ds(r0, XR), :], modv(0), modv(1))
        for t in range(ND):
            lhs[pl.ds(t * SEG + M, XR), :] = hn[:, t * LANE:(t + 1) * LANE]

    for t in range(ND):
        lhs[pl.ds(t * SEG, M), :] = mem0_ref[:, pl.ds(t * LANE, LANE)].astype(F32)
    cp_x1.wait()
    widen(P // SEG)
    next_rows(P)
    wait(cp_o)

    def step(s, carry):
        q_wr = pl.multiple_of(lax.rem(s * XR, R), 8)
        q_rd = pl.multiple_of(lax.rem(s * SEG + QOFF, R), 8)
        o_wr = pl.multiple_of(lax.rem(s * SEG + OOFF, R), 8)
        o_rd = pl.multiple_of(lax.rem(s * XR + OOFF, R), 8)
        h = jnp.concatenate([lhs[pl.ds(t * SEG, SEG), :] for t in range(ND)], axis=1).astype(BF16)
        tail_rows = pl.ds(pl.multiple_of(jnp.maximum(s - NSEG * XR // SEG, 0) * (HG // 2), HG // 2), HG // 2)
        pad = jnp.zeros((LANE - G, LANE), BF16)

        for u in range(4 * SPLIT):
            n = u // 2 % 2 * H + u // 4 * 2 + u % 2
            early[u] = _dot(h[:, :DH], pltpu.bitcast(wqkv[pl.ds(n * WP, DH // 2), :], BF16))

        def head_pair(t, g):
            n = t * H + 2 * g
            mem_rows = []
            for i in range(2):
                if t < 2 and g < SPLIT:
                    r = (_dot(h[:, DH:], pltpu.bitcast(wqkv[pl.ds((n + i) * WP + DH // 2, DH // 2), :], BF16))
                         + early[4 * g + 2 * t + i])
                else:
                    r = _dot(h, pltpu.bitcast(wqkv[pl.ds((n + i) * WP, DH), :], BF16))
                ring[n + i, pl.ds(q_wr, XR), :] = r[M:]
                mem_rows.append(r[:M])
            return jnp.concatenate(
                mem_rows + [ring[n + i, pl.ds(q_rd, SEG), :] for i in range(2)],
                axis=0).astype(BF16)

        def scores(q, k):
            sc_ = lax.dot_general(q, jnp.concatenate([k, pad], axis=0), (((1,), (1,)), ((), ())),
                                  preferred_element_type=F32)
            fill = fill_ref[...]
            sc_ = jnp.where(fill == 0.0, sc_ * scale, fill)
            e = jnp.exp(sc_ - jnp.max(sc_, axis=-1, keepdims=True))
            return (e * (1.0 / jnp.sum(e, axis=-1, keepdims=True))).astype(BF16)

        def attend(g, p, v):
            o = _dot(p, jnp.concatenate([v, pad], axis=0))
            ops = _strassen_lhs(*(o[2 * M + i * SEG + r:2 * M + i * SEG + r + HG]
                                  for r in (0, HG) for i in range(2)))
            for i in range(7):
                ot[i, tail_rows, pl.ds(g * LANE, LANE)] = ops[i]
            for i in range(2):
                oring[2 * g + i, pl.ds(o_wr, SEG), :] = o[2 * M + i * SEG:2 * M + (i + 1) * SEG]
            return functools.cache(lambda: [jnp.concatenate(
                [o[i * M:(i + 1) * M], oring[2 * g + i, pl.ds(o_rd, XR), :]],
                axis=0).astype(BF16) for i in range(2)])

        heads = {}

        def oproj(g0, g1, j0=0, j1=ND):
            a = jnp.concatenate([r for g in range(g0, g1) for r in heads[g]()], axis=1)
            for j in range(j0, j1):
                cols = pl.ds(j * LANE, LANE)
                r = _dot(a, slab(WO + j * HD + g0 * 2 * LANE, (g1 - g0) * 2 * LANE))
                if g0 > 0:
                    r = r + acc[:, cols]
                if g1 < HP:
                    acc[:, cols] = r
                else:
                    lhs[pl.ds(j * SEG, M), :] = r[:M]
                    xf[rows, cols] = xf[rows, cols] + mod[2, 0:1, cols] * r[M:]

        rows = pl.ds(pl.multiple_of(s * XR, 8), XR)
        qk, val = {}, {}
        LAG = VLAG
        for i in range(2 * HP + LAG):
            if i == PIN1:
                widen(jnp.minimum(P // SEG + 1 + s, NSEG - 1))
                next_rows(pl.multiple_of(jnp.minimum(P + (s + 1) * XR, S - XR), 8))
            if i == PIN2:
                ffn_norm(jnp.maximum(s * XR // SEG - 1, 0))
            if i < HP:
                qk[i] = head_pair(0, i), head_pair(1, i)
            elif i < 2 * HP:
                val[i - HP] = head_pair(2, i - HP)
            else:
                oproj(0, HP // 2, i - 2 * HP, i - 2 * HP + 1)
            i0 = i - SLAG
            if i0 % AGS == 0 and 0 < i0 <= HP:
                for g, q, k in [(g, *qk[g]) for g in range(i0 - AGS, i0)]:
                    prob[g] = pltpu.bitcast(scores(q, k), U32)
            g1 = i - HP - LAG + 1
            if g1 % AG == 0 and g1 > 0:
                for g, v in [(g, val[g]) for g in range(g1 - AG, g1)]:
                    heads[g] = attend(g, pltpu.bitcast(prob[g], BF16), v)
                for g in range(max(g1 - AG - OLAG, 0), g1 - OLAG):
                    heads[g]()
        oproj(0, HP // 2, LAG, ND)
        if OCUT:
            oproj(HP // 2, OCUT)
        oproj(OCUT or HP // 2, HP)
        return carry

    lax.fori_loop(0, NSEG, step, 0, unroll=UNROLL_STEP)

    MH = FB // 2

    def row_tiles(row0, n, par):
        return jnp.concatenate([slab(row0 + (2 * k + par) * LANE, LANE) for k in range(n // 2)], axis=0)

    def otail(j, carry):
        def emit(n, y):
            cols = pl.ds(pl.multiple_of((2 * j + n % 2) * LANE, LANE), LANE)
            idx = (pl.ds(NSEG * XR // SEG, P // SEG), pl.ds(n // 2 * HG, HG), cols)
            xf3[idx] = xf3[idx] + (mod[2, 0:1, cols] * y).reshape(P // SEG, HG, LANE)

        _strassen(lambda i: ot[i],
                  *(row_tiles(WO + (2 * j + u) * HD, H, par) for par in range(2) for u in range(2)), emit)
        return carry

    lax.fori_loop(0, ND // 2, otail, 0)
    G0 = (NSEG - 1) * XR // SEG - 1

    def norm_tail(i, carry):
        for u in range(6):
            ffn_norm(G0 + 6 * i + u)
        return carry

    lax.fori_loop(0, (NSEG - G0) // 6, norm_tail, 0)

    wait(cp_ffn)

    def act_slot(k, i):
        return wqkv.at[pl.ds(pl.multiple_of((7 * k + i) * (MH // 2), MH // 2), MH // 2)]

    def out_copy(blk, j):
        idx = (pl.ds(pl.multiple_of(blk * FB, FB), FB), pl.ds(pl.multiple_of(j * 2 * LANE, 2 * LANE), 2 * LANE))
        return pltpu.make_async_copy(xb.at[idx], out_hbm.at[idx], osems.at[blk * (ND // 2) + j])

    def ffn(blk, carry):
        def normed(i):
            rows = pl.ds(pl.multiple_of(blk * (MH // 2), MH // 2), MH // 2)
            return jnp.concatenate([ring[3 * H + i * (ND // 2) + t, rows, :] for t in range(ND // 2)], axis=1)

        def up(k, c):
            res = {}, {}
            for t in range(2):
                b1, b2 = (pltpu.bitcast(w13_32[4 * k + 2 * u + t], BF16) for u in range(2))
                _strassen(normed,
                          b1[:DH], b2[:DH], b1[DH:], b2[DH:], res[t].__setitem__)
            ops = _strassen_lhs(*(_silu(res[0][n]) * res[1][n] for n in range(4)))
            for i in (1, 3, 6, 0, 2, 4, 5):
                act_slot(k, i)[...] = ops[i]
            return c

        lax.fori_loop(0, NF // 2, up, 0, unroll=UNROLL_UP)

        def down(j, c):
            def emit(n, y):
                cols = pl.ds(pl.multiple_of((2 * j + n % 2) * LANE, LANE), LANE)
                idx = (pl.ds(blk * (FB // SEG), FB // SEG), pl.ds(n // 2 * HG, HG), cols)
                xb3[idx] = (xf3[idx] + (mod[5, 0:1, cols] * y).reshape(FB // SEG, HG, LANE)).astype(BF16)

            _strassen(lambda i: jnp.concatenate([act_slot(k, i)[...] for k in range(NF // 2)], axis=1),
                      *(row_tiles((2 * j + u) * F, NF, par) for par in range(2) for u in range(2)), emit)
            out_copy(blk, j).start()
            return c

        lax.fori_loop(0, ND // 2, down, 0)
        return carry

    lax.fori_loop(0, S // FB, ffn, 0)
    for blk in range(S // FB):
        for j in range(ND // 2):
            out_copy(blk, j).wait()


@functools.partial(jax.jit, static_argnames=("A_seg_len",))
def pallas_adaLN_cond__memory_aug_recurrent_mem_tr__glu_gated_swiglu__prompt_kernel(
    A_x, A_mem0, A_Wq, A_Wk, A_Wv, A_Wo, A_seg_len, B_x, B_w1, B_w3, B_w2, c, w_mod,
):
    del B_x
    B, S, D = A_x.shape
    _, H, Dh = A_Wq.shape
    M = A_mem0.shape[1]
    F = B_w1.shape[1]
    SEG = int(A_seg_len)
    assert (B, S, D, H, Dh, M, SEG) == (1, 2048, 1024, 32, LANE, 8, 32) and F % 512 == 0
    P = S // SEG * M
    R = 576
    FB = 1024

    hbm = pl.BlockSpec(memory_space=pl.ANY)
    vmem = pl.BlockSpec(memory_space=pltpu.VMEM)
    out = pl.pallas_call(
        functools.partial(_kernel, S=S, D=D, H=H, F=F, M=M, SEG=SEG, FB=FB),
        out_shape=jax.ShapeDtypeStruct((S, D), A_x.dtype),
        in_specs=[hbm, vmem, hbm, hbm, hbm, hbm, hbm, hbm, hbm, vmem, hbm],
        out_specs=hbm,
        scratch_shapes=[
            pltpu.VMEM((3 * H * (D // 2 + 2), LANE), U32),
            pltpu.VMEM((D * H // 8, 8, LANE), U32),
            pltpu.VMEM((2 * F // LANE, D // 2, LANE), U32),
            pltpu.VMEM((3 * H + 7 * D // (2 * LANE) + 1, R, LANE), F32),
            pltpu.VMEM((H, R, LANE), F32),
            pltpu.VMEM((S, D), BF16),
            pltpu.VMEM((S, D), F32),
            pltpu.VMEM((6, 8, D), F32),
            pltpu.VMEM((7, P // 2, D // 4), U32),
            pltpu.VMEM((7, P // 4, H * Dh // 2), U32),
            pltpu.VMEM((2 * (M + SEG), LANE), F32),
            pltpu.VMEM((H // 2, M + SEG, LANE), U32),
            pltpu.VMEM((SEG, D), F32),
            pltpu.VMEM((8, SEG, LANE), F32),
            pltpu.SemaphoreType.DMA((7 + 6 * H // 16,)),
            pltpu.SemaphoreType.DMA((S // FB * D // (2 * LANE),)),
        ],
        compiler_params=pltpu.CompilerParams(vmem_limit_bytes=126 * 2**20),
        name="adaln_rmt_swiglu",
    )(A_x.reshape(S, D), A_mem0.reshape(M, D), *(w.reshape(D, H // 16, 16, Dh) for w in (A_Wq, A_Wk, A_Wv)),
      A_Wo.reshape(H * Dh // 16, 16, D), B_w1, B_w3, B_w2.reshape(F // 16, 16, D), c, w_mod)
    return out.reshape(B, S, D)
```

```python
import functools

import jax
import jax.numpy as jnp
from jax import lax
import jax.experimental.pallas as pl
import jax.experimental.pallas.tpu as pltpu

F32 = jnp.float32
BF16 = jnp.bfloat16
U32 = jnp.uint32
LANE = 128
EPS = 1e-5
VLAG = 4
AG = 1
OLAG = 0
OCUT = 0
SLAG = 1
AGS = 4
PIN1 = 14
PIN2 = 18
UNROLL_STEP = 2
SPLIT = 2
UNROLL_UP = 2


def _dot(a, b):
    return jnp.dot(a, b, preferred_element_type=F32)


def _norm(x):
    m = jnp.mean(x, axis=-1, keepdims=True)
    d = x - m
    v = jnp.mean(d * d, axis=-1, keepdims=True)
    return d * lax.rsqrt(v + EPS)


def _ada_ln(x, shift, scale1):
    return _norm(x) * scale1 + shift


def _silu(x):
    h = 0.5 * x
    return h + h * jnp.tanh(h)


def _words(x):
    return pltpu.bitcast(x.astype(BF16), U32)


def _strassen_lhs(a11, a12, a21, a22):
    return [_words(a) for a in (a11 + a22, a21 + a22, a11, a22, a11 + a12, a21 - a11, a12 - a22)]


def _strassen(lhs_fn, b11, b12, b21, b22, emit):
    f11, f12, f21, f22 = (b.astype(F32) for b in (b11, b12, b21, b22))

    def prod(i, b):
        return _dot(pltpu.bitcast(lhs_fn(i), BF16), b.astype(BF16))

    m2 = prod(1, b11)
    m4 = prod(3, f21 - f11)
    emit(2, m2 + m4)
    m3 = prod(2, f12 - f22)
    m5 = prod(4, b22)
    emit(1, m3 + m5)
    m1 = prod(0, f11 + f22)
    emit(3, (m1 - m2 + m3) + prod(5, f11 + f12))
    emit(0, (m1 + m4 - m5) + prod(6, f21 + f22))


def _kernel(x_hbm, mem0_hbm, wq_hbm, wk_hbm, wv_hbm, wo_hbm, w1_hbm, w3_hbm, w2_hbm,
            c_hbm, wmod_hbm, out_hbm,
            wqkv, big32, w13_32, ring, oring, xb, xf, mod, hs, ot, fill_ref, prob, acc, early, c_ref, mem0_ref,
            sems, osems,
            *, S, D, H, F, M, SEG, FB):
    NSEG = S // SEG
    XR = SEG - M
    P = S - NSEG * XR
    R = ring.shape[1]
    QOFF = R - P
    OOFF = (-NSEG * XR) % R
    ND = D // LANE
    NF = F // LANE
    HP = H // 2
    HD = H * LANE
    scale = float(LANE) ** -0.5
    big, w13 = big32.bitcast(BF16), w13_32.bitcast(BF16)
    DH = D // 2
    PG = 8
    NA = HP // PG
    NSLOT = big32.shape[0] // DH
    WP = DH + 2
    WO = ND * HD

    def slab(row0, rows):
        return pltpu.bitcast(big32[pl.ds(row0 // 16, rows // 16)].reshape(rows // 2, LANE), BF16)

    def slab_copies(src, tiles, dst_fn, sem):
        return [pltpu.make_async_copy(src.at[..., pl.ds(j * LANE, LANE)], dst_fn(j), sem) for j in tiles]

    def half_tiles(c):
        return [v * ND + c * ND // 2 + j for v in range(2) for j in range(ND // 2)]

    cp_x0 = pltpu.make_async_copy(x_hbm.at[pl.ds(0, P)], xb.at[pl.ds(0, P)], sems.at[0])
    cp_x1 = pltpu.make_async_copy(x_hbm.at[pl.ds(P, S - P)], xb.at[pl.ds(P, S - P)], sems.at[1])
    mod_tiles = [half_tiles(0), half_tiles(1), list(range(2 * ND, 6 * ND))]
    cp_mod = [slab_copies(wmod_hbm, t, lambda j: w13.at[j], sems.at[2 + i])
              for i, t in enumerate(mod_tiles)]
    cp_w = [pltpu.make_async_copy(w.at[pl.ds(c * DH, DH), a],
                                  big.at[pl.ds(((2 * t + c) * NA + a) % NSLOT * DH, DH)],
                                  sems.at[7 + (2 * t + c) * NA + a])
            for t, w in enumerate((wq_hbm, wk_hbm, wv_hbm)) for c in range(2) for a in range(NA)]
    cp_o = slab_copies(wo_hbm, range(ND), lambda j: big.at[pl.ds((WO + j * HD) // 16, HD // 16)], sems.at[5])
    cp_ffn = (slab_copies(w1_hbm, range(NF), lambda j: w13.at[2 * j], sems.at[6])
              + slab_copies(w3_hbm, range(NF), lambda j: w13.at[2 * j + 1], sems.at[6])
              + slab_copies(w2_hbm, range(ND), lambda j: big.at[pl.ds(j * F // 16, F // 16)], sems.at[6]))

    def start(cps):
        for cp in cps:
            cp.start()

    def wait(cps):
        for cp in cps:
            cp.wait()

    cp_c = pltpu.make_async_copy(c_hbm, c_ref, sems.at[7 + len(cp_w)])
    cp_mem = pltpu.make_async_copy(mem0_hbm, mem0_ref, sems.at[8 + len(cp_w)])
    cp_c.start()
    start(cp_mod[0])
    cp_x0.start()
    cp_w[0].start()
    cp_mem.start()
    cp_c.wait()

    cc = jnp.broadcast_to(c_ref[...].astype(F32), (16, D))
    sc = _silu(cc).astype(BF16)

    def mod_part(i):
        wait(cp_mod[i])
        for j in mod_tiles[i]:
            r = _dot(sc, pltpu.bitcast(w13_32[j], BF16))[0:8]
            if j // ND in (1, 4):
                r = r + 1.0
            mod[j // ND, :, pl.ds((j % ND) * LANE, LANE)] = r

    def modv(i):
        return mod[i, 0:1, :]

    G = 2 * (M + SEG)
    ri = lax.broadcasted_iota(jnp.int32, (G, LANE), 0)
    ci = lax.broadcasted_iota(jnp.int32, (G, LANE), 1)

    def head_pos(i):
        head = jnp.where(i < 2 * M, i // M, (i - 2 * M) // SEG)
        pos = jnp.where(i < 2 * M, i % M, M + (i - 2 * M) % SEG)
        return head, pos

    rh, rp = head_pos(ri)
    ch, cp_ = head_pos(ci)
    visible = (rp < M) | (rp >= cp_)
    fill_ref[...] = jnp.where(rh == ch, jnp.where(visible, 0.0, -1e9), -jnp.inf).astype(F32)

    LB = 128
    PH = P // 2
    DQ = D // 4

    def norm_half(c):
        cols = slice(c * DH, (c + 1) * DH)

        def norm0(k, carry):
            halves = []
            for o in (0, PH):
                rows = pl.ds(pl.multiple_of(o + k * LB, LB), LB)
                xv = xb[rows, :].astype(F32)
                xf[rows, cols] = xv[:, cols]
                halves.append(_norm(xv)[:, cols] * mod[1, 0:1, cols] + mod[0, 0:1, cols])
            top, bot = halves
            ops = _strassen_lhs(top[:, :DQ], top[:, DQ:], bot[:, :DQ], bot[:, DQ:])
            for i in range(7):
                hs[i, pl.ds(pl.multiple_of(c * (PH // 2) + k * (LB // 2), LB // 2), LB // 2), :] = ops[i]
            return carry

        lax.fori_loop(0, PH // LB, norm0, 0)

    def arrivals(it):
        if it == 0:
            cp_w[0].wait()
            start(cp_w[2:3] + cp_mod[1] + cp_w[3:4])
        else:
            wait(cp_w[it + (it > 1):it + 2])
        if it == 1:
            start(cp_w[4:6])
        if it == NA:
            start(cp_w[6:NSLOT])
            mod_part(1)
            norm_half(1)
        if it == 4:
            start(cp_w[NSLOT:] + [cp_x1] + cp_mod[2])
        if it == NSLOT - 1:
            wait(cp_w[it + 2:])
            start(cp_o)

    def head_rows(it):
        chunk, a = it // NA, it % NA
        base = (chunk // 2 * H + 2 * PG * a) * WP + chunk % 2 * (DH // 2)
        return wqkv.at[pl.ds(pl.multiple_of(base, 8), (2 * PG + 2) * WP)]

    def retile(it, r0, r1):
        src = big32.at[pl.ds(it % NSLOT * DH, DH)]
        dst = head_rows(it)
        for r in range(r0, r1):
            even, odd = src[2 * r], src[2 * r + 1]
            dst[pl.ds(r, PG, stride=2 * WP), :] = (even & jnp.uint32(0xFFFF)) | (odd << 16)
            dst[pl.ds(WP + r, PG, stride=2 * WP), :] = (even >> 16) | (odd & jnp.uint32(0xFFFF0000))

    def project(it, carry):
        for ev in range(NSLOT):
            pl.when(it == ev)(functools.partial(arrivals, ev))
        pl.when(it < 2)(lambda: retile(it, 0, DH // 2))
        half = it // NA % 2
        hrows = pl.ds(pl.multiple_of(half * (PH // 2), PH // 2), PH // 2)
        nxt = jnp.where(it == 0, 0, jnp.minimum(it + 1, 6 * NA - 1))
        for b in range(PG):
            n = it // (2 * NA) * H + 2 * (PG * (it % NA) + b)
            lo, hi = (pltpu.bitcast(head_rows(it)[pl.ds((2 * b + i) * WP, DH // 2), :], BF16)
                      for i in range(2))

            def emit(i, r, n=n):
                dst = ring.at[n + i % 2, pl.ds(QOFF + i // 2 * PH, PH)]
                dst[...] = r + jnp.where(half == 1, dst[...], 0.0)

            _strassen(lambda i: hs[i, hrows, :], lo[:DQ], hi[:DQ], lo[DQ:], hi[DQ:], emit)
            retile(nxt, b * (DH // 2) // PG, (b + 1) * (DH // 2) // PG)
        return carry

    mod_part(0)
    cp_x0.wait()
    norm_half(0)
    cp_w[1].start()
    lax.fori_loop(0, 6 * NA, project, 0)
    mod_part(2)
    start(cp_ffn)

    HG = SEG // 2
    xf3, xb3 = xf.reshape(NSEG, SEG, D), xb.reshape(NSEG, SEG, D)

    def ffn_norm(grp):
        hn = _ada_ln(xf[pl.ds(pl.multiple_of(grp * SEG, SEG), SEG), :], modv(3), modv(4))
        ops = _strassen_lhs(hn[:HG, :DH], hn[:HG, DH:], hn[HG:, :DH], hn[HG:, DH:])
        for i in range(7):
            for t in range(ND // 2):
                ring[3 * H + i * (ND // 2) + t, pl.ds(pl.multiple_of(grp * (HG // 2), HG // 2), HG // 2), :] = (
                    pltpu.bitcast(ops[i][:, t * LANE:(t + 1) * LANE], F32))

    lhs = ring.at[3 * H + 7 * (ND // 2)]

    def widen(grp):
        rows = pl.ds(pl.multiple_of(grp * SEG, SEG), SEG)
        xf[rows, :] = xb[rows, :].astype(F32)

    def next_rows(r0):
        hn = _ada_ln(xf[pl.ds(r0, XR), :], modv(0), modv(1))
        for t in range(ND):
            lhs[pl.ds(t * SEG + M, XR), :] = hn[:, t * LANE:(t + 1) * LANE]

    cp_mem.wait()
    for t in range(ND):
        lhs[pl.ds(t * SEG, M), :] = mem0_ref[:, pl.ds(t * LANE, LANE)].astype(F32)
    cp_x1.wait()
    widen(P // SEG)
    next_rows(P)
    wait(cp_o)

    def step(s, carry):
        q_wr = pl.multiple_of(lax.rem(s * XR, R), 8)
        q_rd = pl.multiple_of(lax.rem(s * SEG + QOFF, R), 8)
        o_wr = pl.multiple_of(lax.rem(s * SEG + OOFF, R), 8)
        o_rd = pl.multiple_of(lax.rem(s * XR + OOFF, R), 8)
        h = jnp.concatenate([lhs[pl.ds(t * SEG, SEG), :] for t in range(ND)], axis=1).astype(BF16)
        tail_rows = pl.ds(pl.multiple_of(jnp.maximum(s - NSEG * XR // SEG, 0) * (HG // 2), HG // 2), HG // 2)
        pad = jnp.zeros((LANE - G, LANE), BF16)

        for u in range(4 * SPLIT):
            n = u // 2 % 2 * H + u // 4 * 2 + u % 2
            early[u] = _dot(h[:, :DH], pltpu.bitcast(wqkv[pl.ds(n * WP, DH // 2), :], BF16))

        def head_pair(t, g):
            n = t * H + 2 * g
            mem_rows = []
            for i in range(2):
                if t < 2 and g < SPLIT:
                    r = (_dot(h[:, DH:], pltpu.bitcast(wqkv[pl.ds((n + i) * WP + DH // 2, DH // 2), :], BF16))
                         + early[4 * g + 2 * t + i])
                else:
                    r = _dot(h, pltpu.bitcast(wqkv[pl.ds((n + i) * WP, DH), :], BF16))
                ring[n + i, pl.ds(q_wr, XR), :] = r[M:]
                mem_rows.append(r[:M])
            return jnp.concatenate(
                mem_rows + [ring[n + i, pl.ds(q_rd, SEG), :] for i in range(2)],
                axis=0).astype(BF16)

        def scores(q, k):
            sc_ = lax.dot_general(q, jnp.concatenate([k, pad], axis=0), (((1,), (1,)), ((), ())),
                                  preferred_element_type=F32)
            fill = fill_ref[...]
            sc_ = jnp.where(fill == 0.0, sc_ * scale, fill)
            e = jnp.exp(sc_ - jnp.max(sc_, axis=-1, keepdims=True))
            return (e * (1.0 / jnp.sum(e, axis=-1, keepdims=True))).astype(BF16)

        def attend(g, p, v):
            o = _dot(p, jnp.concatenate([v, pad], axis=0))
            ops = _strassen_lhs(*(o[2 * M + i * SEG + r:2 * M + i * SEG + r + HG]
                                  for r in (0, HG) for i in range(2)))
            for i in range(7):
                ot[i, tail_rows, pl.ds(g * LANE, LANE)] = ops[i]
            for i in range(2):
                oring[2 * g + i, pl.ds(o_wr, SEG), :] = o[2 * M + i * SEG:2 * M + (i + 1) * SEG]
            return functools.cache(lambda: [jnp.concatenate(
                [o[i * M:(i + 1) * M], oring[2 * g + i, pl.ds(o_rd, XR), :]],
                axis=0).astype(BF16) for i in range(2)])

        heads = {}

        def oproj(g0, g1, j0=0, j1=ND):
            a = jnp.concatenate([r for g in range(g0, g1) for r in heads[g]()], axis=1)
            for j in range(j0, j1):
                cols = pl.ds(j * LANE, LANE)
                r = _dot(a, slab(WO + j * HD + g0 * 2 * LANE, (g1 - g0) * 2 * LANE))
                if g0 > 0:
                    r = r + acc[:, cols]
                if g1 < HP:
                    acc[:, cols] = r
                else:
                    lhs[pl.ds(j * SEG, M), :] = r[:M]
                    xf[rows, cols] = xf[rows, cols] + mod[2, 0:1, cols] * r[M:]

        rows = pl.ds(pl.multiple_of(s * XR, 8), XR)
        qk, val = {}, {}
        LAG = VLAG
        for i in range(2 * HP + LAG):
            if i == PIN1:
                widen(jnp.minimum(P // SEG + 1 + s, NSEG - 1))
                next_rows(pl.multiple_of(jnp.minimum(P + (s + 1) * XR, S - XR), 8))
            if i == PIN2:
                ffn_norm(jnp.maximum(s * XR // SEG - 1, 0))
            if i < HP:
                qk[i] = head_pair(0, i), head_pair(1, i)
            elif i < 2 * HP:
                val[i - HP] = head_pair(2, i - HP)
            else:
                oproj(0, HP // 2, i - 2 * HP, i - 2 * HP + 1)
            i0 = i - SLAG
            if i0 % AGS == 0 and 0 < i0 <= HP:
                for g, q, k in [(g, *qk[g]) for g in range(i0 - AGS, i0)]:
                    prob[g] = pltpu.bitcast(scores(q, k), U32)
            g1 = i - HP - LAG + 1
            if g1 % AG == 0 and g1 > 0:
                for g, v in [(g, val[g]) for g in range(g1 - AG, g1)]:
                    heads[g] = attend(g, pltpu.bitcast(prob[g], BF16), v)
                for g in range(max(g1 - AG - OLAG, 0), g1 - OLAG):
                    heads[g]()
        oproj(0, HP // 2, LAG, ND)
        if OCUT:
            oproj(HP // 2, OCUT)
        oproj(OCUT or HP // 2, HP)
        return carry

    lax.fori_loop(0, NSEG, step, 0, unroll=UNROLL_STEP)

    MH = FB // 2

    def row_tiles(row0, n, par):
        return jnp.concatenate([slab(row0 + (2 * k + par) * LANE, LANE) for k in range(n // 2)], axis=0)

    def otail(j, carry):
        def emit(n, y):
            cols = pl.ds(pl.multiple_of((2 * j + n % 2) * LANE, LANE), LANE)
            idx = (pl.ds(NSEG * XR // SEG, P // SEG), pl.ds(n // 2 * HG, HG), cols)
            xf3[idx] = xf3[idx] + (mod[2, 0:1, cols] * y).reshape(P // SEG, HG, LANE)

        _strassen(lambda i: ot[i],
                  *(row_tiles(WO + (2 * j + u) * HD, H, par) for par in range(2) for u in range(2)), emit)
        return carry

    lax.fori_loop(0, ND // 2, otail, 0)
    G0 = (NSEG - 1) * XR // SEG - 1

    def norm_tail(i, carry):
        for u in range(6):
            ffn_norm(G0 + 6 * i + u)
        return carry

    lax.fori_loop(0, (NSEG - G0) // 6, norm_tail, 0)

    wait(cp_ffn)

    def act_slot(k, i):
        return wqkv.at[pl.ds(pl.multiple_of((7 * k + i) * (MH // 2), MH // 2), MH // 2)]

    def out_copy(blk, j):
        idx = (pl.ds(pl.multiple_of(blk * FB, FB), FB), pl.ds(pl.multiple_of(j * 2 * LANE, 2 * LANE), 2 * LANE))
        return pltpu.make_async_copy(xb.at[idx], out_hbm.at[idx], osems.at[blk * (ND // 2) + j])

    def ffn(blk, carry):
        def normed(i):
            rows = pl.ds(pl.multiple_of(blk * (MH // 2), MH // 2), MH // 2)
            return jnp.concatenate([ring[3 * H + i * (ND // 2) + t, rows, :] for t in range(ND // 2)], axis=1)

        def up(k, c):
            res = {}, {}
            for t in range(2):
                b1, b2 = (pltpu.bitcast(w13_32[4 * k + 2 * u + t], BF16) for u in range(2))
                _strassen(normed,
                          b1[:DH], b2[:DH], b1[DH:], b2[DH:], res[t].setdefault)
            ops = _strassen_lhs(*(_silu(res[0][n]) * res[1][n] for n in range(4)))
            for i in (1, 3, 6, 0, 2, 4, 5):
                act_slot(k, i)[...] = ops[i]
            return c

        lax.fori_loop(0, NF // 2, up, 0, unroll=UNROLL_UP)

        def down(j, c):
            def emit(n, y):
                cols = pl.ds(pl.multiple_of((2 * j + n % 2) * LANE, LANE), LANE)
                idx = (pl.ds(blk * (FB // SEG), FB // SEG), pl.ds(n // 2 * HG, HG), cols)
                xb3[idx] = (xf3[idx] + (mod[5, 0:1, cols] * y).reshape(FB // SEG, HG, LANE)).astype(BF16)

            _strassen(lambda i: jnp.concatenate([act_slot(k, i)[...] for k in range(NF // 2)], axis=1),
                      *(row_tiles((2 * j + u) * F, NF, par) for par in range(2) for u in range(2)), emit)
            out_copy(blk, j).start()
            return c

        lax.fori_loop(0, ND // 2, down, 0)
        return carry

    lax.fori_loop(0, S // FB, ffn, 0)
    for blk in range(S // FB):
        for j in range(ND // 2):
            out_copy(blk, j).wait()


@functools.partial(jax.jit, static_argnames=("A_seg_len",))
def pallas_adaLN_cond__memory_aug_recurrent_mem_tr__glu_gated_swiglu__prompt_kernel(
    A_x, A_mem0, A_Wq, A_Wk, A_Wv, A_Wo, A_seg_len, B_x, B_w1, B_w3, B_w2, c, w_mod,
):
    del B_x
    B, S, D = A_x.shape
    _, H, Dh = A_Wq.shape
    M = A_mem0.shape[1]
    F = B_w1.shape[1]
    SEG = int(A_seg_len)
    assert (B, S, D, H, Dh, M, SEG) == (1, 2048, 1024, 32, LANE, 8, 32) and F % 512 == 0
    P = S // SEG * M
    R = 576
    FB = 1024

    hbm = pl.BlockSpec(memory_space=pl.ANY)
    out = pl.pallas_call(
        functools.partial(_kernel, S=S, D=D, H=H, F=F, M=M, SEG=SEG, FB=FB),
        out_shape=jax.ShapeDtypeStruct((S, D), A_x.dtype),
        in_specs=[hbm] * 11,
        out_specs=hbm,
        scratch_shapes=[
            pltpu.VMEM(((3 * H + 4) * (D // 2 + 2), LANE), U32),
            pltpu.VMEM((D * H // 8, 8, LANE), U32),
            pltpu.VMEM((2 * F // LANE, D // 2, LANE), U32),
            pltpu.VMEM((3 * H + 7 * D // (2 * LANE) + 1, R, LANE), F32),
            pltpu.VMEM((H, R, LANE), F32),
            pltpu.VMEM((S, D), BF16),
            pltpu.VMEM((S, D), F32),
            pltpu.VMEM((6, 8, D), F32),
            pltpu.VMEM((7, P // 2, D // 4), U32),
            pltpu.VMEM((7, P // 4, H * Dh // 2), U32),
            pltpu.VMEM((2 * (M + SEG), LANE), F32),
            pltpu.VMEM((H // 2, M + SEG, LANE), U32),
            pltpu.VMEM((SEG, D), F32),
            pltpu.VMEM((8, SEG, LANE), F32),
            pltpu.VMEM((1, D), c.dtype),
            pltpu.VMEM((M, D), A_mem0.dtype),
            pltpu.SemaphoreType.DMA((9 + 6 * H // 16,)),
            pltpu.SemaphoreType.DMA((S // FB * D // (2 * LANE),)),
        ],
        compiler_params=pltpu.CompilerParams(vmem_limit_bytes=126 * 2**20),
        name="adaln_rmt_swiglu",
    )(A_x.reshape(S, D), A_mem0.reshape(M, D), *(w.reshape(D, H // 16, 16, Dh) for w in (A_Wq, A_Wk, A_Wv)),
      A_Wo.reshape(H * Dh // 16, 16, D), B_w1, B_w3, B_w2.reshape(F // 16, 16, D), c, w_mod)
    return out.reshape(B, S, D)
```

```python
import functools

import jax
import jax.numpy as jnp
from jax import lax
import jax.experimental.pallas as pl
import jax.experimental.pallas.tpu as pltpu

F32 = jnp.float32
BF16 = jnp.bfloat16
U32 = jnp.uint32
LANE = 128
EPS = 1e-5
VLAG = 2
AG = 1
OLAG = 2
PADW = 1024
WPAD = 4
OCUT = 0
SLAG = 1
AGS = 4
PIN1 = 7
PIN2 = 24
UNROLL_STEP = 2
SPLIT = 2
UNROLL_UP = 2


def _dot(a, b):
    return jnp.dot(a, b, preferred_element_type=F32)


def _norm(x):
    m = jnp.mean(x, axis=-1, keepdims=True)
    d = x - m
    v = jnp.mean(d * d, axis=-1, keepdims=True)
    return d * lax.rsqrt(v + EPS)


def _ada_ln(x, shift, scale1):
    return _norm(x) * scale1 + shift


def _silu(x):
    h = 0.5 * x
    return h + h * jnp.tanh(h)


def _words(x):
    return pltpu.bitcast(x.astype(BF16), U32)


def _strassen_lhs(a11, a12, a21, a22):
    return [_words(a) for a in (a11 + a22, a21 + a22, a11, a22, a11 + a12, a21 - a11, a12 - a22)]


def _strassen(lhs_fn, b11, b12, b21, b22, emit):
    f11, f12, f21, f22 = (b.astype(F32) for b in (b11, b12, b21, b22))

    def prod(i, b):
        return _dot(pltpu.bitcast(lhs_fn(i), BF16), b.astype(BF16))

    m2 = prod(1, b11)
    m4 = prod(3, f21 - f11)
    emit(2, m2 + m4)
    m3 = prod(2, f12 - f22)
    m5 = prod(4, b22)
    emit(1, m3 + m5)
    m1 = prod(0, f11 + f22)
    emit(3, (m1 - m2 + m3) + prod(5, f11 + f12))
    emit(0, (m1 + m4 - m5) + prod(6, f21 + f22))


def _kernel(x_hbm, mem0_hbm, wq_hbm, wk_hbm, wv_hbm, wo_hbm, w1_hbm, w3_hbm, w2_hbm,
            c_hbm, wmod_hbm, out_hbm,
            wqkv, big32, w13_32, ring, oring, xb, xf, mod, hs, ot, fill_ref, prob, acc, early, c_ref, mem0_ref,
            sems, osems,
            *, S, D, H, F, M, SEG, FB):
    NSEG = S // SEG
    XR = SEG - M
    P = S - NSEG * XR
    R = ring.shape[0]
    QOFF = R - P
    OOFF = (-NSEG * XR) % R
    ND = D // LANE
    NF = F // LANE
    HP = H // 2
    HD = H * LANE
    scale = float(LANE) ** -0.5
    big, w13 = big32.bitcast(BF16), w13_32.bitcast(BF16)
    DH = D // 2
    PG = 8
    NA = HP // PG
    NSLOT = big32.shape[0] // DH
    WP = DH + WPAD
    WO = ND * HD

    def tile(n, width=1):
        return pl.ds(n * LANE if isinstance(n, int) else pl.multiple_of(n * LANE, LANE), width * LANE)

    def head_slab(n):
        return (n // (2 * PG) * 2 * PG + n % 2 * PG + n % (2 * PG) // 2) * WP

    def slab(row0, rows):
        return pltpu.bitcast(big32[pl.ds(row0 // 16, rows // 16)].reshape(rows // 2, LANE), BF16)

    def slab_copies(src, tiles, dst_fn, sem):
        return [pltpu.make_async_copy(src.at[..., pl.ds(j * LANE, LANE)], dst_fn(j), sem) for j in tiles]

    def half_tiles(c):
        return [v * ND + c * ND // 2 + j for v in range(2) for j in range(ND // 2)]

    cp_x0 = pltpu.make_async_copy(x_hbm.at[pl.ds(0, P)], xb.at[pl.ds(0, P)], sems.at[0])
    cp_x1 = pltpu.make_async_copy(x_hbm.at[pl.ds(P, S - P)], xb.at[pl.ds(P, S - P)], sems.at[1])
    mod_tiles = [half_tiles(0), half_tiles(1), list(range(2 * ND, 6 * ND))]
    cp_mod = [slab_copies(wmod_hbm, t, lambda j: w13.at[j], sems.at[2 + i])
              for i, t in enumerate(mod_tiles)]
    cp_w = [pltpu.make_async_copy(w.at[pl.ds(c * DH, DH), a],
                                  big.at[pl.ds(((2 * t + c) * NA + a) % NSLOT * DH, DH)],
                                  sems.at[7 + (2 * t + c) * NA + a])
            for t, w in enumerate((wq_hbm, wk_hbm, wv_hbm)) for c in range(2) for a in range(NA)]
    cp_o = slab_copies(wo_hbm, range(ND), lambda j: big.at[pl.ds((WO + j * HD) // 16, HD // 16)], sems.at[5])
    cp_ffn = (slab_copies(w1_hbm, range(NF), lambda j: w13.at[2 * j], sems.at[6])
              + slab_copies(w3_hbm, range(NF), lambda j: w13.at[2 * j + 1], sems.at[6])
              + slab_copies(w2_hbm, range(ND), lambda j: big.at[pl.ds(j * F // 16, F // 16)], sems.at[6]))

    def start(cps):
        for cp in cps:
            cp.start()

    def wait(cps):
        for cp in cps:
            cp.wait()

    cp_c = pltpu.make_async_copy(c_hbm, c_ref, sems.at[7 + len(cp_w)])
    cp_mem = pltpu.make_async_copy(mem0_hbm, mem0_ref, sems.at[8 + len(cp_w)])
    cp_c.start()
    start(cp_mod[0])
    cp_x0.start()
    cp_w[0].start()
    cp_mem.start()
    cp_c.wait()

    cc = jnp.broadcast_to(c_ref[...].astype(F32), (16, D))
    sc = _silu(cc).astype(BF16)

    def mod_part(i):
        wait(cp_mod[i])
        for j in mod_tiles[i]:
            r = _dot(sc, pltpu.bitcast(w13_32[j], BF16))[0:8]
            if j // ND in (1, 4):
                r = r + 1.0
            mod[j // ND, :, pl.ds((j % ND) * LANE, LANE)] = r

    def modv(i):
        return mod[i, 0:1, :]

    G = 2 * (M + SEG)
    ri = lax.broadcasted_iota(jnp.int32, (G, LANE), 0)
    ci = lax.broadcasted_iota(jnp.int32, (G, LANE), 1)

    def head_pos(i):
        head = jnp.where(i < 2 * M, i // M, (i - 2 * M) // SEG)
        pos = jnp.where(i < 2 * M, i % M, M + (i - 2 * M) % SEG)
        return head, pos

    rh, rp = head_pos(ri)
    ch, cp_ = head_pos(ci)
    visible = (rp < M) | (rp >= cp_)
    fill_ref[0:G, :] = jnp.where(rh == ch, jnp.where(visible, 0.0, -1e9), -jnp.inf).astype(F32)

    LB = 128
    PH = P // 2
    DQ = D // 4

    def norm_half(c):
        cols = slice(c * DH, (c + 1) * DH)

        def norm0(k, carry):
            halves = []
            for o in (0, PH):
                rows = pl.ds(pl.multiple_of(o + k * LB, LB), LB)
                xv = xb[rows, :].astype(F32)
                xf[rows, cols] = xv[:, cols]
                halves.append(_norm(xv)[:, cols] * mod[1, 0:1, cols] + mod[0, 0:1, cols])
            top, bot = halves
            ops = _strassen_lhs(top[:, :DQ], top[:, DQ:], bot[:, :DQ], bot[:, DQ:])
            for i in range(7):
                hs[i, pl.ds(pl.multiple_of(c * (PH // 2) + k * (LB // 2), LB // 2), LB // 2), :] = ops[i]
            return carry

        lax.fori_loop(0, PH // LB, norm0, 0)

    def arrivals(it):
        if it == 0:
            cp_w[0].wait()
            start(cp_w[2:3] + cp_mod[1] + cp_w[3:4])
        else:
            wait(cp_w[it + (it > 1):it + 2])
        if it == 1:
            start(cp_w[4:6])
        if it == NA:
            start(cp_w[6:NSLOT])
            mod_part(1)
            norm_half(1)
        if it == 4:
            start(cp_w[NSLOT:] + [cp_x1] + cp_mod[2])
        if it == NSLOT - 1:
            wait(cp_w[it + 2:])
            start(cp_o)

    def head_rows(it):
        chunk, a = it // NA, it % NA
        base = (chunk // 2 * H + 2 * PG * a) * WP + chunk % 2 * (DH // 2)
        return wqkv.at[pl.ds(pl.multiple_of(base, 32), (2 * PG + 1) * WP)]

    def retile(it, r0, r1):
        src = big32.at[pl.ds(it % NSLOT * DH, DH)]
        dst = head_rows(it)
        for r in range(r0, r1):
            even, odd = src[2 * r], src[2 * r + 1]
            dst[pl.ds(r, PG, stride=WP), :] = (even & jnp.uint32(0xFFFF)) | (odd << 16)
            dst[pl.ds(PG * WP + r, PG, stride=WP), :] = (even >> 16) | (odd & jnp.uint32(0xFFFF0000))

    def project(it, carry):
        for ev in range(NSLOT):
            pl.when(it == ev)(functools.partial(arrivals, ev))
        pl.when(it < 2)(lambda: retile(it, 0, DH // 2))
        half = it // NA % 2
        hrows = pl.ds(pl.multiple_of(half * (PH // 2), PH // 2), PH // 2)
        nxt = jnp.where(it == 0, 0, jnp.minimum(it + 1, 6 * NA - 1))
        dst = ring.at[:, tile(it // (2 * NA) * H + 2 * PG * (it % NA), 2 * PG)]
        for b in range(PG):
            lo, hi = (pltpu.bitcast(head_rows(it)[pl.ds((i * PG + b) * WP, DH // 2), :], BF16)
                      for i in range(2))

            def emit(i, r, b=b):
                idx = pl.ds(QOFF + i // 2 * PH, PH), tile(2 * b + i % 2)
                dst[idx] = r + jnp.where(half == 1, dst[idx], 0.0)

            _strassen(lambda i: hs[i, hrows, :], lo[:DQ], hi[:DQ], lo[DQ:], hi[DQ:], emit)
            retile(nxt, b * (DH // 2) // PG, (b + 1) * (DH // 2) // PG)
        return carry

    mod_part(0)
    cp_x0.wait()
    norm_half(0)
    cp_w[1].start()
    lax.fori_loop(0, 6 * NA, project, 0)
    mod_part(2)
    start(cp_ffn)

    HG = SEG // 2
    xf3, xb3 = xf.reshape(NSEG, SEG, D), xb.reshape(NSEG, SEG, D)

    def ffn_norm(grp):
        hn = _ada_ln(xf[pl.ds(pl.multiple_of(grp * SEG, SEG), SEG), :], modv(3), modv(4))
        ops = _strassen_lhs(hn[:HG, :DH], hn[:HG, DH:], hn[HG:, :DH], hn[HG:, DH:])
        for i in range(7):
            ring[pl.ds(pl.multiple_of(grp * (HG // 2), HG // 2), HG // 2),
                 tile(3 * H + i * ND // 2, ND // 2)] = pltpu.bitcast(ops[i], F32)

    L0 = S // 4

    def widen(grp):
        rows = pl.ds(pl.multiple_of(grp * SEG, SEG), SEG)
        xf[rows, :] = xb[rows, :].astype(F32)

    def next_rows(r0):
        ring[pl.ds(L0 + M, XR), tile(3 * H, ND)] = _ada_ln(xf[pl.ds(r0, XR), :], modv(0), modv(1))

    cp_mem.wait()
    ring[pl.ds(L0, M), tile(3 * H, ND)] = mem0_ref[...].astype(F32)
    cp_x1.wait()
    widen(P // SEG)
    next_rows(P)
    wait(cp_o)

    def step(s, carry):
        q_wr = pl.multiple_of(lax.rem(s * XR, R), 8)
        q_rd = pl.multiple_of(lax.rem(s * SEG + QOFF, R), SEG)
        o_wr = pl.multiple_of(lax.rem(s * SEG + OOFF, R), SEG)
        o_rd = pl.multiple_of(lax.rem(s * XR + OOFF, R), 8)
        h = ring[pl.ds(L0, SEG), tile(3 * H, ND)].astype(BF16)
        tail_rows = pl.ds(pl.multiple_of(jnp.maximum(s - NSEG * XR // SEG, 0) * (HG // 2), HG // 2), HG // 2)
        pad = jnp.zeros((LANE - G, LANE), BF16)

        for u in range(4 * SPLIT):
            n = u // 2 % 2 * H + u // 4 * 2 + u % 2
            early[u] = _dot(h[:, :DH], pltpu.bitcast(wqkv[pl.ds(head_slab(n), DH // 2), :], BF16))

        def head_pair(t, g):
            n = t * H + 2 * g
            mem_rows = []
            for i in range(2):
                if t < 2 and g < SPLIT:
                    r = (_dot(h[:, DH:], pltpu.bitcast(wqkv[pl.ds(head_slab(n + i) + DH // 2, DH // 2), :], BF16))
                         + early[4 * g + 2 * t + i])
                else:
                    r = _dot(h, pltpu.bitcast(wqkv[pl.ds(head_slab(n + i), DH), :], BF16))
                ring[pl.ds(q_wr, XR), tile(n + i)] = r[M:]
                mem_rows.append(r[:M])
            return jnp.concatenate(
                mem_rows + [ring[pl.ds(q_rd, SEG), tile(n + i)] for i in range(2)],
                axis=0).astype(BF16)

        def scores(q, k):
            sc_ = lax.dot_general(q, jnp.concatenate([k, pad], axis=0), (((1,), (1,)), ((), ())),
                                  preferred_element_type=F32)
            fill = fill_ref[0:G, :]
            sc_ = jnp.where(fill == 0.0, sc_ * scale, fill)
            e = jnp.exp(sc_ - jnp.max(sc_, axis=-1, keepdims=True))
            return (e * (1.0 / jnp.sum(e, axis=-1, keepdims=True))).astype(BF16)

        def attend(g, p, v):
            o = _dot(p, jnp.concatenate([v, pad], axis=0))
            ops = _strassen_lhs(*(o[2 * M + i * SEG + r:2 * M + i * SEG + r + HG]
                                  for r in (0, HG) for i in range(2)))
            for i in range(7):
                ot[i, tail_rows, pl.ds(g * LANE, LANE)] = ops[i]
            for i in range(2):
                oring[pl.ds(o_wr, SEG), tile(2 * g + i)] = o[2 * M + i * SEG:2 * M + (i + 1) * SEG]
            return functools.cache(lambda: [jnp.concatenate(
                [o[i * M:(i + 1) * M], oring[pl.ds(o_rd, XR), tile(2 * g + i)]],
                axis=0).astype(BF16) for i in range(2)])

        heads = {}

        def oproj(g0, g1, j0=0, j1=ND):
            a = jnp.concatenate([r for g in range(g0, g1) for r in heads[g]()], axis=1)
            for j in range(j0, j1):
                cols = pl.ds(j * LANE, LANE)
                r = _dot(a, slab(WO + j * HD + g0 * 2 * LANE, (g1 - g0) * 2 * LANE))
                if g0 > 0:
                    r = r + acc[:, cols]
                if g1 < HP:
                    acc[:, cols] = r
                else:
                    ring[pl.ds(L0, M), tile(3 * H + j)] = r[:M]
                    xf[rows, cols] = xf[rows, cols] + mod[2, 0:1, cols] * r[M:]

        rows = pl.ds(pl.multiple_of(s * XR, 8), XR)
        qk, val = {}, {}
        LAG = VLAG
        for i in range(2 * HP + LAG):
            if i == PIN1:
                widen(jnp.minimum(P // SEG + 1 + s, NSEG - 1))
                next_rows(pl.multiple_of(jnp.minimum(P + (s + 1) * XR, S - XR), 8))
            if i == PIN2:
                ffn_norm(jnp.maximum(s * XR // SEG - 1, 0))
            if i < HP:
                qk[i] = head_pair(0, i), head_pair(1, i)
            elif i < 2 * HP:
                val[i - HP] = head_pair(2, i - HP)
            else:
                oproj(0, HP // 2, i - 2 * HP, i - 2 * HP + 1)
            i0 = i - SLAG
            if i0 % AGS == 0 and 0 < i0 <= HP:
                for g, q, k in [(g, *qk[g]) for g in range(i0 - AGS, i0)]:
                    prob[g] = pltpu.bitcast(scores(q, k), U32)
            g1 = i - HP - LAG + 1
            if g1 % AG == 0 and g1 > 0:
                for g, v in [(g, val[g]) for g in range(g1 - AG, g1)]:
                    heads[g] = attend(g, pltpu.bitcast(prob[g], BF16), v)
                for g in range(max(g1 - AG - OLAG, 0), g1 - OLAG):
                    heads[g]()
        oproj(0, HP // 2, LAG, ND)
        if OCUT:
            oproj(HP // 2, OCUT)
        oproj(OCUT or HP // 2, HP)
        return carry

    lax.fori_loop(0, NSEG, step, 0, unroll=UNROLL_STEP)

    MH = FB // 2

    def row_tiles(row0, n, par):
        return jnp.concatenate([slab(row0 + (2 * k + par) * LANE, LANE) for k in range(n // 2)], axis=0)

    def otail(j, carry):
        def emit(n, y):
            cols = pl.ds(pl.multiple_of((2 * j + n % 2) * LANE, LANE), LANE)
            idx = (pl.ds(NSEG * XR // SEG, P // SEG), pl.ds(n // 2 * HG, HG), cols)
            xf3[idx] = xf3[idx] + (mod[2, 0:1, cols] * y).reshape(P // SEG, HG, LANE)

        _strassen(lambda i: ot[i],
                  *(row_tiles(WO + (2 * j + u) * HD, H, par) for par in range(2) for u in range(2)), emit)
        return carry

    lax.fori_loop(0, ND // 2, otail, 0)
    G0 = (NSEG - 1) * XR // SEG - 1

    def norm_tail(i, carry):
        for u in range(6):
            ffn_norm(G0 + 6 * i + u)
        return carry

    lax.fori_loop(0, (NSEG - G0) // 6, norm_tail, 0)

    wait(cp_ffn)

    def act_slot(k, i):
        return wqkv.at[pl.ds(pl.multiple_of((7 * k + i) * (MH // 2), MH // 2), MH // 2)]

    def out_copy(blk, j):
        idx = (pl.ds(pl.multiple_of(blk * FB, FB), FB), pl.ds(pl.multiple_of(j * 2 * LANE, 2 * LANE), 2 * LANE))
        return pltpu.make_async_copy(xb.at[idx], out_hbm.at[idx], osems.at[blk * (ND // 2) + j])

    def ffn(blk, carry):
        def normed(i):
            rows = pl.ds(pl.multiple_of(blk * (MH // 2), MH // 2), MH // 2)
            return ring[rows, tile(3 * H + i * ND // 2, ND // 2)]

        def up(k, c):
            res = {}, {}
            for t in range(2):
                b1, b2 = (pltpu.bitcast(w13_32[4 * k + 2 * u + t], BF16) for u in range(2))
                _strassen(normed,
                          b1[:DH], b2[:DH], b1[DH:], b2[DH:], res[t].setdefault)
            ops = _strassen_lhs(*(_silu(res[0][n]) * res[1][n] for n in range(4)))
            for i in (1, 3, 6, 0, 2, 4, 5):
                act_slot(k, i)[...] = ops[i]
            return c

        lax.fori_loop(0, NF // 2, up, 0, unroll=UNROLL_UP)

        def down(j, c):
            def emit(n, y):
                cols = pl.ds(pl.multiple_of((2 * j + n % 2) * LANE, LANE), LANE)
                idx = (pl.ds(blk * (FB // SEG), FB // SEG), pl.ds(n // 2 * HG, HG), cols)
                xb3[idx] = (xf3[idx] + (mod[5, 0:1, cols] * y).reshape(FB // SEG, HG, LANE)).astype(BF16)

            _strassen(lambda i: jnp.concatenate([act_slot(k, i)[...] for k in range(NF // 2)], axis=1),
                      *(row_tiles((2 * j + u) * F, NF, par) for par in range(2) for u in range(2)), emit)
            out_copy(blk, j).start()
            return c

        lax.fori_loop(0, ND // 2, down, 0)
        return carry

    lax.fori_loop(0, S // FB, ffn, 0)
    for blk in range(S // FB):
        for j in range(ND // 2):
            out_copy(blk, j).wait()


@functools.partial(jax.jit, static_argnames=("A_seg_len",))
def pallas_adaLN_cond__memory_aug_recurrent_mem_tr__glu_gated_swiglu__prompt_kernel(
    A_x, A_mem0, A_Wq, A_Wk, A_Wv, A_Wo, A_seg_len, B_x, B_w1, B_w3, B_w2, c, w_mod,
):
    del B_x
    B, S, D = A_x.shape
    _, H, Dh = A_Wq.shape
    M = A_mem0.shape[1]
    F = B_w1.shape[1]
    SEG = int(A_seg_len)
    assert (B, S, D, H, Dh, M, SEG) == (1, 2048, 1024, 32, LANE, 8, 32) and F % 512 == 0
    P = S // SEG * M
    R = 576
    FB = 1024

    hbm = pl.BlockSpec(memory_space=pl.ANY)
    out = pl.pallas_call(
        functools.partial(_kernel, S=S, D=D, H=H, F=F, M=M, SEG=SEG, FB=FB),
        out_shape=jax.ShapeDtypeStruct((S, D), A_x.dtype),
        in_specs=[hbm] * 11,
        out_specs=hbm,
        scratch_shapes=[
            pltpu.VMEM((3 * H * (D // 2 + WPAD) + PADW, LANE), U32),
            pltpu.VMEM((D * H // 8, 8, LANE), U32),
            pltpu.VMEM((2 * F // LANE, D // 2, LANE), U32),
            pltpu.VMEM((R, 3 * H * Dh + 7 * D // 2), F32),
            pltpu.VMEM((R, H * Dh), F32),
            pltpu.VMEM((S, D), BF16),
            pltpu.VMEM((S, D), F32),
            pltpu.VMEM((6, 8, D), F32),
            pltpu.VMEM((7, P // 2, D // 4), U32),
            pltpu.VMEM((7, P // 4, H * Dh // 2), U32),
            pltpu.VMEM((3 * SEG, LANE), F32),
            pltpu.VMEM((H // 2, M + SEG, LANE), U32),
            pltpu.VMEM((SEG, D), F32),
            pltpu.VMEM((8, SEG, LANE), F32),
            pltpu.VMEM((1, D), c.dtype),
            pltpu.VMEM((M, D), A_mem0.dtype),
            pltpu.SemaphoreType.DMA((9 + 6 * H // 16,)),
            pltpu.SemaphoreType.DMA((S // FB * D // (2 * LANE),)),
        ],
        compiler_params=pltpu.CompilerParams(vmem_limit_bytes=126 * 2**20),
        name="adaln_rmt_swiglu",
    )(A_x.reshape(S, D), A_mem0.reshape(M, D), *(w.reshape(D, H // 16, 16, Dh) for w in (A_Wq, A_Wk, A_Wv)),
      A_Wo.reshape(H * Dh // 16, 16, D), B_w1, B_w3, B_w2.reshape(F // 16, 16, D), c, w_mod)
    return out.reshape(B, S, D)
```

```python
import functools

import jax
import jax.numpy as jnp
from jax import lax
import jax.experimental.pallas as pl
import jax.experimental.pallas.tpu as pltpu

F32 = jnp.float32
BF16 = jnp.bfloat16
U32 = jnp.uint32
LANE = 128
EPS = 1e-5
SLAB_PAD = 4
SCORE_GROUP = 4
SCORE_LAG = 1
VALUE_LAG = 3
FFN_NORM_AT = 7
NEXT_ROWS_AT = 28


def _dot(a, b):
    return jnp.dot(a, b, preferred_element_type=F32)


def _norm(x):
    m = jnp.mean(x, axis=-1, keepdims=True)
    d = x - m
    v = jnp.mean(d * d, axis=-1, keepdims=True)
    return d * lax.rsqrt(v + EPS)


def _ada_ln(x, shift, scale1):
    return _norm(x) * scale1 + shift


def _silu(x):
    h = 0.5 * x
    return h + h * jnp.tanh(h)


def _words(x):
    return pltpu.bitcast(x.astype(BF16), U32)


def _strassen_lhs(a11, a12, a21, a22):
    return [_words(a) for a in (a11 + a22, a21 + a22, a11, a22, a11 + a12, a21 - a11, a12 - a22)]


def _strassen(lhs_fn, b11, b12, b21, b22, emit):
    f11, f12, f21, f22 = (b.astype(F32) for b in (b11, b12, b21, b22))

    def prod(i, b):
        return _dot(pltpu.bitcast(lhs_fn(i), BF16), b.astype(BF16))

    m2 = prod(1, b11)
    m4 = prod(3, f21 - f11)
    emit(2, m2 + m4)
    m3 = prod(2, f12 - f22)
    m5 = prod(4, b22)
    emit(1, m3 + m5)
    m1 = prod(0, f11 + f22)
    emit(3, (m1 - m2 + m3) + prod(5, f11 + f12))
    emit(0, (m1 + m4 - m5) + prod(6, f21 + f22))


def _kernel(x_hbm, mem0_hbm, wq_hbm, wk_hbm, wv_hbm, wo_hbm, w1_hbm, w3_hbm, w2_hbm,
            c_hbm, wmod_hbm, out_hbm,
            wqkv, big32, w13_32, ring, oring, xb, xf, mod, hs, ot, fill_ref, prob, acc, early, c_ref, mem0_ref,
            sems, osems,
            *, S, D, H, F, M, SEG, FB):
    NSEG = S // SEG
    XR = SEG - M
    P = S - NSEG * XR
    R = ring.shape[0]
    QOFF = R - P
    OOFF = (-NSEG * XR) % R
    ND = D // LANE
    NF = F // LANE
    HP = H // 2
    HD = H * LANE
    scale = float(LANE) ** -0.5
    big, w13 = big32.bitcast(BF16), w13_32.bitcast(BF16)
    DH = D // 2
    PG = 8
    NA = HP // PG
    NSLOT = big32.shape[0] // DH
    WP = DH + SLAB_PAD
    WO = ND * HD

    def tile(n, width=1):
        return pl.ds(n * LANE if isinstance(n, int) else pl.multiple_of(n * LANE, LANE), width * LANE)

    def head_slab(n):
        return (n // (2 * PG) * 2 * PG + n % 2 * PG + n % (2 * PG) // 2) * WP

    def slab(row0, rows):
        return pltpu.bitcast(big32[pl.ds(row0 // 16, rows // 16)].reshape(rows // 2, LANE), BF16)

    def slab_copies(src, tiles, dst_fn, sem):
        return [pltpu.make_async_copy(src.at[..., pl.ds(j * LANE, LANE)], dst_fn(j), sem) for j in tiles]

    def half_tiles(c):
        return [v * ND + c * ND // 2 + j for v in range(2) for j in range(ND // 2)]

    cp_x0 = pltpu.make_async_copy(x_hbm.at[pl.ds(0, P)], xb.at[pl.ds(0, P)], sems.at[0])
    cp_x1 = pltpu.make_async_copy(x_hbm.at[pl.ds(P, S - P)], xb.at[pl.ds(P, S - P)], sems.at[1])
    mod_tiles = [half_tiles(0), half_tiles(1), list(range(2 * ND, 6 * ND))]
    cp_mod = [slab_copies(wmod_hbm, t, lambda j: w13.at[j], sems.at[2 + i])
              for i, t in enumerate(mod_tiles)]
    cp_w = [pltpu.make_async_copy(w.at[pl.ds(c * DH, DH), a],
                                  big.at[pl.ds(((2 * t + c) * NA + a) % NSLOT * DH, DH)],
                                  sems.at[7 + (2 * t + c) * NA + a])
            for t, w in enumerate((wq_hbm, wk_hbm, wv_hbm)) for c in range(2) for a in range(NA)]
    cp_o = slab_copies(wo_hbm, range(ND), lambda j: big.at[pl.ds((WO + j * HD) // 16, HD // 16)], sems.at[5])
    cp_ffn = (slab_copies(w1_hbm, range(NF), lambda j: w13.at[2 * j], sems.at[6])
              + slab_copies(w3_hbm, range(NF), lambda j: w13.at[2 * j + 1], sems.at[6])
              + slab_copies(w2_hbm, range(ND), lambda j: big.at[pl.ds(j * F // 16, F // 16)], sems.at[6]))

    def start(cps):
        for cp in cps:
            cp.start()

    def wait(cps):
        for cp in cps:
            cp.wait()

    cp_c = pltpu.make_async_copy(c_hbm, c_ref, sems.at[7 + len(cp_w)])
    cp_mem = pltpu.make_async_copy(mem0_hbm, mem0_ref, sems.at[8 + len(cp_w)])
    cp_c.start()
    start(cp_mod[0])
    cp_x0.start()
    cp_w[0].start()
    cp_mem.start()
    cp_c.wait()

    cc = jnp.broadcast_to(c_ref[...].astype(F32), (16, D))
    sc = _silu(cc).astype(BF16)

    def mod_part(i):
        wait(cp_mod[i])
        for j in mod_tiles[i]:
            r = _dot(sc, pltpu.bitcast(w13_32[j], BF16))[0:8]
            if j // ND in (1, 4):
                r = r + 1.0
            mod[j // ND, :, pl.ds((j % ND) * LANE, LANE)] = r

    def modv(i):
        return mod[i, 0:1, :]

    G = 2 * (M + SEG)
    ri = lax.broadcasted_iota(jnp.int32, (G, LANE), 0)
    ci = lax.broadcasted_iota(jnp.int32, (G, LANE), 1)

    def head_pos(i):
        head = jnp.where(i < 2 * M, i // M, (i - 2 * M) // SEG)
        pos = jnp.where(i < 2 * M, i % M, M + (i - 2 * M) % SEG)
        return head, pos

    rh, rp = head_pos(ri)
    ch, cp_ = head_pos(ci)
    visible = (rp < M) | (rp >= cp_)
    fill_ref[0:G, :] = jnp.where(rh == ch, jnp.where(visible, 0.0, -1e9), -jnp.inf).astype(F32)

    LB = 128
    PH = P // 2
    DQ = D // 4

    def norm_half(c):
        cols = slice(c * DH, (c + 1) * DH)

        def norm0(k, carry):
            halves = []
            for o in (0, PH):
                rows = pl.ds(pl.multiple_of(o + k * LB, LB), LB)
                if c == 0:
                    xv = xb[rows, :].astype(F32)
                    xf[rows, :] = xv
                    xn = _norm(xv)
                    oring[rows, 0:DH] = xn[:, DH:]
                    xn = xn[:, :DH]
                else:
                    xn = oring[rows, 0:DH]
                halves.append(xn * mod[1, 0:1, cols] + mod[0, 0:1, cols])
            top, bot = halves
            ops = _strassen_lhs(top[:, :DQ], top[:, DQ:], bot[:, :DQ], bot[:, DQ:])
            for i in range(7):
                hs[i, pl.ds(pl.multiple_of(c * (PH // 2) + k * (LB // 2), LB // 2), LB // 2), :] = ops[i]
            return carry

        lax.fori_loop(0, PH // LB, norm0, 0)

    def arrivals(it):
        if it == 0:
            cp_w[0].wait()
            start(cp_w[2:3] + cp_mod[1] + cp_w[3:4])
        else:
            wait(cp_w[it + (it > 1):it + 2])
        if it == 1:
            start(cp_w[4:6])
        if it == NA:
            start(cp_w[6:NSLOT])
            mod_part(1)
            norm_half(1)
        if it == 4:
            start(cp_w[NSLOT:] + [cp_x1] + cp_mod[2])
        if it == NSLOT - 1:
            wait(cp_w[it + 2:])
            start(cp_o)

    def head_rows(it):
        chunk, a = it // NA, it % NA
        base = (chunk // 2 * H + 2 * PG * a) * WP + chunk % 2 * (DH // 2)
        return wqkv.at[pl.ds(pl.multiple_of(base, 32), (2 * PG + 1) * WP)]

    def retile(it, r0, r1):
        src = big32.at[pl.ds(it % NSLOT * DH, DH)]
        dst = head_rows(it)
        for r in range(r0, r1):
            even, odd = src[2 * r], src[2 * r + 1]
            dst[pl.ds(r, PG, stride=WP), :] = (even & jnp.uint32(0xFFFF)) | (odd << 16)
            dst[pl.ds(PG * WP + r, PG, stride=WP), :] = (even >> 16) | (odd & jnp.uint32(0xFFFF0000))

    def project(it, carry):
        for ev in range(NSLOT):
            pl.when(it == ev)(functools.partial(arrivals, ev))
        pl.when(it < 2)(lambda: retile(it, 0, DH // 2))
        half = it // NA % 2
        hrows = pl.ds(pl.multiple_of(half * (PH // 2), PH // 2), PH // 2)
        nxt = jnp.where(it == 0, 0, jnp.minimum(it + 1, 6 * NA - 1))
        dst = ring.at[:, tile(it // (2 * NA) * H + 2 * PG * (it % NA), 2 * PG)]
        for b in range(PG):
            lo, hi = (pltpu.bitcast(head_rows(it)[pl.ds((i * PG + b) * WP, DH // 2), :], BF16)
                      for i in range(2))

            def emit(i, r, b=b):
                idx = pl.ds(QOFF + i // 2 * PH, PH), tile(2 * b + i % 2)
                dst[idx] = r + jnp.where(half == 1, dst[idx], 0.0)

            _strassen(lambda i: hs[i, hrows, :], lo[:DQ], hi[:DQ], lo[DQ:], hi[DQ:], emit)
            retile(nxt, b * (DH // 2) // PG, (b + 1) * (DH // 2) // PG)
        return carry

    mod_part(0)
    cp_x0.wait()
    norm_half(0)
    cp_w[1].start()
    lax.fori_loop(0, 6 * NA, project, 0)
    mod_part(2)
    start(cp_ffn)

    HG = SEG // 2
    xf3, xb3 = xf.reshape(NSEG, SEG, D), xb.reshape(NSEG, SEG, D)

    def ffn_norm(grp):
        hn = _ada_ln(xf[pl.ds(pl.multiple_of(grp * SEG, SEG), SEG), :], modv(3), modv(4))
        ops = _strassen_lhs(hn[:HG, :DH], hn[:HG, DH:], hn[HG:, :DH], hn[HG:, DH:])
        for i in range(7):
            ring[pl.ds(pl.multiple_of(grp * (HG // 2), HG // 2), HG // 2),
                 tile(3 * H + i * ND // 2, ND // 2)] = pltpu.bitcast(ops[i], F32)

    L0 = S // 4

    def widen(grp):
        rows = pl.ds(pl.multiple_of(grp * SEG, SEG), SEG)
        xf[rows, :] = xb[rows, :].astype(F32)

    def next_rows(r0):
        ring[pl.ds(L0 + M, XR), tile(3 * H, ND)] = _ada_ln(xf[pl.ds(r0, XR), :], modv(0), modv(1))

    cp_mem.wait()
    ring[pl.ds(L0, M), tile(3 * H, ND)] = mem0_ref[...].astype(F32)
    cp_x1.wait()
    widen(P // SEG)
    next_rows(P)
    wait(cp_o)

    def step(s, carry):
        q_wr = pl.multiple_of(lax.rem(s * XR, R), 8)
        q_rd = pl.multiple_of(lax.rem(s * SEG + QOFF, R), SEG)
        o_wr = pl.multiple_of(lax.rem(s * SEG + OOFF, R), SEG)
        o_rd = pl.multiple_of(lax.rem(s * XR + OOFF, R), 8)
        h = ring[pl.ds(L0, SEG), tile(3 * H, ND)].astype(BF16)
        tail_rows = pl.ds(pl.multiple_of(jnp.maximum(s - NSEG * XR // SEG, 0) * (HG // 2), HG // 2), HG // 2)
        pad = jnp.zeros((LANE - G, LANE), BF16)

        def weights(n, d0, d):
            return pltpu.bitcast(wqkv[pl.ds(head_slab(n) + d0 // 2, d // 2), :], BF16)

        for u in range(4):
            early[u] = _dot(h[:, :DH], weights(u // 2 * H + u % 2, 0, DH))

        def head_pair(t, g):
            n = t * H + 2 * g
            mem_rows = []
            for i in range(2):
                if t < 2 and g == 0:
                    r = _dot(h[:, DH:], weights(n + i, DH, DH)) + early[2 * t + i]
                else:
                    r = _dot(h, weights(n + i, 0, D))
                ring[pl.ds(q_wr, XR), tile(n + i)] = r[M:]
                mem_rows.append(r[:M])
            return jnp.concatenate(
                mem_rows + [ring[pl.ds(q_rd, SEG), tile(n + i)] for i in range(2)],
                axis=0).astype(BF16)

        def scores(q, k):
            sc_ = lax.dot_general(q, jnp.concatenate([k, pad], axis=0), (((1,), (1,)), ((), ())),
                                  preferred_element_type=F32)
            fill = fill_ref[0:G, :]
            sc_ = jnp.where(fill == 0.0, sc_ * scale, fill)
            e = jnp.exp(sc_ - jnp.max(sc_, axis=-1, keepdims=True))
            return (e * (1.0 / jnp.sum(e, axis=-1, keepdims=True))).astype(BF16)

        def attend(g, p, v):
            o = _dot(p, jnp.concatenate([v, pad], axis=0))
            ops = _strassen_lhs(*(o[2 * M + i * SEG + r:2 * M + i * SEG + r + HG]
                                  for r in (0, HG) for i in range(2)))
            for i in range(7):
                ot[i, tail_rows, pl.ds(g * LANE, LANE)] = ops[i]
            for i in range(2):
                oring[pl.ds(o_wr, SEG), tile(2 * g + i)] = o[2 * M + i * SEG:2 * M + (i + 1) * SEG]
            return [jnp.concatenate([o[i * M:(i + 1) * M], oring[pl.ds(o_rd, XR), tile(2 * g + i)]],
                                    axis=0).astype(BF16) for i in range(2)]

        heads = {}

        def oproj(g0, g1, j0=0, j1=ND):
            a = jnp.concatenate([r for g in range(g0, g1) for r in heads[g]], axis=1)
            for j in range(j0, j1):
                cols = pl.ds(j * LANE, LANE)
                r = _dot(a, slab(WO + j * HD + g0 * 2 * LANE, (g1 - g0) * 2 * LANE))
                if g0 > 0:
                    r = r + acc[:, cols]
                if g1 < HP:
                    acc[:, cols] = r
                else:
                    ring[pl.ds(L0, M), tile(3 * H + j)] = r[:M]
                    xf[rows, cols] = xf[rows, cols] + mod[2, 0:1, cols] * r[M:]

        rows = pl.ds(pl.multiple_of(s * XR, 8), XR)
        qk, val = {}, {}
        for i in range(2 * HP + VALUE_LAG):
            if i == NEXT_ROWS_AT:
                widen(jnp.minimum(P // SEG + 1 + s, NSEG - 1))
                next_rows(pl.multiple_of(jnp.minimum(P + (s + 1) * XR, S - XR), 8))
            if i == FFN_NORM_AT:
                ffn_norm(jnp.maximum(s * XR // SEG - 1, 0))
            if i < HP:
                qk[i] = head_pair(0, i), head_pair(1, i)
            elif i < 2 * HP:
                val[i - HP] = head_pair(2, i - HP)
            else:
                oproj(0, HP // 2, i - 2 * HP, i - 2 * HP + 1)
            g = i - SCORE_LAG
            if g % SCORE_GROUP == 0 and 0 < g <= HP:
                for u in range(g - SCORE_GROUP, g):
                    prob[u] = pltpu.bitcast(scores(*qk[u]), U32)
            g = i - HP - VALUE_LAG
            if g >= 0:
                heads[g] = attend(g, pltpu.bitcast(prob[g], BF16), val[g])
        oproj(0, HP // 2, VALUE_LAG, ND)
        oproj(HP // 2, HP)
        return carry

    lax.fori_loop(0, NSEG, step, 0, unroll=2)

    MH = FB // 2

    def row_tiles(row0, n, par):
        return jnp.concatenate([slab(row0 + (2 * k + par) * LANE, LANE) for k in range(n // 2)], axis=0)

    def otail(j, carry):
        def emit(n, y):
            cols = pl.ds(pl.multiple_of((2 * j + n % 2) * LANE, LANE), LANE)
            idx = (pl.ds(NSEG * XR // SEG, P // SEG), pl.ds(n // 2 * HG, HG), cols)
            xf3[idx] = xf3[idx] + (mod[2, 0:1, cols] * y).reshape(P // SEG, HG, LANE)

        _strassen(lambda i: ot[i],
                  *(row_tiles(WO + (2 * j + u) * HD, H, par) for par in range(2) for u in range(2)), emit)
        return carry

    lax.fori_loop(0, ND // 2, otail, 0)
    G0 = (NSEG - 1) * XR // SEG - 1

    def norm_tail(i, carry):
        for u in range(6):
            ffn_norm(G0 + 6 * i + u)
        return carry

    lax.fori_loop(0, (NSEG - G0) // 6, norm_tail, 0)

    wait(cp_ffn)

    def act_slot(k, i):
        return wqkv.at[pl.ds(pl.multiple_of((7 * k + i) * (MH // 2), MH // 2), MH // 2)]

    def out_copy(blk, j):
        idx = (pl.ds(pl.multiple_of(blk * FB, FB), FB), pl.ds(pl.multiple_of(j * 2 * LANE, 2 * LANE), 2 * LANE))
        return pltpu.make_async_copy(xb.at[idx], out_hbm.at[idx], osems.at[blk * (ND // 2) + j])

    def ffn(blk, carry):
        def normed(i):
            rows = pl.ds(pl.multiple_of(blk * (MH // 2), MH // 2), MH // 2)
            return ring[rows, tile(3 * H + i * ND // 2, ND // 2)]

        def up(k, c):
            res = {}, {}
            for t in range(2):
                b1, b2 = (pltpu.bitcast(w13_32[4 * k + 2 * u + t], BF16) for u in range(2))
                _strassen(normed,
                          b1[:DH], b2[:DH], b1[DH:], b2[DH:], res[t].setdefault)
            ops = _strassen_lhs(*(_silu(res[0][n]) * res[1][n] for n in range(4)))
            for i in (1, 3, 6, 0, 2, 4, 5):
                act_slot(k, i)[...] = ops[i]
            return c

        lax.fori_loop(0, NF // 2, up, 0, unroll=2)

        def down(j, c):
            def emit(n, y):
                cols = pl.ds(pl.multiple_of((2 * j + n % 2) * LANE, LANE), LANE)
                idx = (pl.ds(blk * (FB // SEG), FB // SEG), pl.ds(n // 2 * HG, HG), cols)
                xb3[idx] = (xf3[idx] + (mod[5, 0:1, cols] * y).reshape(FB // SEG, HG, LANE)).astype(BF16)

            _strassen(lambda i: jnp.concatenate([act_slot(k, i)[...] for k in range(NF // 2)], axis=1),
                      *(row_tiles((2 * j + u) * F, NF, par) for par in range(2) for u in range(2)), emit)
            out_copy(blk, j).start()
            return c

        lax.fori_loop(0, ND // 2, down, 0)
        return carry

    lax.fori_loop(0, S // FB, ffn, 0)
    for blk in range(S // FB):
        for j in range(ND // 2):
            out_copy(blk, j).wait()


@functools.partial(jax.jit, static_argnames=("A_seg_len",))
def pallas_adaLN_cond__memory_aug_recurrent_mem_tr__glu_gated_swiglu__prompt_kernel(
    A_x, A_mem0, A_Wq, A_Wk, A_Wv, A_Wo, A_seg_len, B_x, B_w1, B_w3, B_w2, c, w_mod,
):
    del B_x
    B, S, D = A_x.shape
    _, H, Dh = A_Wq.shape
    M = A_mem0.shape[1]
    F = B_w1.shape[1]
    SEG = int(A_seg_len)
    assert (B, S, D, H, Dh, M, SEG) == (1, 2048, 1024, 32, LANE, 8, 32) and F == 3584
    P = S // SEG * M
    R = 576
    FB = 1024

    hbm = pl.BlockSpec(memory_space=pl.ANY)
    out = pl.pallas_call(
        functools.partial(_kernel, S=S, D=D, H=H, F=F, M=M, SEG=SEG, FB=FB),
        out_shape=jax.ShapeDtypeStruct((S, D), A_x.dtype),
        in_specs=[hbm] * 11,
        out_specs=hbm,
        scratch_shapes=[
            pltpu.VMEM((3 * H * (D // 2 + SLAB_PAD) + D, LANE), U32),
            pltpu.VMEM((D * H // 8, 8, LANE), U32),
            pltpu.VMEM((2 * F // LANE, D // 2, LANE), U32),
            pltpu.VMEM((R, 3 * H * Dh + 7 * D // 2), F32),
            pltpu.VMEM((R, H * Dh), F32),
            pltpu.VMEM((S, D), BF16),
            pltpu.VMEM((S, D), F32),
            pltpu.VMEM((6, 8, D), F32),
            pltpu.VMEM((7, P // 2, D // 4), U32),
            pltpu.VMEM((7, P // 4, H * Dh // 2), U32),
            pltpu.VMEM((3 * SEG, LANE), F32),
            pltpu.VMEM((H // 2, M + SEG, LANE), U32),
            pltpu.VMEM((SEG, D), F32),
            pltpu.VMEM((4, SEG, LANE), F32),
            pltpu.VMEM((1, D), c.dtype),
            pltpu.VMEM((M, D), A_mem0.dtype),
            pltpu.SemaphoreType.DMA((9 + 6 * H // 16,)),
            pltpu.SemaphoreType.DMA((S // FB * D // (2 * LANE),)),
        ],
        compiler_params=pltpu.CompilerParams(vmem_limit_bytes=126 * 2**20),
        name="adaln_rmt_swiglu",
    )(A_x.reshape(S, D), A_mem0.reshape(M, D), *(w.reshape(D, H // 16, 16, Dh) for w in (A_Wq, A_Wk, A_Wv)),
      A_Wo.reshape(H * Dh // 16, 16, D), B_w1, B_w3, B_w2.reshape(F // 16, 16, D), c, w_mod)
    return out.reshape(B, S, D)
```

```python
import functools

import jax
import jax.numpy as jnp
from jax import lax
import jax.experimental.pallas as pl
import jax.experimental.pallas.tpu as pltpu

F32 = jnp.float32
BF16 = jnp.bfloat16
U32 = jnp.uint32
LANE = 128
EPS = 1e-5
SLAB_PAD = 4
SCORE_GROUP = 4
SCORE_LAG = 1
VALUE_LAG = 3
FFN_NORM_AT = 7
NEXT_ROWS_AT = 28


def _dot(a, b):
    return jnp.dot(a, b, preferred_element_type=F32)


def _norm(x):
    m = jnp.mean(x, axis=-1, keepdims=True)
    d = x - m
    v = jnp.mean(d * d, axis=-1, keepdims=True)
    return d * lax.rsqrt(v + EPS)


def _ada_ln(x, shift, scale1):
    return _norm(x) * scale1 + shift


def _silu(x):
    h = 0.5 * x
    return h + h * jnp.tanh(h)


def _words(x):
    return pltpu.bitcast(x.astype(BF16), U32)


def _strassen_lhs(a11, a12, a21, a22):
    return [_words(a) for a in (a11 + a22, a21 + a22, a11, a22, a11 + a12, a21 - a11, a12 - a22)]


def _strassen(lhs_fn, b11, b12, b21, b22, emit):
    f11, f12, f21, f22 = (b.astype(F32) for b in (b11, b12, b21, b22))

    def prod(i, b):
        return _dot(pltpu.bitcast(lhs_fn(i), BF16), b.astype(BF16))

    m2 = prod(1, b11)
    m4 = prod(3, f21 - f11)
    emit(2, m2 + m4)
    m3 = prod(2, f12 - f22)
    m5 = prod(4, b22)
    emit(1, m3 + m5)
    m1 = prod(0, f11 + f22)
    emit(3, (m1 - m2 + m3) + prod(5, f11 + f12))
    emit(0, (m1 + m4 - m5) + prod(6, f21 + f22))


def _kernel(x_hbm, mem0_hbm, wq_hbm, wk_hbm, wv_hbm, wo_hbm, w1_hbm, w3_hbm, w2_hbm,
            c_hbm, wmod_hbm, out_hbm,
            wqkv, big, w13, ring, oring, xb, xf, mod, hs, ot, fill_ref, prob, acc, early, c_ref, mem0_ref,
            sems, osems,
            *, S, D, H, F, M, SEG, FB):
    NSEG = S // SEG
    XR = SEG - M
    P = S - NSEG * XR
    R = ring.shape[0]
    QOFF = R - P
    OOFF = (-NSEG * XR) % R
    ND = D // LANE
    NF = F // LANE
    HP = H // 2
    HD = H * LANE
    scale = float(LANE) ** -0.5
    DH = D // 2
    PG = 8
    NA = HP // PG
    NSLOT = big.shape[0] // DH
    WP = DH + SLAB_PAD
    WO = ND * HD

    def tile(n, width=1):
        return pl.ds(n * LANE if isinstance(n, int) else pl.multiple_of(n * LANE, LANE), width * LANE)

    def head_slab(n):
        return (n // (2 * PG) * 2 * PG + n % 2 * PG + n % (2 * PG) // 2) * WP

    def slab(row0, rows):
        return big[pl.ds(row0 // 16, rows // 16)].reshape(rows, LANE)

    def slab_copies(src, tiles, dst_fn, sem):
        return [pltpu.make_async_copy(src.at[..., pl.ds(j * LANE, LANE)], dst_fn(j), sem) for j in tiles]

    def half_tiles(c):
        return [v * ND + c * ND // 2 + j for v in range(2) for j in range(ND // 2)]

    cp_x0 = pltpu.make_async_copy(x_hbm.at[pl.ds(0, P)], xb.at[pl.ds(0, P)], sems.at[0])
    cp_x1 = pltpu.make_async_copy(x_hbm.at[pl.ds(P, S - P)], xb.at[pl.ds(P, S - P)], sems.at[1])
    mod_tiles = [half_tiles(0), half_tiles(1), list(range(2 * ND, 6 * ND))]
    cp_mod = [slab_copies(wmod_hbm, t, lambda j: w13.at[j], sems.at[2 + i])
              for i, t in enumerate(mod_tiles)]
    cp_w = [pltpu.make_async_copy(w.at[pl.ds(c * DH, DH), a],
                                  big.at[pl.ds(((2 * t + c) * NA + a) % NSLOT * DH, DH)],
                                  sems.at[7 + (2 * t + c) * NA + a])
            for t, w in enumerate((wq_hbm, wk_hbm, wv_hbm)) for c in range(2) for a in range(NA)]
    cp_o = slab_copies(wo_hbm, range(ND), lambda j: big.at[pl.ds((WO + j * HD) // 16, HD // 16)], sems.at[5])
    cp_ffn = (slab_copies(w1_hbm, range(NF), lambda j: w13.at[2 * j], sems.at[6])
              + slab_copies(w3_hbm, range(NF), lambda j: w13.at[2 * j + 1], sems.at[6])
              + slab_copies(w2_hbm, range(ND), lambda j: big.at[pl.ds(j * F // 16, F // 16)], sems.at[6]))

    def start(cps):
        for cp in cps:
            cp.start()

    def wait(cps):
        for cp in cps:
            cp.wait()

    cp_c = pltpu.make_async_copy(c_hbm, c_ref, sems.at[7 + len(cp_w)])
    cp_mem = pltpu.make_async_copy(mem0_hbm, mem0_ref, sems.at[8 + len(cp_w)])
    cp_c.start()
    start(cp_mod[0])
    cp_x0.start()
    cp_w[0].start()
    cp_mem.start()
    cp_c.wait()

    cc = jnp.broadcast_to(c_ref[...].astype(F32), (16, D))
    sc = _silu(cc).astype(BF16)

    def mod_part(i):
        for j in mod_tiles[i]:
            r = _dot(sc, w13[j])[0:8]
            if j // ND in (1, 4):
                r = r + 1.0
            mod[j // ND, :, pl.ds((j % ND) * LANE, LANE)] = r

    def modv(i):
        return mod[i, 0:1, :]

    G = 2 * (M + SEG)
    ri = lax.broadcasted_iota(jnp.int32, (G, LANE), 0)
    ci = lax.broadcasted_iota(jnp.int32, (G, LANE), 1)

    def head_pos(i):
        head = jnp.where(i < 2 * M, i // M, (i - 2 * M) // SEG)
        pos = jnp.where(i < 2 * M, i % M, M + (i - 2 * M) % SEG)
        return head, pos

    rh, rp = head_pos(ri)
    ch, cp_ = head_pos(ci)
    visible = (rp < M) | (rp >= cp_)
    fill_ref[0:G, :] = jnp.where(rh == ch, jnp.where(visible, 0.0, -1e9), -jnp.inf).astype(F32)

    LB = 128
    PH = P // 2
    DQ = D // 4

    def norm_half(c):
        cols = slice(c * DH, (c + 1) * DH)

        def norm0(k, carry):
            halves = []
            for o in (0, PH):
                rows = pl.ds(pl.multiple_of(o + k * LB, LB), LB)
                if c == 0:
                    xv = xb[rows, :].astype(F32)
                    xf[rows, :] = xv
                    xn = _norm(xv)
                    oring[rows, 0:DH] = xn[:, DH:]
                    xn = xn[:, :DH]
                else:
                    xn = oring[rows, 0:DH]
                halves.append(xn * mod[1, 0:1, cols] + mod[0, 0:1, cols])
            top, bot = halves
            ops = _strassen_lhs(top[:, :DQ], top[:, DQ:], bot[:, :DQ], bot[:, DQ:])
            for i in range(7):
                hs[i, pl.ds(pl.multiple_of(c * (PH // 2) + k * (LB // 2), LB // 2), LB // 2), :] = ops[i]
            return carry

        lax.fori_loop(0, PH // LB, norm0, 0)

    def arrivals(it):
        if it == 0:
            cp_w[0].wait()
            start(cp_w[2:3] + cp_mod[1] + cp_w[3:4])
        else:
            wait(cp_w[it + (it > 1):it + 2])
        if it == 1:
            start(cp_w[4:6])
        if it == NA:
            start(cp_w[6:NSLOT])
            wait(cp_mod[1])
            mod_part(1)
            norm_half(1)
        if it == 4:
            start(cp_w[NSLOT:] + [cp_x1] + cp_mod[2])
        if it == NSLOT - 1:
            wait(cp_w[it + 2:])
            start(cp_o)

    def head_rows(it):
        chunk, a = it // NA, it % NA
        base = (chunk // 2 * H + 2 * PG * a) * WP + chunk % 2 * (DH // 2)
        return wqkv.at[pl.ds(pl.multiple_of(base, 32), (2 * PG + 1) * WP)]

    def retile(it, r0, r1):
        src = big.at[pl.ds(it % NSLOT * DH, DH)]
        dst = head_rows(it)
        for r in range(r0, r1):
            even, odd = pltpu.bitcast(src[2 * r], U32), pltpu.bitcast(src[2 * r + 1], U32)
            dst[pl.ds(r, PG, stride=WP), :] = (even & jnp.uint32(0xFFFF)) | (odd << 16)
            dst[pl.ds(PG * WP + r, PG, stride=WP), :] = (even >> 16) | (odd & jnp.uint32(0xFFFF0000))

    def project(it, carry):
        for ev in range(NSLOT):
            pl.when(it == ev)(functools.partial(arrivals, ev))
        pl.when(it < 2)(lambda: retile(it, 0, DH // 2))
        half = it // NA % 2
        hrows = pl.ds(pl.multiple_of(half * (PH // 2), PH // 2), PH // 2)
        nxt = jnp.where(it == 0, 0, jnp.minimum(it + 1, 6 * NA - 1))
        dst = ring.at[:, tile(it // (2 * NA) * H + 2 * PG * (it % NA), 2 * PG)]
        for b in range(PG):
            lo, hi = (pltpu.bitcast(head_rows(it)[pl.ds((i * PG + b) * WP, DH // 2), :], BF16)
                      for i in range(2))

            def emit(i, r, b=b):
                idx = pl.ds(QOFF + i // 2 * PH, PH), tile(2 * b + i % 2)
                dst[idx] = r + jnp.where(half == 1, dst[idx], 0.0)

            _strassen(lambda i: hs[i, hrows, :], lo[:DQ], hi[:DQ], lo[DQ:], hi[DQ:], emit)
            retile(nxt, b * (DH // 2) // PG, (b + 1) * (DH // 2) // PG)
        return carry

    wait(cp_mod[0])
    mod_part(0)
    cp_x0.wait()
    norm_half(0)
    cp_w[1].start()
    lax.fori_loop(0, 6 * NA, project, 0)

    HG = SEG // 2

    def residual(dst, row0, j, gate, n, y):
        cols = tile(2 * j + n % 2)
        y = mod[gate, 0:1, cols] * y
        for u in range(y.shape[0] // HG):
            rows = pl.ds(row0 + u * SEG + n // 2 * HG, HG)
            dst[rows, cols] = (xf[rows, cols] + y[u * HG:(u + 1) * HG]).astype(dst.dtype)

    def ffn_norm(grp):
        hn = _ada_ln(xf[pl.ds(pl.multiple_of(grp * SEG, SEG), SEG), :], modv(3), modv(4))
        ops = _strassen_lhs(hn[:HG, :DH], hn[:HG, DH:], hn[HG:, :DH], hn[HG:, DH:])
        for i in range(7):
            ring[pl.ds(pl.multiple_of(grp * (HG // 2), HG // 2), HG // 2),
                 tile(3 * H + i * ND // 2, ND // 2)] = pltpu.bitcast(ops[i], F32)

    L0 = S // 4

    def widen(grp):
        rows = pl.ds(pl.multiple_of(grp * SEG, SEG), SEG)
        xf[rows, :] = xb[rows, :].astype(F32)

    def next_rows(r0):
        ring[pl.ds(L0 + M, XR), tile(3 * H, ND)] = _ada_ln(xf[pl.ds(r0, XR), :], modv(0), modv(1))

    wait([cp_mem, cp_x1] + cp_o + cp_mod[2])
    ring[pl.ds(L0, M), tile(3 * H, ND)] = mem0_ref[...].astype(F32)
    widen(P // SEG)
    next_rows(P)
    mod_part(2)
    start(cp_ffn)

    def step(s, carry):
        q_wr = pl.multiple_of(lax.rem(s * XR, R), 8)
        q_rd = pl.multiple_of(lax.rem(s * SEG + QOFF, R), SEG)
        o_wr = pl.multiple_of(lax.rem(s * SEG + OOFF, R), SEG)
        o_rd = pl.multiple_of(lax.rem(s * XR + OOFF, R), 8)
        h = ring[pl.ds(L0, SEG), tile(3 * H, ND)].astype(BF16)
        tail_rows = pl.ds(pl.multiple_of(jnp.maximum(s - NSEG * XR // SEG, 0) * (HG // 2), HG // 2), HG // 2)
        pad = jnp.zeros((LANE - G, LANE), BF16)

        def weights(n, d0, d):
            return pltpu.bitcast(wqkv[pl.ds(head_slab(n) + d0 // 2, d // 2), :], BF16)

        for u in range(4):
            early[u] = _dot(h[:, :DH], weights(u // 2 * H + u % 2, 0, DH))

        def head_pair(t, g):
            n = t * H + 2 * g
            mem_rows = []
            for i in range(2):
                if t < 2 and g == 0:
                    r = _dot(h[:, DH:], weights(n + i, DH, DH)) + early[2 * t + i]
                else:
                    r = _dot(h, weights(n + i, 0, D))
                ring[pl.ds(q_wr, XR), tile(n + i)] = r[M:]
                mem_rows.append(r[:M])
            return jnp.concatenate(
                mem_rows + [ring[pl.ds(q_rd, SEG), tile(n + i)] for i in range(2)],
                axis=0).astype(BF16)

        def scores(q, k):
            sc_ = lax.dot_general(q, jnp.concatenate([k, pad], axis=0), (((1,), (1,)), ((), ())),
                                  preferred_element_type=F32)
            fill = fill_ref[0:G, :]
            sc_ = jnp.where(fill == 0.0, sc_ * scale, fill)
            e = jnp.exp(sc_ - jnp.max(sc_, axis=-1, keepdims=True))
            return (e * (1.0 / jnp.sum(e, axis=-1, keepdims=True))).astype(BF16)

        def attend(g, p, v):
            o = _dot(p, jnp.concatenate([v, pad], axis=0))
            ops = _strassen_lhs(*(o[2 * M + i * SEG + r:2 * M + i * SEG + r + HG]
                                  for r in (0, HG) for i in range(2)))
            for i in range(7):
                ot[i, tail_rows, pl.ds(g * LANE, LANE)] = ops[i]
            for i in range(2):
                oring[pl.ds(o_wr, SEG), tile(2 * g + i)] = o[2 * M + i * SEG:2 * M + (i + 1) * SEG]
            return [jnp.concatenate([o[i * M:(i + 1) * M], oring[pl.ds(o_rd, XR), tile(2 * g + i)]],
                                    axis=0).astype(BF16) for i in range(2)]

        heads = {}

        def oproj(g0, g1, j0=0, j1=ND):
            a = jnp.concatenate([r for g in range(g0, g1) for r in heads[g]], axis=1)
            for j in range(j0, j1):
                cols = pl.ds(j * LANE, LANE)
                r = _dot(a, slab(WO + j * HD + g0 * 2 * LANE, (g1 - g0) * 2 * LANE))
                if g0 > 0:
                    r = r + acc[:, cols]
                if g1 < HP:
                    acc[:, cols] = r
                else:
                    ring[pl.ds(L0, M), tile(3 * H + j)] = r[:M]
                    xf[rows, cols] = xf[rows, cols] + mod[2, 0:1, cols] * r[M:]

        rows = pl.ds(pl.multiple_of(s * XR, 8), XR)
        qk, val = {}, {}
        for i in range(2 * HP + VALUE_LAG):
            if i == NEXT_ROWS_AT:
                widen(jnp.minimum(P // SEG + 1 + s, NSEG - 1))
                next_rows(pl.multiple_of(jnp.minimum(P + (s + 1) * XR, S - XR), 8))
            if i == FFN_NORM_AT:
                ffn_norm(jnp.maximum(s * XR // SEG - 1, 0))
            if i < HP:
                qk[i] = head_pair(0, i), head_pair(1, i)
            elif i < 2 * HP:
                val[i - HP] = head_pair(2, i - HP)
            else:
                oproj(0, HP // 2, i - 2 * HP, i - 2 * HP + 1)
            g = i - SCORE_LAG
            if g % SCORE_GROUP == 0 and 0 < g <= HP:
                for u in range(g - SCORE_GROUP, g):
                    prob[u] = pltpu.bitcast(scores(*qk[u]), U32)
            g = i - HP - VALUE_LAG
            if g >= 0:
                heads[g] = attend(g, pltpu.bitcast(prob[g], BF16), val[g])
        oproj(0, HP // 2, VALUE_LAG, ND)
        oproj(HP // 2, HP)
        return carry

    lax.fori_loop(0, NSEG, step, 0, unroll=2)

    MH = FB // 2

    def row_tiles(row0, n, par):
        return jnp.concatenate([slab(row0 + (2 * k + par) * LANE, LANE) for k in range(n // 2)], axis=0)

    def otail(j, carry):
        emit = functools.partial(residual, xf, NSEG * XR, j, 2)
        _strassen(lambda i: ot[i],
                  *(row_tiles(WO + (2 * j + u) * HD, H, par) for par in range(2) for u in range(2)), emit)
        return carry

    lax.fori_loop(0, ND // 2, otail, 0)
    G0 = (NSEG - 1) * XR // SEG - 1

    def norm_tail(i, carry):
        for u in range(6):
            ffn_norm(G0 + 6 * i + u)
        return carry

    lax.fori_loop(0, (NSEG - G0) // 6, norm_tail, 0)

    wait(cp_ffn)

    def act_slot(k, i):
        return wqkv.at[pl.ds(pl.multiple_of((7 * k + i) * (MH // 2), MH // 2), MH // 2)]

    def out_copy(blk, j):
        idx = (pl.ds(pl.multiple_of(blk * FB, FB), FB), pl.ds(pl.multiple_of(j * 2 * LANE, 2 * LANE), 2 * LANE))
        return pltpu.make_async_copy(xb.at[idx], out_hbm.at[idx], osems.at[blk * (ND // 2) + j])

    def ffn(blk, carry):
        def normed(i):
            rows = pl.ds(pl.multiple_of(blk * (MH // 2), MH // 2), MH // 2)
            return ring[rows, tile(3 * H + i * ND // 2, ND // 2)]

        def up(k, c):
            res = {}, {}
            for t in range(2):
                b1, b2 = (w13[4 * k + 2 * u + t] for u in range(2))
                _strassen(normed,
                          b1[:DH], b2[:DH], b1[DH:], b2[DH:], res[t].setdefault)
            ops = _strassen_lhs(*(_silu(res[0][n]) * res[1][n] for n in range(4)))
            for i in (1, 3, 6, 0, 2, 4, 5):
                act_slot(k, i)[...] = ops[i]
            return c

        lax.fori_loop(0, NF // 2, up, 0, unroll=2)

        def down(j, c):
            emit = functools.partial(residual, xb, pl.multiple_of(blk * FB, FB), j, 5)
            _strassen(lambda i: jnp.concatenate([act_slot(k, i)[...] for k in range(NF // 2)], axis=1),
                      *(row_tiles((2 * j + u) * F, NF, par) for par in range(2) for u in range(2)), emit)
            out_copy(blk, j).start()
            return c

        lax.fori_loop(0, ND // 2, down, 0)
        return carry

    lax.fori_loop(0, S // FB, ffn, 0)
    for blk in range(S // FB):
        for j in range(ND // 2):
            out_copy(blk, j).wait()


@functools.partial(jax.jit, static_argnames=("A_seg_len",))
def pallas_adaLN_cond__memory_aug_recurrent_mem_tr__glu_gated_swiglu__prompt_kernel(
    A_x, A_mem0, A_Wq, A_Wk, A_Wv, A_Wo, A_seg_len, B_x, B_w1, B_w3, B_w2, c, w_mod,
):
    del B_x
    B, S, D = A_x.shape
    _, H, Dh = A_Wq.shape
    M = A_mem0.shape[1]
    F = B_w1.shape[1]
    SEG = int(A_seg_len)
    assert (B, S, D, H, Dh, M, SEG) == (1, 2048, 1024, 32, LANE, 8, 32) and F == 3584
    P = S // SEG * M
    R = 576
    FB = 1024

    hbm = pl.BlockSpec(memory_space=pl.ANY)
    out = pl.pallas_call(
        functools.partial(_kernel, S=S, D=D, H=H, F=F, M=M, SEG=SEG, FB=FB),
        out_shape=jax.ShapeDtypeStruct((S, D), A_x.dtype),
        in_specs=[hbm] * 11,
        out_specs=hbm,
        scratch_shapes=[
            pltpu.VMEM((3 * H * (D // 2 + SLAB_PAD) + D, LANE), U32),
            pltpu.VMEM((D * H // 8, 16, LANE), BF16),
            pltpu.VMEM((2 * F // LANE, D, LANE), BF16),
            pltpu.VMEM((R, 3 * H * Dh + 7 * D // 2), F32),
            pltpu.VMEM((R, H * Dh), F32),
            pltpu.VMEM((S, D), BF16),
            pltpu.VMEM((S, D), F32),
            pltpu.VMEM((6, 8, D), F32),
            pltpu.VMEM((7, P // 2, D // 4), U32),
            pltpu.VMEM((7, P // 4, H * Dh // 2), U32),
            pltpu.VMEM((3 * SEG, LANE), F32),
            pltpu.VMEM((H // 2, M + SEG, LANE), U32),
            pltpu.VMEM((SEG, D), F32),
            pltpu.VMEM((4, SEG, LANE), F32),
            pltpu.VMEM((1, D), c.dtype),
            pltpu.VMEM((M, D), A_mem0.dtype),
            pltpu.SemaphoreType.DMA((9 + 6 * H // 16,)),
            pltpu.SemaphoreType.DMA((S // FB * D // (2 * LANE),)),
        ],
        compiler_params=pltpu.CompilerParams(vmem_limit_bytes=126 * 2**20),
        name="adaln_rmt_swiglu",
    )(A_x.reshape(S, D), A_mem0.reshape(M, D), *(w.reshape(D, H // 16, 16, Dh) for w in (A_Wq, A_Wk, A_Wv)),
      A_Wo.reshape(H * Dh // 16, 16, D), B_w1, B_w3, B_w2.reshape(F // 16, 16, D), c, w_mod)
    return out.reshape(B, S, D)
```

```python
import functools

import jax
import jax.numpy as jnp
from jax import lax
import jax.experimental.pallas as pl
import jax.experimental.pallas.tpu as pltpu

F32 = jnp.float32
BF16 = jnp.bfloat16
U32 = jnp.uint32
LANE = 128
EPS = 1e-5
SLAB_PAD = 4
SCORE_GROUP = 4
SCORE_LAG = 1
VALUE_LAG = 3
FFN_NORM_AT = 7
NEXT_ROWS_AT = 28


def _dot(a, b):
    return jnp.dot(a, b, preferred_element_type=F32)


def _norm(x):
    m = jnp.mean(x, axis=-1, keepdims=True)
    d = x - m
    v = jnp.mean(d * d, axis=-1, keepdims=True)
    return d * lax.rsqrt(v + EPS)


def _ada_ln(x, shift, scale1):
    return _norm(x) * scale1 + shift


def _recip(x):
    return pl.reciprocal(x, approx=True)


def _silu(x):
    return x * _recip(1.0 + jnp.exp(-x))


def _words(x):
    return pltpu.bitcast(x.astype(BF16), U32)


def _strassen_lhs(a11, a12, a21, a22):
    return [_words(a) for a in (a11 + a22, a21 + a22, a11, a22, a11 + a12, a21 - a11, a12 - a22)]


def _strassen(lhs_fn, b11, b12, b21, b22, emit):
    f11, f12, f21, f22 = (b.astype(F32) for b in (b11, b12, b21, b22))

    def prod(i, b):
        return _dot(pltpu.bitcast(lhs_fn(i), BF16), b.astype(BF16))

    m2 = prod(1, b11)
    m4 = prod(3, f21 - f11)
    emit(2, m2 + m4)
    m3 = prod(2, f12 - f22)
    m5 = prod(4, b22)
    emit(1, m3 + m5)
    m1 = prod(0, f11 + f22)
    emit(3, (m1 - m2 + m3) + prod(5, f11 + f12))
    emit(0, (m1 + m4 - m5) + prod(6, f21 + f22))


def _kernel(x_hbm, mem0_hbm, wq_hbm, wk_hbm, wv_hbm, wo_hbm, w1_hbm, w3_hbm, w2_hbm,
            c_hbm, wmod_hbm, out_hbm,
            wqkv, big, w13, ring, oring, xb, xf, mod, hs, ot, fill_ref, prob, acc, early, c_ref, mem0_ref,
            sems, osems,
            *, S, D, H, F, M, SEG, FB):
    NSEG = S // SEG
    XR = SEG - M
    P = S - NSEG * XR
    R = ring.shape[0]
    QOFF = R - P
    OOFF = (-NSEG * XR) % R
    ND = D // LANE
    NF = F // LANE
    HP = H // 2
    HD = H * LANE
    scale = float(LANE) ** -0.5
    DH = D // 2
    PG = 8
    NA = HP // PG
    NSLOT = big.shape[0] // DH
    WP = DH + SLAB_PAD
    WO = ND * HD

    def tile(n, width=1):
        return pl.ds(n * LANE if isinstance(n, int) else pl.multiple_of(n * LANE, LANE), width * LANE)

    def head_slab(n):
        return (n // (2 * PG) * 2 * PG + n % 2 * PG + n % (2 * PG) // 2) * WP

    def slab(row0, rows):
        return big[pl.ds(row0 // 16, rows // 16)].reshape(rows, LANE)

    def slab_copies(src, tiles, dst_fn, sem):
        return [pltpu.make_async_copy(src.at[..., pl.ds(j * LANE, LANE)], dst_fn(j), sem) for j in tiles]

    def half_tiles(c):
        return [v * ND + c * ND // 2 + j for v in range(2) for j in range(ND // 2)]

    cp_x0 = pltpu.make_async_copy(x_hbm.at[pl.ds(0, P)], xb.at[pl.ds(0, P)], sems.at[0])
    cp_x1 = pltpu.make_async_copy(x_hbm.at[pl.ds(P, S - P)], xb.at[pl.ds(P, S - P)], sems.at[1])
    mod_tiles = [half_tiles(0), half_tiles(1), list(range(2 * ND, 6 * ND))]
    cp_mod = [slab_copies(wmod_hbm, t, lambda j: w13.at[j], sems.at[2 + i])
              for i, t in enumerate(mod_tiles)]
    cp_w = [pltpu.make_async_copy(w.at[pl.ds(c * DH, DH), a],
                                  big.at[pl.ds(((2 * t + c) * NA + a) % NSLOT * DH, DH)],
                                  sems.at[7 + (2 * t + c) * NA + a])
            for t, w in enumerate((wq_hbm, wk_hbm, wv_hbm)) for c in range(2) for a in range(NA)]
    cp_o = slab_copies(wo_hbm, range(ND), lambda j: big.at[pl.ds((WO + j * HD) // 16, HD // 16)], sems.at[5])
    cp_ffn = (slab_copies(w1_hbm, range(NF), lambda j: w13.at[2 * j], sems.at[6])
              + slab_copies(w3_hbm, range(NF), lambda j: w13.at[2 * j + 1], sems.at[6])
              + slab_copies(w2_hbm, range(ND), lambda j: big.at[pl.ds(j * F // 16, F // 16)], sems.at[6]))

    def start(cps):
        for cp in cps:
            cp.start()

    def wait(cps):
        for cp in cps:
            cp.wait()

    cp_c = pltpu.make_async_copy(c_hbm, c_ref, sems.at[7 + len(cp_w)])
    cp_mem = pltpu.make_async_copy(mem0_hbm, mem0_ref, sems.at[8 + len(cp_w)])
    cp_c.start()
    start(cp_mod[0])
    cp_x0.start()
    cp_w[0].start()
    cp_mem.start()
    cp_c.wait()

    cc = jnp.broadcast_to(c_ref[...].astype(F32), (16, D))
    sc = _silu(cc).astype(BF16)

    def mod_part(i):
        for j in mod_tiles[i]:
            r = _dot(sc, w13[j])[0:8]
            if j // ND in (1, 4):
                r = r + 1.0
            mod[j // ND, :, pl.ds((j % ND) * LANE, LANE)] = r

    def modv(i):
        return mod[i, 0:1, :]

    G = 2 * (M + SEG)
    ri = lax.broadcasted_iota(jnp.int32, (G, LANE), 0)
    ci = lax.broadcasted_iota(jnp.int32, (G, LANE), 1)

    def head_pos(i):
        head = jnp.where(i < 2 * M, i // M, (i - 2 * M) // SEG)
        pos = jnp.where(i < 2 * M, i % M, M + (i - 2 * M) % SEG)
        return head, pos

    rh, rp = head_pos(ri)
    ch, cp_ = head_pos(ci)
    visible = (rp < M) | (rp >= cp_)
    fill_ref[0:G, :] = jnp.where(rh == ch, jnp.where(visible, 0.0, -1e9), -jnp.inf).astype(F32)

    LB = 128
    PH = P // 2
    DQ = D // 4

    def norm_half(c):
        cols = slice(c * DH, (c + 1) * DH)

        def norm0(k, carry):
            halves = []
            for o in (0, PH):
                rows = pl.ds(pl.multiple_of(o + k * LB, LB), LB)
                if c == 0:
                    xv = xb[rows, :].astype(F32)
                    xf[rows, :] = xv
                    xn = _norm(xv)
                    oring[rows, 0:DH] = xn[:, DH:]
                    xn = xn[:, :DH]
                else:
                    xn = oring[rows, 0:DH]
                halves.append(xn * mod[1, 0:1, cols] + mod[0, 0:1, cols])
            top, bot = halves
            ops = _strassen_lhs(top[:, :DQ], top[:, DQ:], bot[:, :DQ], bot[:, DQ:])
            for i in range(7):
                hs[i, pl.ds(pl.multiple_of(c * (PH // 2) + k * (LB // 2), LB // 2), LB // 2), :] = ops[i]
            return carry

        lax.fori_loop(0, PH // LB, norm0, 0)

    def arrivals(it):
        if it == 0:
            cp_w[0].wait()
            start(cp_w[2:3] + cp_mod[1] + cp_w[3:4])
        else:
            wait(cp_w[it + (it > 1):it + 2])
        if it == 1:
            start(cp_w[4:6])
        if it == NA:
            start(cp_w[6:NSLOT])
            wait(cp_mod[1])
            mod_part(1)
            norm_half(1)
        if it == 4:
            start(cp_w[NSLOT:] + [cp_x1] + cp_mod[2])
        if it == NSLOT - 1:
            wait(cp_w[it + 2:])
            start(cp_o)

    def head_rows(it):
        chunk, a = it // NA, it % NA
        base = (chunk // 2 * H + 2 * PG * a) * WP + chunk % 2 * (DH // 2)
        return wqkv.at[pl.ds(pl.multiple_of(base, 32), (2 * PG + 1) * WP)]

    def retile(it, r0, r1):
        src = big.at[pl.ds(it % NSLOT * DH, DH)]
        dst = head_rows(it)
        for r in range(r0, r1):
            even, odd = pltpu.bitcast(src[2 * r], U32), pltpu.bitcast(src[2 * r + 1], U32)
            dst[pl.ds(r, PG, stride=WP), :] = (even & jnp.uint32(0xFFFF)) | (odd << 16)
            dst[pl.ds(PG * WP + r, PG, stride=WP), :] = (even >> 16) | (odd & jnp.uint32(0xFFFF0000))

    def project(it, carry):
        for ev in range(NSLOT):
            pl.when(it == ev)(functools.partial(arrivals, ev))
        pl.when(it < 2)(lambda: retile(it, 0, DH // 2))
        half = it // NA % 2
        hrows = pl.ds(pl.multiple_of(half * (PH // 2), PH // 2), PH // 2)
        nxt = jnp.where(it == 0, 0, jnp.minimum(it + 1, 6 * NA - 1))
        dst = ring.at[:, tile(it // (2 * NA) * H + 2 * PG * (it % NA), 2 * PG)]
        for b in range(PG):
            lo, hi = (pltpu.bitcast(head_rows(it)[pl.ds((i * PG + b) * WP, DH // 2), :], BF16)
                      for i in range(2))

            def emit(i, r, b=b):
                idx = pl.ds(QOFF + i // 2 * PH, PH), tile(2 * b + i % 2)
                dst[idx] = r + jnp.where(half == 1, dst[idx], 0.0)

            _strassen(lambda i: hs[i, hrows, :], lo[:DQ], hi[:DQ], lo[DQ:], hi[DQ:], emit)
            retile(nxt, b * (DH // 2) // PG, (b + 1) * (DH // 2) // PG)
        return carry

    wait(cp_mod[0])
    mod_part(0)
    cp_x0.wait()
    norm_half(0)
    cp_w[1].start()
    lax.fori_loop(0, 6 * NA, project, 0)

    HG = SEG // 2

    def residual(dst, row0, j, gate, n, y):
        cols = tile(2 * j + n % 2)
        y = mod[gate, 0:1, cols] * y
        for u in range(y.shape[0] // HG):
            rows = pl.ds(row0 + u * SEG + n // 2 * HG, HG)
            dst[rows, cols] = (xf[rows, cols] + y[u * HG:(u + 1) * HG]).astype(dst.dtype)

    def ffn_norm(grp):
        hn = _ada_ln(xf[pl.ds(pl.multiple_of(grp * SEG, SEG), SEG), :], modv(3), modv(4))
        ops = _strassen_lhs(hn[:HG, :DH], hn[:HG, DH:], hn[HG:, :DH], hn[HG:, DH:])
        for i in range(7):
            ring[pl.ds(pl.multiple_of(grp * (HG // 2), HG // 2), HG // 2),
                 tile(3 * H + i * ND // 2, ND // 2)] = pltpu.bitcast(ops[i], F32)

    L0 = S // 4

    def widen(grp):
        rows = pl.ds(pl.multiple_of(grp * SEG, SEG), SEG)
        xf[rows, :] = xb[rows, :].astype(F32)

    def next_rows(r0):
        ring[pl.ds(L0 + M, XR), tile(3 * H, ND)] = _ada_ln(xf[pl.ds(r0, XR), :], modv(0), modv(1))

    wait([cp_mem, cp_x1] + cp_o + cp_mod[2])
    ring[pl.ds(L0, M), tile(3 * H, ND)] = mem0_ref[...].astype(F32)
    widen(P // SEG)
    next_rows(P)
    mod_part(2)
    start(cp_ffn)

    def step(s, carry):
        q_wr = pl.multiple_of(lax.rem(s * XR, R), 8)
        q_rd = pl.multiple_of(lax.rem(s * SEG + QOFF, R), SEG)
        o_wr = pl.multiple_of(lax.rem(s * SEG + OOFF, R), SEG)
        o_rd = pl.multiple_of(lax.rem(s * XR + OOFF, R), 8)
        h = ring[pl.ds(L0, SEG), tile(3 * H, ND)].astype(BF16)
        tail_rows = pl.ds(pl.multiple_of(jnp.maximum(s - NSEG * XR // SEG, 0) * (HG // 2), HG // 2), HG // 2)
        pad = jnp.zeros((LANE - G, LANE), BF16)

        def weights(n, d0, d):
            return pltpu.bitcast(wqkv[pl.ds(head_slab(n) + d0 // 2, d // 2), :], BF16)

        for u in range(4):
            early[u] = _dot(h[:, :DH], weights(u // 2 * H + u % 2, 0, DH))

        def head_pair(t, g):
            n = t * H + 2 * g
            mem_rows = []
            for i in range(2):
                if t < 2 and g == 0:
                    r = _dot(h[:, DH:], weights(n + i, DH, DH)) + early[2 * t + i]
                else:
                    r = _dot(h, weights(n + i, 0, D))
                ring[pl.ds(q_wr, XR), tile(n + i)] = r[M:]
                mem_rows.append(r[:M])
            return jnp.concatenate(
                mem_rows + [ring[pl.ds(q_rd, SEG), tile(n + i)] for i in range(2)],
                axis=0).astype(BF16)

        def scores(q, k):
            sc_ = lax.dot_general(q, jnp.concatenate([k, pad], axis=0), (((1,), (1,)), ((), ())),
                                  preferred_element_type=F32)
            fill = fill_ref[0:G, :]
            sc_ = jnp.where(fill == 0.0, sc_ * scale, fill)
            e = jnp.exp(sc_ - jnp.max(sc_, axis=-1, keepdims=True))
            return (e * _recip(jnp.sum(e, axis=-1, keepdims=True))).astype(BF16)

        def attend(g, p, v):
            o = _dot(p, jnp.concatenate([v, pad], axis=0))
            ops = _strassen_lhs(*(o[2 * M + i * SEG + r:2 * M + i * SEG + r + HG]
                                  for r in (0, HG) for i in range(2)))
            for i in range(7):
                ot[i, tail_rows, pl.ds(g * LANE, LANE)] = ops[i]
            for i in range(2):
                oring[pl.ds(o_wr, SEG), tile(2 * g + i)] = o[2 * M + i * SEG:2 * M + (i + 1) * SEG]
            return [jnp.concatenate([o[i * M:(i + 1) * M], oring[pl.ds(o_rd, XR), tile(2 * g + i)]],
                                    axis=0).astype(BF16) for i in range(2)]

        heads = {}

        def oproj(g0, g1, j0=0, j1=ND):
            a = jnp.concatenate([r for g in range(g0, g1) for r in heads[g]], axis=1)
            for j in range(j0, j1):
                cols = pl.ds(j * LANE, LANE)
                r = _dot(a, slab(WO + j * HD + g0 * 2 * LANE, (g1 - g0) * 2 * LANE))
                if g0 > 0:
                    r = r + acc[:, cols]
                if g1 < HP:
                    acc[:, cols] = r
                else:
                    ring[pl.ds(L0, M), tile(3 * H + j)] = r[:M]
                    xf[rows, cols] = xf[rows, cols] + mod[2, 0:1, cols] * r[M:]

        rows = pl.ds(pl.multiple_of(s * XR, 8), XR)
        qk, val = {}, {}
        for i in range(2 * HP + VALUE_LAG):
            if i == NEXT_ROWS_AT:
                widen(jnp.minimum(P // SEG + 1 + s, NSEG - 1))
                next_rows(pl.multiple_of(jnp.minimum(P + (s + 1) * XR, S - XR), 8))
            if i == FFN_NORM_AT:
                ffn_norm(jnp.maximum(s * XR // SEG - 1, 0))
            if i < HP:
                qk[i] = head_pair(0, i), head_pair(1, i)
            elif i < 2 * HP:
                val[i - HP] = head_pair(2, i - HP)
            else:
                oproj(0, HP // 2, i - 2 * HP, i - 2 * HP + 1)
            g = i - SCORE_LAG
            if g % SCORE_GROUP == 0 and 0 < g <= HP:
                for u in range(g - SCORE_GROUP, g):
                    prob[u] = pltpu.bitcast(scores(*qk[u]), U32)
            g = i - HP - VALUE_LAG
            if g >= 0:
                heads[g] = attend(g, pltpu.bitcast(prob[g], BF16), val[g])
        oproj(0, HP // 2, VALUE_LAG, ND)
        oproj(HP // 2, HP)
        return carry

    lax.fori_loop(0, NSEG, step, 0, unroll=2)

    MH = FB // 2

    def row_tiles(row0, n, par):
        return jnp.concatenate([slab(row0 + (2 * k + par) * LANE, LANE) for k in range(n // 2)], axis=0)

    def otail(j, carry):
        emit = functools.partial(residual, xf, NSEG * XR, j, 2)
        _strassen(lambda i: ot[i],
                  *(row_tiles(WO + (2 * j + u) * HD, H, par) for par in range(2) for u in range(2)), emit)
        return carry

    lax.fori_loop(0, ND // 2, otail, 0)
    G0 = (NSEG - 1) * XR // SEG - 1

    def norm_tail(i, carry):
        for u in range(6):
            ffn_norm(G0 + 6 * i + u)
        return carry

    lax.fori_loop(0, (NSEG - G0) // 6, norm_tail, 0)

    wait(cp_ffn)

    def act_slot(k, i):
        return wqkv.at[pl.ds(pl.multiple_of((7 * k + i) * (MH // 2), MH // 2), MH // 2)]

    def out_copy(blk, j):
        idx = (pl.ds(pl.multiple_of(blk * FB, FB), FB), pl.ds(pl.multiple_of(j * 2 * LANE, 2 * LANE), 2 * LANE))
        return pltpu.make_async_copy(xb.at[idx], out_hbm.at[idx], osems.at[blk * (ND // 2) + j])

    def ffn(blk, carry):
        def normed(i):
            rows = pl.ds(pl.multiple_of(blk * (MH // 2), MH // 2), MH // 2)
            return ring[rows, tile(3 * H + i * ND // 2, ND // 2)]

        def up(k, c):
            res = {}, {}
            for t in range(2):
                b1, b2 = (w13[4 * k + 2 * u + t] for u in range(2))
                _strassen(normed,
                          b1[:DH], b2[:DH], b1[DH:], b2[DH:], res[t].setdefault)
            ops = _strassen_lhs(*(_silu(res[0][n]) * res[1][n] for n in range(4)))
            for i in (1, 3, 6, 0, 2, 4, 5):
                act_slot(k, i)[...] = ops[i]
            return c

        lax.fori_loop(0, NF // 2, up, 0, unroll=2)

        def down(j, c):
            emit = functools.partial(residual, xb, pl.multiple_of(blk * FB, FB), j, 5)
            _strassen(lambda i: jnp.concatenate([act_slot(k, i)[...] for k in range(NF // 2)], axis=1),
                      *(row_tiles((2 * j + u) * F, NF, par) for par in range(2) for u in range(2)), emit)
            out_copy(blk, j).start()
            return c

        lax.fori_loop(0, ND // 2, down, 0)
        return carry

    lax.fori_loop(0, S // FB, ffn, 0)
    for blk in range(S // FB):
        for j in range(ND // 2):
            out_copy(blk, j).wait()


@functools.partial(jax.jit, static_argnames=("A_seg_len",))
def pallas_adaLN_cond__memory_aug_recurrent_mem_tr__glu_gated_swiglu__prompt_kernel(
    A_x, A_mem0, A_Wq, A_Wk, A_Wv, A_Wo, A_seg_len, B_x, B_w1, B_w3, B_w2, c, w_mod,
):
    del B_x
    B, S, D = A_x.shape
    _, H, Dh = A_Wq.shape
    M = A_mem0.shape[1]
    F = B_w1.shape[1]
    SEG = int(A_seg_len)
    assert (B, S, D, H, Dh, M, SEG) == (1, 2048, 1024, 32, LANE, 8, 32) and F == 3584
    P = S // SEG * M
    R = 576
    FB = 1024

    hbm = pl.BlockSpec(memory_space=pl.ANY)
    out = pl.pallas_call(
        functools.partial(_kernel, S=S, D=D, H=H, F=F, M=M, SEG=SEG, FB=FB),
        out_shape=jax.ShapeDtypeStruct((S, D), A_x.dtype),
        in_specs=[hbm] * 11,
        out_specs=hbm,
        scratch_shapes=[
            pltpu.VMEM((3 * H * (D // 2 + SLAB_PAD) + D, LANE), U32),
            pltpu.VMEM((D * H // 8, 16, LANE), BF16),
            pltpu.VMEM((2 * F // LANE, D, LANE), BF16),
            pltpu.VMEM((R, 3 * H * Dh + 7 * D // 2), F32),
            pltpu.VMEM((R, H * Dh), F32),
            pltpu.VMEM((S, D), BF16),
            pltpu.VMEM((S, D), F32),
            pltpu.VMEM((6, 8, D), F32),
            pltpu.VMEM((7, P // 2, D // 4), U32),
            pltpu.VMEM((7, P // 4, H * Dh // 2), U32),
            pltpu.VMEM((3 * SEG, LANE), F32),
            pltpu.VMEM((H // 2, M + SEG, LANE), U32),
            pltpu.VMEM((SEG, D), F32),
            pltpu.VMEM((4, SEG, LANE), F32),
            pltpu.VMEM((1, D), c.dtype),
            pltpu.VMEM((M, D), A_mem0.dtype),
            pltpu.SemaphoreType.DMA((9 + 6 * H // 16,)),
            pltpu.SemaphoreType.DMA((S // FB * D // (2 * LANE),)),
        ],
        compiler_params=pltpu.CompilerParams(vmem_limit_bytes=126 * 2**20),
        name="adaln_rmt_swiglu",
    )(A_x.reshape(S, D), A_mem0.reshape(M, D), *(w.reshape(D, H // 16, 16, Dh) for w in (A_Wq, A_Wk, A_Wv)),
      A_Wo.reshape(H * Dh // 16, 16, D), B_w1, B_w3, B_w2.reshape(F // 16, 16, D), c, w_mod)
    return out.reshape(B, S, D)
```

```python
import functools

import jax
import jax.numpy as jnp
from jax import lax
import jax.experimental.pallas as pl
import jax.experimental.pallas.tpu as pltpu

F32 = jnp.float32
BF16 = jnp.bfloat16
U32 = jnp.uint32
LANE = 128
EPS = 1e-5
SLAB_PAD = 4
SCORE_GROUP = 4
SCORE_LAG = 1
VALUE_LAG = 3
FFN_NORM_AT = 7
NEXT_ROWS_AT = 28


def _dot(a, b):
    return jnp.dot(a, b, preferred_element_type=F32)


def _norm(x):
    m = jnp.mean(x, axis=-1, keepdims=True)
    d = x - m
    v = jnp.mean(d * d, axis=-1, keepdims=True)
    return d * lax.rsqrt(v + EPS)


def _ada_ln(x, shift, scale1):
    return _norm(x) * scale1 + shift


def _recip(x):
    return pl.reciprocal(x, approx=True)


def _silu(x):
    return x * _recip(1.0 + jnp.exp(-x))


def _words(x):
    return pltpu.bitcast(x.astype(BF16), U32)


def _lhs_sums(a11, a12, a21, a22):
    return a11 + a22, a21 + a22, a11, a22, a11 + a12, a21 - a11, a12 - a22


def _strassen_lhs(*blocks):
    return [_words(a) for a in _lhs_sums(*blocks)]


def _quarters(a):
    r, c = a.shape[0] // 2, a.shape[1] // 2
    return a[:r, :c], a[:r, c:], a[r:, :c], a[r:, c:]


def _strassen(lhs_fn, b11, b12, b21, b22, emit, nested=False):
    f11, f12, f21, f22 = (b.astype(F32) for b in (b11, b12, b21, b22))

    def prod(i, b):
        if not nested:
            return _dot(pltpu.bitcast(lhs_fn(i), BF16), b.astype(BF16))
        c = {}
        _strassen(functools.partial(lhs_fn, i), *_quarters(b), c.setdefault)
        return jnp.concatenate([jnp.concatenate([c[0], c[1]], axis=1),
                                jnp.concatenate([c[2], c[3]], axis=1)], axis=0)

    m2 = prod(1, b11)
    m4 = prod(3, f21 - f11)
    emit(2, m2 + m4)
    m3 = prod(2, f12 - f22)
    m5 = prod(4, b22)
    emit(1, m3 + m5)
    m1 = prod(0, f11 + f22)
    emit(3, (m1 - m2 + m3) + prod(5, f11 + f12))
    emit(0, (m1 + m4 - m5) + prod(6, f21 + f22))


def _kernel(x_hbm, mem0_hbm, wq_hbm, wk_hbm, wv_hbm, wo_hbm, w1_hbm, w3_hbm, w2_hbm,
            c_hbm, wmod_hbm, out_hbm,
            wqkv, big, w13, ring, oring, xb, xf, mod, hs, ot, fill_ref, prob, acc, early, c_ref, mem0_ref,
            sems, osems,
            *, S, D, H, F, M, SEG, FB):
    NSEG = S // SEG
    XR = SEG - M
    P = S - NSEG * XR
    R = ring.shape[0]
    QOFF = R - P
    OOFF = (-NSEG * XR) % R
    ND = D // LANE
    NF = F // LANE
    HP = H // 2
    HD = H * LANE
    scale = float(LANE) ** -0.5
    DH = D // 2
    PG = 8
    NA = HP // PG
    NSLOT = big.shape[0] // DH
    WP = DH + SLAB_PAD
    WO = ND * HD

    def tile(n, width=1):
        return pl.ds(n * LANE if isinstance(n, int) else pl.multiple_of(n * LANE, LANE), width * LANE)

    def head_slab(n):
        return (n // (2 * PG) * 2 * PG + n % 2 * PG + n % (2 * PG) // 2) * WP

    def slab(row0, rows):
        return big[pl.ds(row0 // 16, rows // 16)].reshape(rows, LANE)

    def slab_copies(src, tiles, dst_fn, sem):
        return [pltpu.make_async_copy(src.at[..., pl.ds(j * LANE, LANE)], dst_fn(j), sem) for j in tiles]

    def half_tiles(c):
        return [v * ND + c * ND // 2 + j for v in range(2) for j in range(ND // 2)]

    cp_x0 = pltpu.make_async_copy(x_hbm.at[pl.ds(0, P)], xb.at[pl.ds(0, P)], sems.at[0])
    cp_x1 = pltpu.make_async_copy(x_hbm.at[pl.ds(P, S - P)], xb.at[pl.ds(P, S - P)], sems.at[1])
    mod_tiles = [half_tiles(0), half_tiles(1), list(range(2 * ND, 6 * ND))]
    cp_mod = [slab_copies(wmod_hbm, t, lambda j: w13.at[j], sems.at[2 + i])
              for i, t in enumerate(mod_tiles)]
    cp_w = [pltpu.make_async_copy(w.at[pl.ds(c * DH, DH), a],
                                  big.at[pl.ds(((2 * t + c) * NA + a) % NSLOT * DH, DH)],
                                  sems.at[7 + (2 * t + c) * NA + a])
            for t, w in enumerate((wq_hbm, wk_hbm, wv_hbm)) for c in range(2) for a in range(NA)]
    cp_o = slab_copies(wo_hbm, range(ND), lambda j: big.at[pl.ds((WO + j * HD) // 16, HD // 16)], sems.at[5])
    cp_ffn = (slab_copies(w1_hbm, range(NF), lambda j: w13.at[2 * j], sems.at[6])
              + slab_copies(w3_hbm, range(NF), lambda j: w13.at[2 * j + 1], sems.at[6])
              + slab_copies(w2_hbm, range(ND), lambda j: big.at[pl.ds(j * F // 16, F // 16)], sems.at[6]))

    def start(cps):
        for cp in cps:
            cp.start()

    def wait(cps):
        for cp in cps:
            cp.wait()

    cp_c = pltpu.make_async_copy(c_hbm, c_ref, sems.at[7 + len(cp_w)])
    cp_mem = pltpu.make_async_copy(mem0_hbm, mem0_ref, sems.at[8 + len(cp_w)])
    cp_c.start()
    start(cp_mod[0])
    cp_x0.start()
    cp_w[0].start()
    cp_mem.start()
    cp_c.wait()

    cc = jnp.broadcast_to(c_ref[...].astype(F32), (16, D))
    sc = _silu(cc).astype(BF16)

    def mod_part(i):
        for j in mod_tiles[i]:
            r = _dot(sc, w13[j])[0:8]
            if j // ND in (1, 4):
                r = r + 1.0
            mod[j // ND, :, pl.ds((j % ND) * LANE, LANE)] = r

    def modv(i):
        return mod[i, 0:1, :]

    G = 2 * (M + SEG)
    ri = lax.broadcasted_iota(jnp.int32, (G, LANE), 0)
    ci = lax.broadcasted_iota(jnp.int32, (G, LANE), 1)

    def head_pos(i):
        head = jnp.where(i < 2 * M, i // M, (i - 2 * M) // SEG)
        pos = jnp.where(i < 2 * M, i % M, M + (i - 2 * M) % SEG)
        return head, pos

    rh, rp = head_pos(ri)
    ch, cp_ = head_pos(ci)
    visible = (rp < M) | (rp >= cp_)
    fill_ref[0:G, :] = jnp.where(rh == ch, jnp.where(visible, 0.0, -1e9), -jnp.inf).astype(F32)

    LB = 128
    PH = P // 2
    DQ = D // 4

    def norm_half(c):
        cols = slice(c * DH, (c + 1) * DH)

        def norm0(k, carry):
            halves = []
            for o in (0, PH):
                rows = pl.ds(pl.multiple_of(o + k * LB, LB), LB)
                if c == 0:
                    xv = xb[rows, :].astype(F32)
                    xf[rows, :] = xv
                    xn = _norm(xv)
                    oring[rows, 0:DH] = xn[:, DH:]
                    xn = xn[:, :DH]
                else:
                    xn = oring[rows, 0:DH]
                halves.append(xn * mod[1, 0:1, cols] + mod[0, 0:1, cols])
            top, bot = halves
            ops = _strassen_lhs(top[:, :DQ], top[:, DQ:], bot[:, :DQ], bot[:, DQ:])
            for i in range(7):
                hs[i, pl.ds(pl.multiple_of(c * (PH // 2) + k * (LB // 2), LB // 2), LB // 2), :] = ops[i]
            return carry

        lax.fori_loop(0, PH // LB, norm0, 0)

    def arrivals(it):
        if it == 0:
            cp_w[0].wait()
            start(cp_w[2:3] + cp_mod[1] + cp_w[3:4])
        else:
            wait(cp_w[it + (it > 1):it + 2])
        if it == 1:
            start(cp_w[4:6])
        if it == NA:
            start(cp_w[6:NSLOT])
            wait(cp_mod[1])
            mod_part(1)
            norm_half(1)
        if it == 4:
            start(cp_w[NSLOT:] + [cp_x1] + cp_mod[2])
        if it == NSLOT - 1:
            wait(cp_w[it + 2:])
            start(cp_o)

    def head_rows(it):
        chunk, a = it // NA, it % NA
        base = (chunk // 2 * H + 2 * PG * a) * WP + chunk % 2 * (DH // 2)
        return wqkv.at[pl.ds(pl.multiple_of(base, 32), (2 * PG + 1) * WP)]

    def retile(it, r0, r1):
        src = big.at[pl.ds(it % NSLOT * DH, DH)]
        dst = head_rows(it)
        for r in range(r0, r1):
            even, odd = pltpu.bitcast(src[2 * r], U32), pltpu.bitcast(src[2 * r + 1], U32)
            dst[pl.ds(r, PG, stride=WP), :] = (even & jnp.uint32(0xFFFF)) | (odd << 16)
            dst[pl.ds(PG * WP + r, PG, stride=WP), :] = (even >> 16) | (odd & jnp.uint32(0xFFFF0000))

    def project(it, carry):
        for ev in range(NSLOT):
            pl.when(it == ev)(functools.partial(arrivals, ev))
        pl.when(it < 2)(lambda: retile(it, 0, DH // 2))
        half = it // NA % 2
        hrows = pl.ds(pl.multiple_of(half * (PH // 2), PH // 2), PH // 2)
        nxt = jnp.where(it == 0, 0, jnp.minimum(it + 1, 6 * NA - 1))
        dst = ring.at[:, tile(it // (2 * NA) * H + 2 * PG * (it % NA), 2 * PG)]
        for b in range(PG):
            lo, hi = (pltpu.bitcast(head_rows(it)[pl.ds((i * PG + b) * WP, DH // 2), :], BF16)
                      for i in range(2))

            def emit(i, r, b=b):
                idx = pl.ds(QOFF + i // 2 * PH, PH), tile(2 * b + i % 2)
                dst[idx] = r + jnp.where(half == 1, dst[idx], 0.0)

            _strassen(lambda i: hs[i, hrows, :], lo[:DQ], hi[:DQ], lo[DQ:], hi[DQ:], emit)
            retile(nxt, b * (DH // 2) // PG, (b + 1) * (DH // 2) // PG)
        return carry

    wait(cp_mod[0])
    mod_part(0)
    cp_x0.wait()
    norm_half(0)
    cp_w[1].start()
    lax.fori_loop(0, 6 * NA, project, 0)

    HG = SEG // 2

    def residual(dst, row0, parts, j, gate, n, y):
        cols = tile(2 * j + n % 2)
        y = mod[gate, 0:1, cols] * y
        for u in range(y.shape[0] // HG):
            per = y.shape[0] // HG // parts
            rows = pl.ds(row0 + (u % per * parts + u // per) * SEG + n // 2 * HG, HG)
            dst[rows, cols] = (xf[rows, cols] + y[u * HG:(u + 1) * HG]).astype(dst.dtype)

    NG = FB // (2 * SEG)

    def ffn_operands(blk):
        return ring.at[:, tile((1 - blk) * 3 * H, 7 * ND // 2)]

    def operand_at(i, j, rows):
        m = 7 * i + j
        return pl.ds(m % 4 * (FB // 8), rows), tile(m // 4 * 2, 2)

    def ffn_norm(blk, grp):
        hn = _ada_ln(xf[pl.ds(pl.multiple_of(blk * FB + grp * 2 * SEG, 2 * SEG), 2 * SEG), :],
                     modv(3), modv(4))
        hn = jnp.concatenate([hn[q * HG:(q + 1) * HG] for q in (0, 2, 1, 3)], axis=0)
        dst = ffn_operands(blk).at[pl.ds(pl.multiple_of(grp * (HG // 2), HG // 2), 3 * FB // 8 + HG // 2)]
        for i, a in enumerate(_lhs_sums(*_quarters(hn))):
            for j, op in enumerate(_strassen_lhs(*_quarters(a))):
                dst[operand_at(i, j, HG // 2)] = pltpu.bitcast(op, F32)

    L0 = S // 4

    def widen(grp):
        rows = pl.ds(pl.multiple_of(grp * SEG, SEG), SEG)
        xf[rows, :] = xb[rows, :].astype(F32)

    def next_rows(r0):
        ring[pl.ds(L0 + M, XR), tile(3 * H, ND)] = _ada_ln(xf[pl.ds(r0, XR), :], modv(0), modv(1))

    wait([cp_mem, cp_x1] + cp_o + cp_mod[2])
    ring[pl.ds(L0, M), tile(3 * H, ND)] = mem0_ref[...].astype(F32)
    widen(P // SEG)
    next_rows(P)
    mod_part(2)
    start(cp_ffn)

    def step(s, with_norm):
        q_wr = pl.multiple_of(lax.rem(s * XR, R), 8)
        q_rd = pl.multiple_of(lax.rem(s * SEG + QOFF, R), SEG)
        o_wr = pl.multiple_of(lax.rem(s * SEG + OOFF, R), SEG)
        o_rd = pl.multiple_of(lax.rem(s * XR + OOFF, R), 8)
        h = ring[pl.ds(L0, SEG), tile(3 * H, ND)].astype(BF16)
        tail_rows = pl.ds(pl.multiple_of(jnp.maximum(s - NSEG * XR // SEG, 0) * (HG // 2), HG // 2), HG // 2)
        pad = jnp.zeros((LANE - G, LANE), BF16)

        def weights(n, d0, d):
            return pltpu.bitcast(wqkv[pl.ds(head_slab(n) + d0 // 2, d // 2), :], BF16)

        for u in range(4):
            early[u] = _dot(h[:, :DH], weights(u // 2 * H + u % 2, 0, DH))

        def head_pair(t, g):
            n = t * H + 2 * g
            mem_rows = []
            for i in range(2):
                if t < 2 and g == 0:
                    r = _dot(h[:, DH:], weights(n + i, DH, DH)) + early[2 * t + i]
                else:
                    r = _dot(h, weights(n + i, 0, D))
                ring[pl.ds(q_wr, XR), tile(n + i)] = r[M:]
                mem_rows.append(r[:M])
            return jnp.concatenate(
                mem_rows + [ring[pl.ds(q_rd, SEG), tile(n + i)] for i in range(2)],
                axis=0).astype(BF16)

        def scores(q, k):
            sc_ = lax.dot_general(q, jnp.concatenate([k, pad], axis=0), (((1,), (1,)), ((), ())),
                                  preferred_element_type=F32)
            fill = fill_ref[0:G, :]
            sc_ = jnp.where(fill == 0.0, sc_ * scale, fill)
            e = jnp.exp(sc_ - jnp.max(sc_, axis=-1, keepdims=True))
            return (e * _recip(jnp.sum(e, axis=-1, keepdims=True))).astype(BF16)

        def attend(g, p, v):
            o = _dot(p, jnp.concatenate([v, pad], axis=0))
            ops = _strassen_lhs(*(o[2 * M + i * SEG + r:2 * M + i * SEG + r + HG]
                                  for r in (0, HG) for i in range(2)))
            for i in range(7):
                ot[i, tail_rows, pl.ds(g * LANE, LANE)] = ops[i]
            for i in range(2):
                oring[pl.ds(o_wr, SEG), tile(2 * g + i)] = o[2 * M + i * SEG:2 * M + (i + 1) * SEG]
            return [jnp.concatenate([o[i * M:(i + 1) * M], oring[pl.ds(o_rd, XR), tile(2 * g + i)]],
                                    axis=0).astype(BF16) for i in range(2)]

        heads = {}

        def oproj(g0, g1, j0=0, j1=ND):
            a = jnp.concatenate([r for g in range(g0, g1) for r in heads[g]], axis=1)
            for j in range(j0, j1):
                cols = pl.ds(j * LANE, LANE)
                r = _dot(a, slab(WO + j * HD + g0 * 2 * LANE, (g1 - g0) * 2 * LANE))
                if g0 > 0:
                    r = r + acc[:, cols]
                if g1 < HP:
                    acc[:, cols] = r
                else:
                    ring[pl.ds(L0, M), tile(3 * H + j)] = r[:M]
                    xf[rows, cols] = xf[rows, cols] + mod[2, 0:1, cols] * r[M:]

        rows = pl.ds(pl.multiple_of(s * XR, 8), XR)
        qk, val = {}, {}
        for i in range(2 * HP + VALUE_LAG):
            if i == NEXT_ROWS_AT:
                widen(jnp.minimum(P // SEG + 1 + s, NSEG - 1))
                next_rows(pl.multiple_of(jnp.minimum(P + (s + 1) * XR, S - XR), 8))
            if i == FFN_NORM_AT and with_norm:
                ffn_norm(0, jnp.clip(s * XR // (2 * SEG) - 1, 0, NG - 1))
            if i < HP:
                qk[i] = head_pair(0, i), head_pair(1, i)
            elif i < 2 * HP:
                val[i - HP] = head_pair(2, i - HP)
            else:
                oproj(0, HP // 2, i - 2 * HP, i - 2 * HP + 1)
            g = i - SCORE_LAG
            if g % SCORE_GROUP == 0 and 0 < g <= HP:
                for u in range(g - SCORE_GROUP, g):
                    prob[u] = pltpu.bitcast(scores(*qk[u]), U32)
            g = i - HP - VALUE_LAG
            if g >= 0:
                heads[g] = attend(g, pltpu.bitcast(prob[g], BF16), val[g])
        oproj(0, HP // 2, VALUE_LAG, ND)
        oproj(HP // 2, HP)

    def step_pair(i, carry):
        step(2 * i, True)
        step(2 * i + 1, False)
        return carry

    lax.fori_loop(0, NSEG // 2, step_pair, 0)

    MH = FB // 2

    def row_tiles(row0, n, par, rows=LANE):
        return jnp.concatenate([slab(row0 + (2 * k + par) * rows, rows) for k in range(n // 2)], axis=0)

    def otail(j, carry):
        for u in range(2):
            ffn_norm(1, 2 * j + u)
        emit = functools.partial(residual, xf, NSEG * XR, 1, j, 2)
        _strassen(lambda i: ot[i],
                  *(row_tiles(WO + (2 * j + u) * HD, H, par) for par in range(2) for u in range(2)), emit)
        return carry

    lax.fori_loop(0, ND // 2, otail, 0)

    def norm_tail(i, carry):
        for u in range(4):
            ffn_norm(1, NG // 2 + 4 * i + u)
        return carry

    lax.fori_loop(0, NG // 8, norm_tail, 0)

    wait(cp_ffn)

    def act_slot(k, i):
        return wqkv[pl.ds((7 * k + i) * (MH // 2), MH // 2), :]

    def out_copy(blk, j):
        idx = (pl.ds(pl.multiple_of(blk * FB, FB), FB), pl.ds(pl.multiple_of(j * 2 * LANE, 2 * LANE), 2 * LANE))
        return pltpu.make_async_copy(xb.at[idx], out_hbm.at[idx], osems.at[blk * (ND // 2) + j])

    def ffn(blk, carry):
        def normed(i, j):
            return ffn_operands(blk)[operand_at(i, j, FB // 8)]

        def up(k, c):
            dst = wqkv.at[pl.ds(pl.multiple_of(k * 7 * MH, MH), 7 * MH)]
            res = {}, {}
            for t in range(2):
                w = jnp.concatenate([w13[8 * k + 2 * u + t] for u in range(4)], axis=1)
                _strassen(normed, *_quarters(w), res[t].setdefault, nested=True)
            ops = _strassen_lhs(*(_silu(res[0][n]) * res[1][n] for n in range(4)))
            for i in (1, 3, 6, 0, 2, 4, 5):
                for u in range(2):
                    dst[pl.ds((7 * u + i) * (MH // 2), MH // 2), :] = ops[i][:, u * LANE:(u + 1) * LANE]
            return c

        lax.fori_loop(0, NF // 4, up, 0)

        def down(j, c):
            emit = functools.partial(residual, xb, pl.multiple_of(blk * FB, FB), 2, j, 5)
            _strassen(lambda i: jnp.concatenate([act_slot(k, i) for k in range(NF // 2)], axis=1),
                      *(row_tiles((2 * j + u) * F, NF // 2, par, 2 * LANE) for par in range(2) for u in range(2)), emit)
            out_copy(blk, j).start()
            return c

        lax.fori_loop(0, ND // 2, down, 0)
        return carry

    lax.fori_loop(0, S // FB, ffn, 0)
    for blk in range(S // FB):
        for j in range(ND // 2):
            out_copy(blk, j).wait()


@functools.partial(jax.jit, static_argnames=("A_seg_len",))
def pallas_adaLN_cond__memory_aug_recurrent_mem_tr__glu_gated_swiglu__prompt_kernel(
    A_x, A_mem0, A_Wq, A_Wk, A_Wv, A_Wo, A_seg_len, B_x, B_w1, B_w3, B_w2, c, w_mod,
):
    del B_x
    B, S, D = A_x.shape
    _, H, Dh = A_Wq.shape
    M = A_mem0.shape[1]
    F = B_w1.shape[1]
    SEG = int(A_seg_len)
    assert (B, S, D, H, Dh, M, SEG) == (1, 2048, 1024, 32, LANE, 8, 32) and F == 3584
    P = S // SEG * M
    R = 576
    FB = 1024

    hbm = pl.BlockSpec(memory_space=pl.ANY)
    out = pl.pallas_call(
        functools.partial(_kernel, S=S, D=D, H=H, F=F, M=M, SEG=SEG, FB=FB),
        out_shape=jax.ShapeDtypeStruct((S, D), A_x.dtype),
        in_specs=[hbm] * 11,
        out_specs=hbm,
        scratch_shapes=[
            pltpu.VMEM((3 * H * (D // 2 + SLAB_PAD) + D, LANE), U32),
            pltpu.VMEM((D * H // 8, 16, LANE), BF16),
            pltpu.VMEM((2 * F // LANE, D, LANE), BF16),
            pltpu.VMEM((R, 3 * H * Dh + 7 * D // 2), F32),
            pltpu.VMEM((R, H * Dh), F32),
            pltpu.VMEM((S, D), BF16),
            pltpu.VMEM((S, D), F32),
            pltpu.VMEM((6, 8, D), F32),
            pltpu.VMEM((7, P // 2, D // 4), U32),
            pltpu.VMEM((7, P // 4, H * Dh // 2), U32),
            pltpu.VMEM((3 * SEG, LANE), F32),
            pltpu.VMEM((H // 2, M + SEG, LANE), U32),
            pltpu.VMEM((SEG, D), F32),
            pltpu.VMEM((4, SEG, LANE), F32),
            pltpu.VMEM((1, D), c.dtype),
            pltpu.VMEM((M, D), A_mem0.dtype),
            pltpu.SemaphoreType.DMA((9 + 6 * H // 16,)),
            pltpu.SemaphoreType.DMA((S // FB * D // (2 * LANE),)),
        ],
        compiler_params=pltpu.CompilerParams(vmem_limit_bytes=127 * 2**20),
        name="adaln_rmt_swiglu",
    )(A_x.reshape(S, D), A_mem0.reshape(M, D), *(w.reshape(D, H // 16, 16, Dh) for w in (A_Wq, A_Wk, A_Wv)),
      A_Wo.reshape(H * Dh // 16, 16, D), B_w1, B_w3, B_w2.reshape(F // 16, 16, D), c, w_mod)
    return out.reshape(B, S, D)
```

```python
import functools

import jax
import jax.numpy as jnp
from jax import lax
import jax.experimental.pallas as pl
import jax.experimental.pallas.tpu as pltpu

F32 = jnp.float32
BF16 = jnp.bfloat16
U32 = jnp.uint32
LANE = 128
EPS = 1e-5
SLAB_PAD = 4
SCORE_GROUP = 4
SCORE_LAG = 2
VALUE_LAG = 3
FFN_NORM_AT = 24
NEXT_ROWS_AT = 18


def _dot(a, b):
    return jnp.dot(a, b, preferred_element_type=F32)


def _norm(x):
    m = jnp.mean(x, axis=-1, keepdims=True)
    d = x - m
    v = jnp.mean(d * d, axis=-1, keepdims=True)
    return d * lax.rsqrt(v + EPS)


def _ada_ln(x, shift, scale1):
    return _norm(x) * scale1 + shift


def _recip(x):
    return pl.reciprocal(x, approx=True)


def _silu(x):
    return x * _recip(1.0 + jnp.exp(-x))


def _words(x):
    return pltpu.bitcast(x.astype(BF16), U32)


def _lhs_sums(a11, a12, a21, a22):
    return a11 + a22, a21 + a22, a11, a22, a11 + a12, a21 - a11, a12 - a22


def _strassen_lhs(*blocks):
    return [_words(a) for a in _lhs_sums(*blocks)]


def _quarters(a):
    r, c = a.shape[0] // 2, a.shape[1] // 2
    return a[:r, :c], a[:r, c:], a[r:, :c], a[r:, c:]


def _strassen(lhs_fn, b11, b12, b21, b22, emit, nested=False):
    f11, f12, f21, f22 = (b.astype(F32) for b in (b11, b12, b21, b22))

    def prod(i, b):
        if not nested:
            return _dot(pltpu.bitcast(lhs_fn(i), BF16), b.astype(BF16))
        c = {}
        _strassen(functools.partial(lhs_fn, i), *_quarters(b), c.setdefault)
        return jnp.concatenate([jnp.concatenate([c[0], c[1]], axis=1),
                                jnp.concatenate([c[2], c[3]], axis=1)], axis=0)

    m2 = prod(1, b11)
    m4 = prod(3, f21 - f11)
    emit(2, m2 + m4)
    m3 = prod(2, f12 - f22)
    m5 = prod(4, b22)
    emit(1, m3 + m5)
    m1 = prod(0, f11 + f22)
    emit(3, (m1 - m2 + m3) + prod(5, f11 + f12))
    emit(0, (m1 + m4 - m5) + prod(6, f21 + f22))


def _kernel(x_hbm, mem0_hbm, wq_hbm, wk_hbm, wv_hbm, wo_hbm, w1_hbm, w3_hbm, w2_hbm,
            c_hbm, wmod_hbm, out_hbm,
            wqkv, big, w13, ring, oring, xb, xf, mod, hs, ot, fill_ref, prob, acc, early, c_ref, mem0_ref,
            sems, osems,
            *, S, D, H, F, M, SEG, FB):
    NSEG = S // SEG
    XR = SEG - M
    P = S - NSEG * XR
    R = ring.shape[0]
    QOFF = R - P
    OOFF = (-NSEG * XR) % R
    ND = D // LANE
    NF = F // LANE
    HP = H // 2
    HD = H * LANE
    scale = float(LANE) ** -0.5
    DH = D // 2
    PG = 8
    NA = HP // PG
    NSLOT = big.shape[0] // DH
    WP = DH + SLAB_PAD
    WO = ND * HD

    def tile(n, width=1):
        return pl.ds(n * LANE if isinstance(n, int) else pl.multiple_of(n * LANE, LANE), width * LANE)

    def head_slab(n):
        return (n // (2 * PG) * 2 * PG + n % 2 * PG + n % (2 * PG) // 2) * WP

    def slab(row0, rows):
        return big[pl.ds(row0 // 16, rows // 16)].reshape(rows, LANE)

    def slab_copies(src, tiles, dst_fn, sem):
        return [pltpu.make_async_copy(src.at[..., pl.ds(j * LANE, LANE)], dst_fn(j), sem) for j in tiles]

    def half_tiles(c):
        return [v * ND + c * ND // 2 + j for v in range(2) for j in range(ND // 2)]

    cp_x0 = pltpu.make_async_copy(x_hbm.at[pl.ds(0, P)], xb.at[pl.ds(0, P)], sems.at[0])
    cp_x1 = pltpu.make_async_copy(x_hbm.at[pl.ds(P, S - P)], xb.at[pl.ds(P, S - P)], sems.at[1])
    mod_tiles = [half_tiles(0), half_tiles(1), list(range(2 * ND, 6 * ND))]
    cp_mod = [slab_copies(wmod_hbm, t, lambda j: w13.at[j], sems.at[2 + i])
              for i, t in enumerate(mod_tiles)]
    cp_w = [pltpu.make_async_copy(w.at[pl.ds(c * DH, DH), a],
                                  big.at[pl.ds(((2 * t + c) * NA + a) % NSLOT * DH, DH)],
                                  sems.at[7 + (2 * t + c) * NA + a])
            for t, w in enumerate((wq_hbm, wk_hbm, wv_hbm)) for c in range(2) for a in range(NA)]
    cp_o = slab_copies(wo_hbm, range(ND), lambda j: big.at[pl.ds((WO + j * HD) // 16, HD // 16)], sems.at[5])
    cp_ffn = (slab_copies(w1_hbm, range(NF), lambda j: w13.at[2 * j], sems.at[6])
              + slab_copies(w3_hbm, range(NF), lambda j: w13.at[2 * j + 1], sems.at[6])
              + slab_copies(w2_hbm, range(ND), lambda j: big.at[pl.ds(j * F // 16, F // 16)], sems.at[6]))

    def start(cps):
        for cp in cps:
            cp.start()

    def wait(cps):
        for cp in cps:
            cp.wait()

    cp_c = pltpu.make_async_copy(c_hbm, c_ref, sems.at[7 + len(cp_w)])
    cp_mem = pltpu.make_async_copy(mem0_hbm, mem0_ref, sems.at[8 + len(cp_w)])
    cp_c.start()
    start(cp_mod[0])
    cp_x0.start()
    cp_w[0].start()
    cp_mem.start()
    cp_c.wait()

    cc = jnp.broadcast_to(c_ref[...].astype(F32), (16, D))
    sc = _silu(cc).astype(BF16)

    def mod_part(i):
        for j in mod_tiles[i]:
            r = _dot(sc, w13[j])[0:8]
            if j // ND in (1, 4):
                r = r + 1.0
            mod[j // ND, :, pl.ds((j % ND) * LANE, LANE)] = r

    def modv(i):
        return mod[i, 0:1, :]

    G = 2 * (M + SEG)
    ri = lax.broadcasted_iota(jnp.int32, (G, LANE), 0)
    ci = lax.broadcasted_iota(jnp.int32, (G, LANE), 1)

    def head_pos(i):
        head = jnp.where(i < 2 * M, i // M, (i - 2 * M) // SEG)
        pos = jnp.where(i < 2 * M, i % M, M + (i - 2 * M) % SEG)
        return head, pos

    rh, rp = head_pos(ri)
    ch, cp_ = head_pos(ci)
    visible = (rp < M) | (rp >= cp_)
    fill_ref[0:G, :] = jnp.where(rh == ch, jnp.where(visible, 0.0, -1e9), -jnp.inf).astype(F32)

    LB = 128
    PH = P // 2
    DQ = D // 4

    def norm_half(c):
        cols = slice(c * DH, (c + 1) * DH)

        def norm0(k, carry):
            halves = []
            for o in (0, PH):
                rows = pl.ds(pl.multiple_of(o + k * LB, LB), LB)
                if c == 0:
                    xv = xb[rows, :].astype(F32)
                    xf[rows, :] = xv
                    xn = _norm(xv)
                    oring[rows, 0:DH] = xn[:, DH:]
                    xn = xn[:, :DH]
                else:
                    xn = oring[rows, 0:DH]
                halves.append(xn * mod[1, 0:1, cols] + mod[0, 0:1, cols])
            top, bot = halves
            ops = _strassen_lhs(top[:, :DQ], top[:, DQ:], bot[:, :DQ], bot[:, DQ:])
            for i in range(7):
                hs[i, pl.ds(pl.multiple_of(c * (PH // 2) + k * (LB // 2), LB // 2), LB // 2), :] = ops[i]
            return carry

        lax.fori_loop(0, PH // LB, norm0, 0)

    def arrivals(it):
        if it == 0:
            cp_w[0].wait()
            start(cp_w[2:3] + cp_mod[1] + cp_w[3:4])
        else:
            wait(cp_w[it + (it > 1):it + 2])
        if it == 1:
            start(cp_w[4:6])
        if it == NA:
            start(cp_w[6:NSLOT])
            wait(cp_mod[1])
            mod_part(1)
            norm_half(1)
        if it == 4:
            start(cp_w[NSLOT:] + [cp_x1] + cp_mod[2])
        if it == NSLOT - 1:
            wait(cp_w[it + 2:])
            start(cp_o)

    def head_rows(it):
        chunk, a = it // NA, it % NA
        base = (chunk // 2 * H + 2 * PG * a) * WP + chunk % 2 * (DH // 2)
        return wqkv.at[pl.ds(pl.multiple_of(base, 32), (2 * PG + 1) * WP)]

    def retile(it, r0, r1):
        src = big.at[pl.ds(it % NSLOT * DH, DH)]
        dst = head_rows(it)
        for r in range(r0, r1):
            even, odd = pltpu.bitcast(src[2 * r], U32), pltpu.bitcast(src[2 * r + 1], U32)
            dst[pl.ds(r, PG, stride=WP), :] = (even & jnp.uint32(0xFFFF)) | (odd << 16)
            dst[pl.ds(PG * WP + r, PG, stride=WP), :] = (even >> 16) | (odd & jnp.uint32(0xFFFF0000))

    def project(it, carry):
        for ev in range(NSLOT):
            pl.when(it == ev)(functools.partial(arrivals, ev))
        pl.when(it < 2)(lambda: retile(it, 0, DH // 2))
        half = it // NA % 2
        hrows = pl.ds(pl.multiple_of(half * (PH // 2), PH // 2), PH // 2)
        nxt = jnp.where(it == 0, 0, jnp.minimum(it + 1, 6 * NA - 1))
        dst = ring.at[:, tile(it // (2 * NA) * H + 2 * PG * (it % NA), 2 * PG)]
        for b in range(PG):
            lo, hi = (pltpu.bitcast(head_rows(it)[pl.ds((i * PG + b) * WP, DH // 2), :], BF16)
                      for i in range(2))

            def emit(i, r, b=b):
                idx = pl.ds(QOFF + i // 2 * PH, PH), tile(2 * b + i % 2)
                dst[idx] = r + jnp.where(half == 1, dst[idx], 0.0)

            _strassen(lambda i: hs[i, hrows, :], lo[:DQ], hi[:DQ], lo[DQ:], hi[DQ:], emit)
            retile(nxt, b * (DH // 2) // PG, (b + 1) * (DH // 2) // PG)
        return carry

    wait(cp_mod[0])
    mod_part(0)
    cp_x0.wait()
    norm_half(0)
    cp_w[1].start()
    lax.fori_loop(0, 6 * NA, project, 0)

    HG = SEG // 2

    def residual(dst, row0, parts, j, gate, n, y):
        cols = tile(2 * j + n % 2)
        y = mod[gate, 0:1, cols] * y
        per = y.shape[0] // HG // parts
        for u in range(per * parts):
            rows = pl.ds(row0 + (u % per * parts + u // per) * SEG + n // 2 * HG, HG)
            dst[rows, cols] = (xf[rows, cols] + y[u * HG:(u + 1) * HG]).astype(dst.dtype)

    NG = FB // (2 * SEG)

    def ffn_operands(blk):
        return ring.at[:, tile((1 - blk) * 3 * H, 7 * ND // 2)]

    def operand_at(i, j, rows):
        m = 7 * i + j
        return pl.ds(m % 4 * (FB // 8), rows), tile(m // 4 * 2, 2)

    def ffn_norm(blk, grp):
        hn = _ada_ln(xf[pl.ds(pl.multiple_of(blk * FB + grp * 2 * SEG, 2 * SEG), 2 * SEG), :],
                     modv(3), modv(4))
        hn = jnp.concatenate([hn[q * HG:(q + 1) * HG] for q in (0, 2, 1, 3)], axis=0)
        dst = ffn_operands(blk).at[pl.ds(pl.multiple_of(grp * (HG // 2), HG // 2), 3 * FB // 8 + HG // 2)]
        for i, a in enumerate(_lhs_sums(*_quarters(hn))):
            for j, op in enumerate(_strassen_lhs(*_quarters(a))):
                dst[operand_at(i, j, HG // 2)] = pltpu.bitcast(op, F32)

    L0 = S // 4

    def widen(grp):
        rows = pl.ds(pl.multiple_of(grp * SEG, SEG), SEG)
        xf[rows, :] = xb[rows, :].astype(F32)

    def next_rows(r0):
        ring[pl.ds(L0 + M, XR), tile(3 * H, ND)] = _ada_ln(xf[pl.ds(r0, XR), :], modv(0), modv(1))

    wait([cp_mem, cp_x1] + cp_o + cp_mod[2])
    ring[pl.ds(L0, M), tile(3 * H, ND)] = mem0_ref[...].astype(F32)
    widen(P // SEG)
    next_rows(P)
    mod_part(2)
    start(cp_ffn)

    def step(s, with_norm):
        q_wr = pl.multiple_of(lax.rem(s * XR, R), 8)
        q_rd = pl.multiple_of(lax.rem(s * SEG + QOFF, R), SEG)
        o_wr = pl.multiple_of(lax.rem(s * SEG + OOFF, R), SEG)
        o_rd = pl.multiple_of(lax.rem(s * XR + OOFF, R), 8)
        h = ring[pl.ds(L0, SEG), tile(3 * H, ND)].astype(BF16)
        tail_rows = pl.ds(pl.multiple_of(jnp.maximum(s - NSEG * XR // SEG, 0) * (HG // 2), HG // 2), HG // 2)
        pad = jnp.zeros((LANE - G, LANE), BF16)

        def weights(n, d0, d):
            return pltpu.bitcast(wqkv[pl.ds(head_slab(n) + d0 // 2, d // 2), :], BF16)

        for u in range(4):
            early[u] = _dot(h[:, :DH], weights(u // 2 * H + u % 2, 0, DH))

        def head_pair(t, g):
            n = t * H + 2 * g
            mem_rows = []
            for i in range(2):
                if t < 2 and g == 0:
                    r = _dot(h[:, DH:], weights(n + i, DH, DH)) + early[2 * t + i]
                else:
                    r = _dot(h, weights(n + i, 0, D))
                ring[pl.ds(q_wr, XR), tile(n + i)] = r[M:]
                mem_rows.append(r[:M])
            return jnp.concatenate(
                mem_rows + [ring[pl.ds(q_rd, SEG), tile(n + i)] for i in range(2)],
                axis=0).astype(BF16)

        def scores(q, k):
            sc_ = lax.dot_general(q, jnp.concatenate([k, pad], axis=0), (((1,), (1,)), ((), ())),
                                  preferred_element_type=F32)
            fill = fill_ref[0:G, :]
            sc_ = jnp.where(fill == 0.0, sc_ * scale, fill)
            e = jnp.exp(sc_ - jnp.max(sc_, axis=-1, keepdims=True))
            return (e * _recip(jnp.sum(e, axis=-1, keepdims=True))).astype(BF16)

        def attend(g, p, v):
            o = _dot(p, jnp.concatenate([v, pad], axis=0))
            ops = _strassen_lhs(*(o[2 * M + i * SEG + r:2 * M + i * SEG + r + HG]
                                  for r in (0, HG) for i in range(2)))
            for i in range(7):
                ot[i, tail_rows, pl.ds(g * LANE, LANE)] = ops[i]
            for i in range(2):
                oring[pl.ds(o_wr, SEG), tile(2 * g + i)] = o[2 * M + i * SEG:2 * M + (i + 1) * SEG]
            return [jnp.concatenate([o[i * M:(i + 1) * M], oring[pl.ds(o_rd, XR), tile(2 * g + i)]],
                                    axis=0).astype(BF16) for i in range(2)]

        heads = {}

        def oproj(g0, g1, j0=0, j1=ND):
            a = jnp.concatenate([r for g in range(g0, g1) for r in heads[g]], axis=1)
            for j in range(j0, j1):
                cols = pl.ds(j * LANE, LANE)
                r = _dot(a, slab(WO + j * HD + g0 * 2 * LANE, (g1 - g0) * 2 * LANE))
                if g0 > 0:
                    r = r + acc[:, cols]
                if g1 < HP:
                    acc[:, cols] = r
                else:
                    ring[pl.ds(L0, M), tile(3 * H + j)] = r[:M]
                    xf[rows, cols] = xf[rows, cols] + mod[2, 0:1, cols] * r[M:]

        rows = pl.ds(pl.multiple_of(s * XR, 8), XR)
        qk, val = {}, {}
        for i in range(2 * HP + VALUE_LAG):
            if i == NEXT_ROWS_AT:
                widen(jnp.minimum(P // SEG + 1 + s, NSEG - 1))
                next_rows(pl.multiple_of(jnp.minimum(P + (s + 1) * XR, S - XR), 8))
            if i == FFN_NORM_AT and with_norm:
                ffn_norm(0, jnp.clip(s * XR // (2 * SEG) - 1, 0, NG - 1))
            if i < HP:
                qk[i] = head_pair(0, i), head_pair(1, i)
            elif i < 2 * HP:
                val[i - HP] = head_pair(2, i - HP)
            else:
                oproj(0, HP // 2, i - 2 * HP, i - 2 * HP + 1)
            g = i - SCORE_LAG
            if g % SCORE_GROUP == 0 and 0 < g <= HP:
                for u in range(g - SCORE_GROUP, g):
                    prob[u] = pltpu.bitcast(scores(*qk[u]), U32)
            g = i - HP - VALUE_LAG
            if g >= 0:
                heads[g] = attend(g, pltpu.bitcast(prob[g], BF16), val[g])
        oproj(0, HP // 2, VALUE_LAG, ND)
        oproj(HP // 2, HP)

    def step_pair(i, carry):
        step(2 * i, True)
        step(2 * i + 1, False)
        return carry

    lax.fori_loop(0, NSEG // 2, step_pair, 0)

    MH = FB // 2

    def row_tiles(row0, n, par, rows=LANE):
        return jnp.concatenate([slab(row0 + (2 * k + par) * rows, rows) for k in range(n // 2)], axis=0)

    def otail(j, carry):
        for u in range(2):
            ffn_norm(1, 2 * j + u)
        emit = functools.partial(residual, xf, NSEG * XR, 1, j, 2)
        _strassen(lambda i: ot[i],
                  *(row_tiles(WO + (2 * j + u) * HD, H, par) for par in range(2) for u in range(2)), emit)
        return carry

    lax.fori_loop(0, ND // 2, otail, 0)

    def norm_tail(i, carry):
        for u in range(4):
            ffn_norm(1, NG // 2 + 4 * i + u)
        return carry

    lax.fori_loop(0, NG // 8, norm_tail, 0)

    wait(cp_ffn)

    def act_slot(k, i):
        return wqkv[pl.ds((7 * k + i) * (MH // 2), MH // 2), :]

    def out_copy(blk, j):
        idx = (pl.ds(pl.multiple_of(blk * FB, FB), FB), pl.ds(pl.multiple_of(j * 2 * LANE, 2 * LANE), 2 * LANE))
        return pltpu.make_async_copy(xb.at[idx], out_hbm.at[idx], osems.at[blk * (ND // 2) + j])

    def ffn(blk, carry):
        def normed(i, j):
            return ffn_operands(blk)[operand_at(i, j, FB // 8)]

        def up(k, c):
            dst = wqkv.at[pl.ds(pl.multiple_of(k * 7 * MH, MH), 7 * MH)]
            res = {}, {}
            for t in range(2):
                w = jnp.concatenate([w13[8 * k + 2 * u + t] for u in range(4)], axis=1)
                _strassen(normed, *_quarters(w), res[t].setdefault, nested=True)
            ops = _strassen_lhs(*(_silu(res[0][n]) * res[1][n] for n in range(4)))
            for i in (1, 3, 6, 0, 2, 4, 5):
                for u in range(2):
                    dst[pl.ds((7 * u + i) * (MH // 2), MH // 2), :] = ops[i][:, u * LANE:(u + 1) * LANE]
            return c

        lax.fori_loop(0, NF // 4, up, 0)

        def down(j, c):
            emit = functools.partial(residual, xb, pl.multiple_of(blk * FB, FB), 2, j, 5)
            _strassen(lambda i: jnp.concatenate([act_slot(k, i) for k in range(NF // 2)], axis=1),
                      *(row_tiles((2 * j + u) * F, NF // 2, par, 2 * LANE) for par in range(2) for u in range(2)), emit)
            out_copy(blk, j).start()
            return c

        lax.fori_loop(0, ND // 2, down, 0)
        return carry

    lax.fori_loop(0, S // FB, ffn, 0)
    for blk in range(S // FB):
        for j in range(ND // 2):
            out_copy(blk, j).wait()


@functools.partial(jax.jit, static_argnames=("A_seg_len",))
def pallas_adaLN_cond__memory_aug_recurrent_mem_tr__glu_gated_swiglu__prompt_kernel(
    A_x, A_mem0, A_Wq, A_Wk, A_Wv, A_Wo, A_seg_len, B_x, B_w1, B_w3, B_w2, c, w_mod,
):
    del B_x
    B, S, D = A_x.shape
    _, H, Dh = A_Wq.shape
    M = A_mem0.shape[1]
    F = B_w1.shape[1]
    SEG = int(A_seg_len)
    assert (B, S, D, H, Dh, M, SEG) == (1, 2048, 1024, 32, LANE, 8, 32) and F == 3584
    P = S // SEG * M
    R = 576
    FB = 1024

    hbm = pl.BlockSpec(memory_space=pl.ANY)
    out = pl.pallas_call(
        functools.partial(_kernel, S=S, D=D, H=H, F=F, M=M, SEG=SEG, FB=FB),
        out_shape=jax.ShapeDtypeStruct((S, D), A_x.dtype),
        in_specs=[hbm] * 11,
        out_specs=hbm,
        scratch_shapes=[
            pltpu.VMEM((3 * H * (D // 2 + SLAB_PAD) + D, LANE), U32),
            pltpu.VMEM((D * H // 8, 16, LANE), BF16),
            pltpu.VMEM((2 * F // LANE, D, LANE), BF16),
            pltpu.VMEM((R, 3 * H * Dh + 7 * D // 2), F32),
            pltpu.VMEM((R, H * Dh), F32),
            pltpu.VMEM((S, D), BF16),
            pltpu.VMEM((S, D), F32),
            pltpu.VMEM((6, 8, D), F32),
            pltpu.VMEM((7, P // 2, D // 4), U32),
            pltpu.VMEM((7, P // 4, H * Dh // 2), U32),
            pltpu.VMEM((3 * SEG, LANE), F32),
            pltpu.VMEM((H // 2, M + SEG, LANE), U32),
            pltpu.VMEM((SEG, D), F32),
            pltpu.VMEM((4, SEG, LANE), F32),
            pltpu.VMEM((1, D), c.dtype),
            pltpu.VMEM((M, D), A_mem0.dtype),
            pltpu.SemaphoreType.DMA((9 + 6 * H // 16,)),
            pltpu.SemaphoreType.DMA((S // FB * D // (2 * LANE),)),
        ],
        compiler_params=pltpu.CompilerParams(vmem_limit_bytes=127 * 2**20),
        name="adaln_rmt_swiglu",
    )(A_x.reshape(S, D), A_mem0.reshape(M, D), *(w.reshape(D, H // 16, 16, Dh) for w in (A_Wq, A_Wk, A_Wv)),
      A_Wo.reshape(H * Dh // 16, 16, D), B_w1, B_w3, B_w2.reshape(F // 16, 16, D), c, w_mod)
    return out.reshape(B, S, D)
```

```python
import functools

import jax
import jax.numpy as jnp
from jax import lax
import jax.experimental.pallas as pl
import jax.experimental.pallas.tpu as pltpu

F32 = jnp.float32
BF16 = jnp.bfloat16
U32 = jnp.uint32
LANE = 128
EPS = 1e-5
SLAB_PAD = 4
SCORE_GROUP = 4
SCORE_LAG = 2
VALUE_LAG = 3
FFN_NORM_AT = 24
NEXT_ROWS_AT = 18


def _dot(a, b):
    return jnp.dot(a, b, preferred_element_type=F32)


def _norm(x):
    m = jnp.mean(x, axis=-1, keepdims=True)
    d = x - m
    v = jnp.mean(d * d, axis=-1, keepdims=True)
    return d * lax.rsqrt(v + EPS)


def _ada_ln(x, shift, scale1):
    return _norm(x) * scale1 + shift


def _recip(x):
    return pl.reciprocal(x, approx=True)


def _silu(x):
    return x * _recip(1.0 + jnp.exp(-x))


def _words(x):
    return pltpu.bitcast(x.astype(BF16), U32)


def _lhs_sums(a11, a12, a21, a22):
    return a11 + a22, a21 + a22, a11, a22, a11 + a12, a21 - a11, a12 - a22


def _strassen_lhs(*blocks):
    return [_words(a) for a in _lhs_sums(*blocks)]


def _quarters(a):
    r, c = a.shape[0] // 2, a.shape[1] // 2
    return a[:r, :c], a[:r, c:], a[r:, :c], a[r:, c:]


def _strassen(lhs_fn, b11, b12, b21, b22, emit, nested=False):
    f11, f12, f21, f22 = (b.astype(F32) for b in (b11, b12, b21, b22))

    def prod(i, b):
        if not nested:
            return _dot(pltpu.bitcast(lhs_fn(i), BF16), b.astype(BF16))
        c = {}
        _strassen(functools.partial(lhs_fn, i), *_quarters(b), c.setdefault)
        return jnp.concatenate([jnp.concatenate([c[0], c[1]], axis=1),
                                jnp.concatenate([c[2], c[3]], axis=1)], axis=0)

    m2 = prod(1, b11)
    m4 = prod(3, f21 - f11)
    emit(2, m2 + m4)
    m3 = prod(2, f12 - f22)
    m5 = prod(4, b22)
    emit(1, m3 + m5)
    m1 = prod(0, f11 + f22)
    emit(3, (m1 - m2 + m3) + prod(5, f11 + f12))
    emit(0, (m1 + m4 - m5) + prod(6, f21 + f22))


def _kernel(x_hbm, mem0_hbm, wq_hbm, wk_hbm, wv_hbm, wo_hbm, w1_hbm, w3_hbm, w2_hbm,
            c_hbm, wmod_hbm, out_hbm,
            wqkv, big, w13, ring, oring, xb, xf, mod, ot, fill_ref, prob, acc, early, c_ref, mem0_ref,
            sems, osems,
            *, S, D, H, F, M, SEG, FB):
    NSEG = S // SEG
    XR = SEG - M
    P = S - NSEG * XR
    R = ring.shape[0]
    QOFF = R - P
    OOFF = (-NSEG * XR) % R
    ND = D // LANE
    NF = F // LANE
    HP = H // 2
    HD = H * LANE
    scale = float(LANE) ** -0.5
    DH = D // 2
    PG = 8
    NA = HP // PG
    NSLOT = big.shape[0] // DH
    WP = DH + SLAB_PAD
    WO = ND * HD

    def tile(n, width=1):
        return pl.ds(n * LANE if isinstance(n, int) else pl.multiple_of(n * LANE, LANE), width * LANE)

    def head_slab(n):
        return (n // (2 * PG) * 2 * PG + n % 2 * PG + n % (2 * PG) // 2) * WP

    def slab(row0, rows):
        return big[pl.ds(row0 // 16, rows // 16)].reshape(rows, LANE)

    def slab_copies(src, tiles, dst_fn, sem):
        return [pltpu.make_async_copy(src.at[..., pl.ds(j * LANE, LANE)], dst_fn(j), sem) for j in tiles]

    def half_tiles(c):
        return [v * ND + c * ND // 2 + j for v in range(2) for j in range(ND // 2)]

    cp_x0 = pltpu.make_async_copy(x_hbm.at[pl.ds(0, P)], xb.at[pl.ds(0, P)], sems.at[0])
    cp_x1 = pltpu.make_async_copy(x_hbm.at[pl.ds(P, S - P)], xb.at[pl.ds(P, S - P)], sems.at[1])
    mod_tiles = [half_tiles(0), half_tiles(1), list(range(2 * ND, 6 * ND))]
    cp_mod = [slab_copies(wmod_hbm, t, lambda j: w13.at[j], sems.at[2 + i])
              for i, t in enumerate(mod_tiles)]
    cp_w = [pltpu.make_async_copy(w.at[pl.ds(c * DH, DH), a],
                                  big.at[pl.ds(((2 * t + c) * NA + a) % NSLOT * DH, DH)],
                                  sems.at[7 + (2 * t + c) * NA + a])
            for t, w in enumerate((wq_hbm, wk_hbm, wv_hbm)) for c in range(2) for a in range(NA)]
    cp_o = slab_copies(wo_hbm, range(ND), lambda j: big.at[pl.ds((WO + j * HD) // 16, HD // 16)], sems.at[5])
    cp_ffn = (slab_copies(w1_hbm, range(NF), lambda j: w13.at[2 * j], sems.at[6])
              + slab_copies(w3_hbm, range(NF), lambda j: w13.at[2 * j + 1], sems.at[6])
              + slab_copies(w2_hbm, range(ND), lambda j: big.at[pl.ds(j * F // 16, F // 16)], sems.at[6]))

    def start(cps):
        for cp in cps:
            cp.start()

    def wait(cps):
        for cp in cps:
            cp.wait()

    cp_c = pltpu.make_async_copy(c_hbm, c_ref, sems.at[7 + len(cp_w)])
    cp_mem = pltpu.make_async_copy(mem0_hbm, mem0_ref, sems.at[8 + len(cp_w)])
    cp_c.start()
    start(cp_mod[0])
    cp_x0.start()
    cp_w[0].start()
    cp_mem.start()
    cp_c.wait()

    cc = jnp.broadcast_to(c_ref[...].astype(F32), (16, D))
    sc = _silu(cc).astype(BF16)

    def mod_part(i):
        for j in mod_tiles[i]:
            r = _dot(sc, w13[j])[0:8]
            if j // ND in (1, 4):
                r = r + 1.0
            mod[j // ND, :, pl.ds((j % ND) * LANE, LANE)] = r

    def modv(i):
        return mod[i, 0:1, :]

    G = 2 * (M + SEG)
    ri = lax.broadcasted_iota(jnp.int32, (G, LANE), 0)
    ci = lax.broadcasted_iota(jnp.int32, (G, LANE), 1)

    def head_pos(i):
        head = jnp.where(i < 2 * M, i // M, (i - 2 * M) // SEG)
        pos = jnp.where(i < 2 * M, i % M, M + (i - 2 * M) % SEG)
        return head, pos

    rh, rp = head_pos(ri)
    ch, cp_ = head_pos(ci)
    visible = (rp < M) | (rp >= cp_)
    fill_ref[0:G, :] = jnp.where(rh == ch, jnp.where(visible, 0.0, -1e9), -jnp.inf).astype(F32)

    LB = 128
    PH = P // 2
    DQ = D // 4

    def norm_half(c):
        cols = slice(c * DH, (c + 1) * DH)

        def norm0(k, carry):
            halves = []
            for o in (0, PH):
                rows = pl.ds(pl.multiple_of(o + k * LB, LB), LB)
                if c == 0:
                    xv = xb[rows, :].astype(F32)
                    xf[rows, :] = xv
                    xn = _norm(xv)
                    oring[rows, 0:DH] = xn[:, DH:]
                    xn = xn[:, :DH]
                else:
                    xn = oring[rows, 0:DH]
                halves.append(xn * mod[1, 0:1, cols] + mod[0, 0:1, cols])
            top, bot = halves
            ops = _strassen_lhs(top[:, :DQ], top[:, DQ:], bot[:, :DQ], bot[:, DQ:])
            for i in range(7):
                ot[i, pl.ds(pl.multiple_of(k * (LB // 2), LB // 2), LB // 2), tile(4 * c, 2)] = ops[i]
            return carry

        lax.fori_loop(0, PH // LB, norm0, 0)

    def arrivals(it):
        if it == 0:
            cp_w[0].wait()
            start(cp_w[2:3] + cp_mod[1] + cp_w[3:4])
        else:
            wait(cp_w[it + (it > 1):it + 2])
        if it == 1:
            start(cp_w[4:6])
        if it == NA:
            start(cp_w[6:NSLOT])
            wait(cp_mod[1])
            mod_part(1)
            norm_half(1)
        if it == 4:
            start(cp_w[NSLOT:] + [cp_x1] + cp_mod[2])
        if it == NSLOT - 1:
            wait(cp_w[it + 2:])
            start(cp_o)

    def head_rows(it):
        chunk, a = it // NA, it % NA
        base = (chunk // 2 * H + 2 * PG * a) * WP + chunk % 2 * (DH // 2)
        return wqkv.at[pl.ds(pl.multiple_of(base, 32), (2 * PG + 1) * WP)]

    def retile(it, r0, r1):
        src = big.at[pl.ds(it % NSLOT * DH, DH)]
        dst = head_rows(it)
        for r in range(r0, r1):
            even, odd = pltpu.bitcast(src[2 * r], U32), pltpu.bitcast(src[2 * r + 1], U32)
            dst[pl.ds(r, PG, stride=WP), :] = (even & jnp.uint32(0xFFFF)) | (odd << 16)
            dst[pl.ds(PG * WP + r, PG, stride=WP), :] = (even >> 16) | (odd & jnp.uint32(0xFFFF0000))

    def project(it, carry):
        for ev in range(NSLOT):
            pl.when(it == ev)(functools.partial(arrivals, ev))
        pl.when(it < 2)(lambda: retile(it, 0, DH // 2))
        half = it // NA % 2
        normed = ot.at[:, :, tile(4 * half, 2)]
        nxt = jnp.where(it == 0, 0, jnp.minimum(it + 1, 6 * NA - 1))
        dst = ring.at[:, tile(it // (2 * NA) * H + 2 * PG * (it % NA), 2 * PG)]
        for b in range(PG):
            lo, hi = (pltpu.bitcast(head_rows(it)[pl.ds((i * PG + b) * WP, DH // 2), :], BF16)
                      for i in range(2))

            def emit(i, r, b=b):
                idx = pl.ds(QOFF + i // 2 * PH, PH), tile(2 * b + i % 2)
                dst[idx] = r + jnp.where(half == 1, dst[idx], 0.0)

            _strassen(lambda i: normed[i], lo[:DQ], hi[:DQ], lo[DQ:], hi[DQ:], emit)
            retile(nxt, b * (DH // 2) // PG, (b + 1) * (DH // 2) // PG)
        return carry

    wait(cp_mod[0])
    mod_part(0)
    cp_x0.wait()
    norm_half(0)
    cp_w[1].start()
    lax.fori_loop(0, 6 * NA, project, 0)

    HG = SEG // 2

    def residual(dst, row0, parts, j, gate, n, y):
        cols = tile(2 * j + n % 2)
        y = mod[gate, 0:1, cols] * y
        per = y.shape[0] // HG // parts
        for u in range(per * parts):
            rows = pl.ds(row0 + (u % per * parts + u // per) * SEG + n // 2 * HG, HG)
            dst[rows, cols] = (xf[rows, cols] + y[u * HG:(u + 1) * HG]).astype(dst.dtype)

    NG = FB // (2 * SEG)

    def ffn_operands(blk):
        return ring.at[:, tile((1 - blk) * 3 * H, 7 * ND // 2)]

    def operand_at(i, j, rows):
        m = 7 * i + j
        return pl.ds(m % 4 * (FB // 8), rows), tile(m // 4 * 2, 2)

    def ffn_norm(blk, grp):
        hn = _ada_ln(xf[pl.ds(pl.multiple_of(blk * FB + grp * 2 * SEG, 2 * SEG), 2 * SEG), :],
                     modv(3), modv(4))
        hn = jnp.concatenate([hn[q * HG:(q + 1) * HG] for q in (0, 2, 1, 3)], axis=0)
        dst = ffn_operands(blk).at[pl.ds(pl.multiple_of(grp * (HG // 2), HG // 2), 3 * FB // 8 + HG // 2)]
        for i, a in enumerate(_lhs_sums(*_quarters(hn))):
            for j, op in enumerate(_strassen_lhs(*_quarters(a))):
                dst[operand_at(i, j, HG // 2)] = pltpu.bitcast(op, F32)

    L0 = S // 4

    def widen(grp):
        rows = pl.ds(pl.multiple_of(grp * SEG, SEG), SEG)
        xf[rows, :] = xb[rows, :].astype(F32)

    def next_rows(r0):
        ring[pl.ds(L0 + M, XR), tile(3 * H, ND)] = _ada_ln(xf[pl.ds(r0, XR), :], modv(0), modv(1))

    wait([cp_mem, cp_x1] + cp_o + cp_mod[2])
    ring[pl.ds(L0, M), tile(3 * H, ND)] = mem0_ref[...].astype(F32)
    widen(P // SEG)
    next_rows(P)
    mod_part(2)
    start(cp_ffn)

    def step(s, with_norm):
        q_wr = pl.multiple_of(lax.rem(s * XR, R), 8)
        q_rd = pl.multiple_of(lax.rem(s * SEG + QOFF, R), SEG)
        o_wr = pl.multiple_of(lax.rem(s * SEG + OOFF, R), SEG)
        o_rd = pl.multiple_of(lax.rem(s * XR + OOFF, R), 8)
        h = ring[pl.ds(L0, SEG), tile(3 * H, ND)].astype(BF16)
        tail_rows = pl.ds(pl.multiple_of(jnp.maximum(s - NSEG * XR // SEG, 0) * (HG // 2), HG // 2), HG // 2)
        pad = jnp.zeros((LANE - G, LANE), BF16)

        def weights(n, d0, d):
            return pltpu.bitcast(wqkv[pl.ds(head_slab(n) + d0 // 2, d // 2), :], BF16)

        for u in range(4):
            early[u] = _dot(h[:, :DH], weights(u // 2 * H + u % 2, 0, DH))

        def head_pair(t, g):
            n = t * H + 2 * g
            mem_rows = []
            for i in range(2):
                if t < 2 and g == 0:
                    r = _dot(h[:, DH:], weights(n + i, DH, DH)) + early[2 * t + i]
                else:
                    r = _dot(h, weights(n + i, 0, D))
                ring[pl.ds(q_wr, XR), tile(n + i)] = r[M:]
                mem_rows.append(r[:M])
            return jnp.concatenate(
                mem_rows + [ring[pl.ds(q_rd, SEG), tile(n + i)] for i in range(2)],
                axis=0).astype(BF16)

        def scores(q, k):
            sc_ = lax.dot_general(q, jnp.concatenate([k, pad], axis=0), (((1,), (1,)), ((), ())),
                                  preferred_element_type=F32)
            fill = fill_ref[0:G, :]
            sc_ = jnp.where(fill == 0.0, sc_ * scale, fill)
            e = jnp.exp(sc_ - jnp.max(sc_, axis=-1, keepdims=True))
            return (e * _recip(jnp.sum(e, axis=-1, keepdims=True))).astype(BF16)

        def attend(g, p, v):
            o = _dot(p, jnp.concatenate([v, pad], axis=0))
            ops = _strassen_lhs(*(o[2 * M + i * SEG + r:2 * M + i * SEG + r + HG]
                                  for r in (0, HG) for i in range(2)))
            for i in range(7):
                ot[i, tail_rows, pl.ds(g * LANE, LANE)] = ops[i]
            for i in range(2):
                oring[pl.ds(o_wr, SEG), tile(2 * g + i)] = o[2 * M + i * SEG:2 * M + (i + 1) * SEG]
            return [jnp.concatenate([o[i * M:(i + 1) * M], oring[pl.ds(o_rd, XR), tile(2 * g + i)]],
                                    axis=0).astype(BF16) for i in range(2)]

        heads = {}

        def oproj(g0, g1, j0=0, j1=ND):
            a = jnp.concatenate([r for g in range(g0, g1) for r in heads[g]], axis=1)
            for j in range(j0, j1):
                cols = pl.ds(j * LANE, LANE)
                r = _dot(a, slab(WO + j * HD + g0 * 2 * LANE, (g1 - g0) * 2 * LANE))
                if g0 > 0:
                    r = r + acc[:, cols]
                if g1 < HP:
                    acc[:, cols] = r
                else:
                    ring[pl.ds(L0, M), tile(3 * H + j)] = r[:M]
                    xf[rows, cols] = xf[rows, cols] + mod[2, 0:1, cols] * r[M:]

        rows = pl.ds(pl.multiple_of(s * XR, 8), XR)
        qk, val = {}, {}
        for i in range(2 * HP + VALUE_LAG):
            if i == NEXT_ROWS_AT:
                widen(jnp.minimum(P // SEG + 1 + s, NSEG - 1))
                next_rows(pl.multiple_of(jnp.minimum(P + (s + 1) * XR, S - XR), 8))
            if i == FFN_NORM_AT and with_norm:
                ffn_norm(0, jnp.clip(s * XR // (2 * SEG) - 1, 0, NG - 1))
            if i < HP:
                qk[i] = head_pair(0, i), head_pair(1, i)
            elif i < 2 * HP:
                val[i - HP] = head_pair(2, i - HP)
            else:
                oproj(0, HP // 2, i - 2 * HP, i - 2 * HP + 1)
            g = i - SCORE_LAG
            if g % SCORE_GROUP == 0 and 0 < g <= HP:
                for u in range(g - SCORE_GROUP, g):
                    prob[u] = pltpu.bitcast(scores(*qk[u]), U32)
            g = i - HP - VALUE_LAG
            if g >= 0:
                heads[g] = attend(g, pltpu.bitcast(prob[g], BF16), val[g])
        oproj(0, HP // 2, VALUE_LAG, ND)
        oproj(HP // 2, HP)

    def step_pair(i, carry):
        step(2 * i, True)
        step(2 * i + 1, False)
        return carry

    lax.fori_loop(0, NSEG // 2, step_pair, 0)

    MH = FB // 2

    def row_tiles(row0, n, par, rows=LANE):
        return jnp.concatenate([slab(row0 + (2 * k + par) * rows, rows) for k in range(n // 2)], axis=0)

    def otail(j, carry):
        for u in range(2):
            ffn_norm(1, 2 * j + u)
        emit = functools.partial(residual, xf, NSEG * XR, 1, j, 2)
        _strassen(lambda i: ot[i],
                  *(row_tiles(WO + (2 * j + u) * HD, H, par) for par in range(2) for u in range(2)), emit)
        return carry

    lax.fori_loop(0, ND // 2, otail, 0)

    def norm_tail(i, carry):
        for u in range(4):
            ffn_norm(1, NG // 2 + 4 * i + u)
        return carry

    lax.fori_loop(0, NG // 8, norm_tail, 0)

    wait(cp_ffn)

    def act_slot(k, i):
        return wqkv[pl.ds((7 * k + i) * (MH // 2), MH // 2), :]

    def out_copy(blk, j):
        idx = (pl.ds(pl.multiple_of(blk * FB, FB), FB), pl.ds(pl.multiple_of(j * 2 * LANE, 2 * LANE), 2 * LANE))
        return pltpu.make_async_copy(xb.at[idx], out_hbm.at[idx], osems.at[blk * (ND // 2) + j])

    def ffn(blk, carry):
        def normed(i, j):
            return ffn_operands(blk)[operand_at(i, j, FB // 8)]

        def up(k, c):
            dst = wqkv.at[pl.ds(pl.multiple_of(k * 7 * MH, MH), 7 * MH)]
            res = {}, {}
            for t in range(2):
                w = jnp.concatenate([w13[8 * k + 2 * u + t] for u in range(4)], axis=1)
                _strassen(normed, *_quarters(w), res[t].setdefault, nested=True)
            ops = _strassen_lhs(*(_silu(res[0][n]) * res[1][n] for n in range(4)))
            for i in (1, 3, 6, 0, 2, 4, 5):
                for u in range(2):
                    dst[pl.ds((7 * u + i) * (MH // 2), MH // 2), :] = ops[i][:, u * LANE:(u + 1) * LANE]
            return c

        lax.fori_loop(0, NF // 4, up, 0)

        def down(j, c):
            emit = functools.partial(residual, xb, pl.multiple_of(blk * FB, FB), 2, j, 5)
            _strassen(lambda i: jnp.concatenate([act_slot(k, i) for k in range(NF // 2)], axis=1),
                      *(row_tiles((2 * j + u) * F, NF // 2, par, 2 * LANE) for par in range(2) for u in range(2)), emit)
            out_copy(blk, j).start()
            return c

        lax.fori_loop(0, ND // 2, down, 0)
        return carry

    lax.fori_loop(0, S // FB, ffn, 0)
    for blk in range(S // FB):
        for j in range(ND // 2):
            out_copy(blk, j).wait()


@functools.partial(jax.jit, static_argnames=("A_seg_len",))
def pallas_adaLN_cond__memory_aug_recurrent_mem_tr__glu_gated_swiglu__prompt_kernel(
    A_x, A_mem0, A_Wq, A_Wk, A_Wv, A_Wo, A_seg_len, B_x, B_w1, B_w3, B_w2, c, w_mod,
):
    del B_x
    B, S, D = A_x.shape
    _, H, Dh = A_Wq.shape
    M = A_mem0.shape[1]
    F = B_w1.shape[1]
    SEG = int(A_seg_len)
    assert (B, S, D, H, Dh, M, SEG) == (1, 2048, 1024, 32, LANE, 8, 32) and F == 3584
    P = S // SEG * M
    R = 576
    FB = 1024

    hbm = pl.BlockSpec(memory_space=pl.ANY)
    out = pl.pallas_call(
        functools.partial(_kernel, S=S, D=D, H=H, F=F, M=M, SEG=SEG, FB=FB),
        out_shape=jax.ShapeDtypeStruct((S, D), A_x.dtype),
        in_specs=[hbm] * 11,
        out_specs=hbm,
        scratch_shapes=[
            pltpu.VMEM((3 * H * (D // 2 + SLAB_PAD) + D, LANE), U32),
            pltpu.VMEM((D * H // 8, 16, LANE), BF16),
            pltpu.VMEM((2 * F // LANE, D, LANE), BF16),
            pltpu.VMEM((R, 3 * H * Dh + 7 * D // 2), F32),
            pltpu.VMEM((R, H * Dh), F32),
            pltpu.VMEM((S, D), BF16),
            pltpu.VMEM((S, D), F32),
            pltpu.VMEM((6, 8, D), F32),
            pltpu.VMEM((7, P // 4, H * Dh // 2), U32),
            pltpu.VMEM((3 * SEG, LANE), F32),
            pltpu.VMEM((H // 2, M + SEG, LANE), U32),
            pltpu.VMEM((SEG, D), F32),
            pltpu.VMEM((4, SEG, LANE), F32),
            pltpu.VMEM((1, D), c.dtype),
            pltpu.VMEM((M, D), A_mem0.dtype),
            pltpu.SemaphoreType.DMA((9 + 6 * H // 16,)),
            pltpu.SemaphoreType.DMA((S // FB * D // (2 * LANE),)),
        ],
        compiler_params=pltpu.CompilerParams(vmem_limit_bytes=127 * 2**20),
        name="adaln_rmt_swiglu",
    )(A_x.reshape(S, D), A_mem0.reshape(M, D), *(w.reshape(D, H // 16, 16, Dh) for w in (A_Wq, A_Wk, A_Wv)),
      A_Wo.reshape(H * Dh // 16, 16, D), B_w1, B_w3, B_w2.reshape(F // 16, 16, D), c, w_mod)
    return out.reshape(B, S, D)
```
